```python
import jax
import jax.numpy as jnp

def _softmax(x, axis=-1):
    return jax.nn.softmax(x, axis=axis)

def _gelu(x):
    return jax.nn.gelu(x, approximate=True)

def _silu(x):
    return jax.nn.silu(x)

def _sigmoid(x):
    return jax.nn.sigmoid(x)

def _layernorm(x, axis=-1, eps=1e-05):
    m = jnp.mean(x, axis=axis, keepdims=True)
    v = jnp.var(x, axis=axis, keepdims=True)
    return (x - m) / jnp.sqrt(v + eps)

def _scatter_add(tgt, idx, src, axis=0):
    return tgt.at[idx].add(src)

def _segment_sum(src, seg, n):
    return jax.ops.segment_sum(src, seg, n)

class _Rng:

    def __init__(self, key):
        self._k = key

    def _next(self):
        self._k, sub = jax.random.split(self._k)
        return sub

    def normal(self, shape):
        return jax.random.normal(self._next(), shape, dtype=jnp.bfloat16)

    def randint(self, lo, hi, shape):
        return jax.random.randint(self._next(), shape, lo, hi, dtype=jnp.int32)

    def uniform(self, shape, lo=0.0, hi=1.0):
        return jax.random.uniform(self._next(), shape, jnp.bfloat16, lo, hi)

    def permutation(self, n):
        return jax.random.permutation(self._next(), n)
kernel_name = 'interleave_layers__linear_kernel_hedgehog__memory_aug_recurrent_mem_tr__prompt'

def setup_inputs():
    _rng = _Rng(jax.random.key(int.from_bytes(__import__("os").urandom(4), "little")))
    _w = lambda a: (lambda t: t.astype(jnp.bfloat16) if jnp.issubdtype(t.dtype, jnp.floating) else t)(jnp.asarray(a))

    def _A_setup():
        B, S, D, H = (1, 2048, 640, 32)
        Dh = D // H
        return {'x': _w((lambda *s: _rng.normal(s) * 0.05)(B, S, D)), 'wqkv': _w((lambda *s: _rng.normal(s) * 0.05)(D, 3 * D)), 'w_phi': _w((lambda *s: _rng.normal(s) * 0.05)(H, Dh, Dh) * Dh ** (-0.5)), 'wo': _w((lambda *s: _rng.normal(s) * 0.05)(D, D))}
    _A_in = _A_setup()

    def _B_setup():
        B, S, Dm = (1, 2048, 640)
        H, Dh = (32, 192)
        M, seg = (8, 32)
        seg = min(seg, S)
        S = S // seg * seg
        return {'x': _w((lambda *s: _rng.normal(s) * 0.05)(B, S, Dm)), 'mem0': _w((lambda *s: _rng.normal(s) * 0.05)(B, M, Dm)), 'Wq': _w((lambda *s: _rng.normal(s) * 0.05)(Dm, H, Dh) * Dm ** (-0.5)), 'Wk': _w((lambda *s: _rng.normal(s) * 0.05)(Dm, H, Dh) * Dm ** (-0.5)), 'Wv': _w((lambda *s: _rng.normal(s) * 0.05)(Dm, H, Dh) * Dm ** (-0.5)), 'Wo': _w((lambda *s: _rng.normal(s) * 0.05)(H, Dh, Dm) * (H * Dh) ** (-0.5)), 'seg_len': seg}
    _B_in = _B_setup()
    return {'A_x': _A_in['x'], 'A_wqkv': _A_in['wqkv'], 'A_w_phi': _A_in['w_phi'], 'A_wo': _A_in['wo'], 'B_x': _B_in['x'], 'B_mem0': _B_in['mem0'], 'B_Wq': _B_in['Wq'], 'B_Wk': _B_in['Wk'], 'B_Wv': _B_in['Wv'], 'B_Wo': _B_in['Wo'], 'B_seg_len': _B_in['seg_len']}

def reference(A_x, A_wqkv, A_w_phi, A_wo, B_x, B_mem0, B_Wq, B_Wk, B_Wv, B_Wo, B_seg_len):

    def _A_ref(x, wqkv, w_phi, wo):
        B, S, D = x.shape
        H = 32
        Dh = D // H
        qkv = (lambda x, *d: x.transpose(*d))((x @ wqkv).reshape(B, S, 3, H, Dh), 2, 0, 3, 1, 4)
        q, k, v = (qkv[0], qkv[1], qkv[2])
        pq = jnp.einsum('bhsd,hdf->bhsf', q, w_phi)
        pk = jnp.einsum('bhsd,hdf->bhsf', k, w_phi)
        phi_q = jnp.concatenate([_softmax(pq, axis=-1), _softmax(-pq, axis=-1)], axis=-1)
        phi_k = jnp.concatenate([_softmax(pk, axis=-1), _softmax(-pk, axis=-1)], axis=-1)
        kv = jnp.einsum('bhsf,bhsd->bhfd', phi_k, v)
        z = jnp.einsum('bhsf->bhf', phi_k)
        num = jnp.einsum('bhqf,bhfd->bhqd', phi_q, kv)
        den = jnp.einsum('bhqf,bhf->bhq', phi_q, z)[..., None] + 1e-06
        o = num / den
        return (lambda x, *d: x.transpose(*d))(o, 0, 2, 1, 3).reshape(B, S, D) @ wo

    def _B_ref(x, mem0, Wq, Wk, Wv, Wo, seg_len):
        B, S, Dm = x.shape
        H, Dh = (Wq.shape[1], Wq.shape[2])
        M = mem0.shape[1]
        scale = Dh ** (-0.5)
        n_seg = S // seg_len
        L = M + seg_len
        idx = jnp.arange(L)
        mask = (idx[:, None] < M) | (idx[:, None] >= idx[None, :])
        mem = mem0
        outs = []
        for s in range(n_seg):
            xs = x[:, s * seg_len:(s + 1) * seg_len, :].copy()
            h = jnp.concatenate([mem, xs], axis=1)
            q = jnp.einsum('btd,dhe->bhte', h, Wq)
            k = jnp.einsum('btd,dhe->bhte', h, Wk)
            v = jnp.einsum('btd,dhe->bhte', h, Wv)
            scores = jnp.einsum('bhqe,bhke->bhqk', q, k) * scale
            scores = jnp.where(mask[None, None], scores, -1000000000.0)
            p = _softmax(scores, axis=-1)
            o = jnp.einsum('bhqk,bhke->bhqe', p, v)
            o = jnp.einsum('bhte,hed->btd', o, Wo)
            mem = o[:, :M, :].copy()
            outs.append(o[:, M:, :])
        return jnp.concatenate(outs, axis=1)
    x = A_x
    x = x + _A_ref(_layernorm(x, axis=-1), A_wqkv, A_w_phi, A_wo)
    x = x + _B_ref(_layernorm(x, axis=-1), B_mem0, B_Wq, B_Wk, B_Wv, B_Wo, B_seg_len)
    x = x + _A_ref(_layernorm(x, axis=-1), A_wqkv, A_w_phi, A_wo)
    x = x + _B_ref(_layernorm(x, axis=-1), B_mem0, B_Wq, B_Wk, B_Wv, B_Wo, B_seg_len)
    return x
```

```python
import functools

import jax
import jax.numpy as jnp
import jax.experimental.pallas as pl
import jax.experimental.pallas.tpu as pltpu

F32 = jnp.float32
BF16 = jnp.bfloat16

S = 2048
D = 640
HA = 32
DA = 20
HB = 32
DB = 192
NM = 8
SEG = 32
NPAIR = HB // 2
TB = 512
LN_EPS = 1e-5

_NN = (((1,), (0,)), ((), ()))
_NT = (((1,), (1,)), ((), ()))


def _dot(a, b):
    return jax.lax.dot_general(a, b, _NN, preferred_element_type=F32)


def _dot_nt(a, b):
    return jax.lax.dot_general(a, b, _NT, preferred_element_type=F32)


def _ln(x):
    m = jnp.mean(x, axis=-1, keepdims=True)
    xc = x - m
    v = jnp.mean(xc * xc, axis=-1, keepdims=True)
    return xc * jax.lax.rsqrt(v + LN_EPS)


def _iota(shape, dim):
    return jax.lax.broadcasted_iota(jnp.int32, shape, dim)


def _div20(i):
    return (i * 3277) >> 16


def _kernel(x_hbm, wqkv_hbm, wphi_ref, wo_hbm, mem0_ref, wqt_hbm, wkt_hbm, wvt_hbm, bwo_hbm,
            out_hbm,
            xin, wqkv, woa, wt, wb, bwo, xres, xn32, xnb, wqp, wkpt, kvacc, zacc, zrow,
            kvwo32, kvwo, memv, sqkv, so, sems):
    cp_x = pltpu.make_async_copy(x_hbm, xin, sems.at[0])
    cp_wqkv = pltpu.make_async_copy(wqkv_hbm, wqkv, sems.at[1])
    cp_wo = pltpu.make_async_copy(wo_hbm, woa, sems.at[2])
    cp_x.start()
    cp_wqkv.start()
    cp_wo.start()
    cp_big = [
        pltpu.make_async_copy(wqt_hbm, wt.at[0], sems.at[3]),
        pltpu.make_async_copy(wkt_hbm, wt.at[1], sems.at[4]),
        pltpu.make_async_copy(wvt_hbm, wt.at[2], sems.at[5]),
        pltpu.make_async_copy(bwo_hbm, bwo, sems.at[6]),
    ]

    wphi = wphi_ref[...].astype(F32)
    wd = jnp.concatenate([wphi[:, f, :] for f in range(DA)], axis=1)
    wd = jnp.concatenate([wd, jnp.zeros((128 - DA, D), F32)], axis=0).astype(BF16)
    r = _iota((D, 128), 0)
    c = _iota((D, 128), 1)
    sel = jnp.where(r - _div20(r) * DA == c, 1.0, 0.0).astype(BF16)
    r = _iota((D, D), 0)
    c = _iota((D, D), 1)
    phi = jnp.where(_div20(r) == (c & (HA - 1)), _dot(sel, wd), 0.0).astype(BF16)

    cp_x.wait()
    cp_wqkv.wait()
    cp_wo.wait()
    for cp in cp_big:
        cp.start()

    wqp[...] = _dot(wqkv[:, 0:D], phi).astype(BF16)
    wkpt[...] = _dot(wqkv[:, D:2 * D], phi).T.astype(BF16)

    def init_blk(i, carry):
        rows = pl.ds(pl.multiple_of(i * 256, 256), 256)
        x = xin[rows, :].astype(F32)
        xres[rows, :] = x
        xnb[rows, :] = _ln(x).astype(BF16)
        return carry

    jax.lax.fori_loop(0, S // 256, init_blk, 0)

    def layer_a():
        kvacc[...] = jnp.zeros_like(kvacc)
        zacc[...] = jnp.zeros_like(zacc)

        def phase1(i, carry):
            rows = pl.ds(pl.multiple_of(i * TB, TB), TB)
            xn = xnb[rows, :]
            pkt = _dot_nt(wkpt[...], xn).reshape(DA, HA, TB)
            v = _dot(xn, wqkv[:, 2 * D:3 * D]).astype(BF16)
            for g in range(4):
                pk = pkt[:, 8 * g:8 * g + 8, :]
                mx = jnp.max(pk, axis=0, keepdims=True)
                mn = jnp.min(pk, axis=0, keepdims=True)
                ep = jnp.exp(pk - mx)
                en = jnp.exp(mn - pk)
                ep = ep * (1.0 / jnp.sum(ep, axis=0, keepdims=True))
                en = en * (1.0 / jnp.sum(en, axis=0, keepdims=True))
                ph = jnp.concatenate([ep, en], axis=0)
                zp = ph[:, :, 0:128]
                for t in range(1, TB // 128):
                    zp = zp + ph[:, :, t * 128:(t + 1) * 128]
                zacc[:, 8 * g:8 * g + 8, :] += zp
                lhs = ph.reshape(2 * DA * 8, TB).astype(BF16)
                kvacc[g] += _dot(lhs, v[:, 128 * g:128 * g + 256])
            return carry

        jax.lax.fori_loop(0, S // TB, phase1, 0)

        zt = zacc[...].reshape(2 * DA * HA, 128).T
        zrow[...] = jnp.broadcast_to(jnp.sum(zt, axis=0, keepdims=True), zrow.shape)
        rr = _iota((2 * DA * 8, 256), 0) & 7
        cc = _iota((2 * DA * 8, 256), 1)
        for g in range(4):
            keep = _div20(cc + 128 * g) == rr + 8 * g
            kvm = jnp.where(keep, kvacc[g], 0.0).astype(BF16)
            tg = _dot(kvm, woa[128 * g:128 * g + 256, :])
            kvwo32[:, 8 * g:8 * g + 8, :] = tg.reshape(2 * DA, 8, D)
        kvwo[...] = kvwo32[...].reshape(2 * DA * HA, D).astype(BF16)

        def lane_all(x, op):
            x = op(x, pltpu.roll(x, 32, 1))
            return op(x, pltpu.roll(x, 64, 1))

        def phase2(i, carry):
            rows = pl.ds(pl.multiple_of(i * TB, TB), TB)
            pq = _dot(xnb[rows, :], wqp[...])
            ts = [pq[:, 128 * t:128 * (t + 1)] for t in range(5)]
            mx = lane_all(functools.reduce(jnp.maximum, ts), jnp.maximum)
            mn = lane_all(functools.reduce(jnp.minimum, ts), jnp.minimum)
            ep = [jnp.exp(t - mx) for t in ts]
            en = [jnp.exp(mn - t) for t in ts]
            z = zrow[0:1, :]
            rp = 1.0 / lane_all(functools.reduce(jnp.add, ep), jnp.add)
            rn = 1.0 / lane_all(functools.reduce(jnp.add, en), jnp.add)
            tp = functools.reduce(
                jnp.add, [ep[t] * z[:, 128 * t:128 * (t + 1)] for t in range(5)])
            tn = functools.reduce(
                jnp.add, [en[t] * z[:, D + 128 * t:D + 128 * (t + 1)] for t in range(5)])
            rden = 1.0 / (lane_all(tp * rp + tn * rn, jnp.add) + 1e-6)
            cp_ = rp * rden
            cn_ = rn * rden
            lhs = jnp.concatenate(
                [(e * cp_).astype(BF16) for e in ep] + [(e * cn_).astype(BF16) for e in en],
                axis=1)
            xnew = xres[rows, :] + _dot(lhs, kvwo[...])
            xres[rows, :] = xnew
            xn32[rows, :] = _ln(xnew)
            return carry

        jax.lax.fori_loop(0, S // TB, phase2, 0)

    scale = DB ** (-0.5)

    def layer_b(layer):
        L = SEG + NM
        rr = _iota((L, 128), 0)
        cc = _iota((L, 128), 1)
        is_a = cc < L
        kx = jnp.where(is_a, cc, cc - (L + NM))
        is_memkey = (cc >= SEG) & (cc < SEG + 2 * NM)
        valid = cc < 2 * L
        allowed = valid & (is_memkey | (rr >= SEG) | (kx <= rr))
        fill = jnp.where(valid, -1000000000.0, -jnp.inf).astype(F32)
        lo64 = _iota((L, 128), 1) < 64

        def expand(y):
            y0, y1, y2 = y[:, 0:128], y[:, 128:256], y[:, 256:384]
            zero = jnp.zeros((L, 128), F32)
            y1a = jnp.where(lo64, y1, 0.0)
            y1b = jnp.where(lo64, 0.0, y1)
            top = jnp.concatenate([y0, y1a, zero], axis=1)
            bot = jnp.concatenate([zero, y1b, y2], axis=1)
            return jnp.concatenate([top, bot[SEG:L], bot[0:SEG]], axis=0).astype(BF16)

        def softmax2(s):
            s = jnp.concatenate([s, jnp.zeros((L, 128 - 2 * L), F32)], axis=1)
            s = jnp.where(allowed, s * scale, fill)
            ma = jnp.max(jnp.where(is_a, s, -jnp.inf), axis=1, keepdims=True)
            mb = jnp.max(jnp.where(is_a, -jnp.inf, s), axis=1, keepdims=True)
            e = jnp.exp(s - jnp.where(is_a, ma, mb))
            sa = jnp.sum(jnp.where(is_a, e, 0.0), axis=1, keepdims=True)
            sb = jnp.sum(jnp.where(is_a, 0.0, e), axis=1, keepdims=True)
            p = e * jnp.where(is_a, 1.0 / sa, 1.0 / sb)
            return p[:, 0:2 * L].astype(BF16)

        def step(h, even):
            def proj(j):
                w = jnp.concatenate([wb[9 * j + t] for t in range(9)], axis=1)
                y = _dot(h, w)
                if even:
                    sqkv[j] = y[SEG:SEG + 8]
                    y = jnp.concatenate([y[0:SEG], y[SEG + 8:SEG + 16]], axis=0)
                else:
                    y = jnp.concatenate([sqkv[j], y[8:SEG], y[0:8]], axis=0)
                q = y[:, 0:384].astype(BF16)
                return q, expand(y[:, 384:768]), expand(y[:, 768:1152])

            def fin(j, o):
                if even:
                    so[j] = o[24:SEG]
                    o = jnp.concatenate([o[0:24], o[SEG:L]], axis=0)
                else:
                    o = jnp.concatenate([o, so[j]], axis=0)
                return o.astype(BF16)

            qkv = [None] * NPAIR
            ps = [None] * NPAIR
            os_ = [None] * NPAIR
            qkv[0] = proj(0)
            for j in range(NPAIR + 1):
                if j + 1 < NPAIR:
                    qkv[j + 1] = proj(j + 1)
                if j < NPAIR:
                    ps[j] = softmax2(_dot_nt(qkv[j][0], qkv[j][1]))
                if j >= 1:
                    os_[j - 1] = fin(j - 1, _dot(ps[j - 1], qkv[j - 1][2]))
            return _dot(jnp.concatenate(os_, axis=1), bwo[...])

        memv[...] = mem0_ref[...].astype(F32)

        def body(i, carry):
            base = pl.multiple_of(i * 64, 64)
            xn = xn32[pl.ds(base, 64), :]
            h0 = jnp.concatenate([xn[0:40], memv[...]], axis=0).astype(BF16)
            o0 = step(h0, True)
            h1 = jnp.concatenate([o0[24:32], xn[40:64]], axis=0).astype(BF16)
            o1 = step(h1, False)
            memv[...] = o1[32:40]
            o = jnp.concatenate([o0[0:24], o1[40:48], o1[0:32]], axis=0)
            xnew = xres[pl.ds(base, 64), :] + o
            xres[pl.ds(base, 64), :] = xnew
            xnb[pl.ds(base, 64), :] = _ln(xnew).astype(BF16)
            xin[pl.ds(base, 64), :] = xnew.astype(BF16)
            return carry

        jax.lax.fori_loop(0, S // 64, body, 0)

    def transpose_weights():
        for m in range(3):
            cp_big[m].wait()

            def tr(j, carry, m=m):
                for t in range(3):
                    off = pl.multiple_of(j * 384 + t * 128, 128)
                    wb[9 * j + 3 * m + t] = wt[m, pl.ds(off, 128), :].T
                return carry

            jax.lax.fori_loop(0, NPAIR, tr, 0)
        cp_big[3].wait()

    def layer(l, carry):
        layer_a()

        @pl.when(l == 0)
        def _():
            transpose_weights()

        layer_b(l)
        return carry

    jax.lax.fori_loop(0, 2, layer, 0)

    cp_out = pltpu.make_async_copy(xin, out_hbm, sems.at[0])
    cp_out.start()
    cp_out.wait()


@functools.partial(jax.jit, static_argnames=("B_seg_len",))
def pallas_interleave_layers__linear_kernel_hedgehog__memory_aug_recurrent_mem_tr__prompt_kernel(
    A_x: jax.Array,
    A_wqkv: jax.Array,
    A_w_phi: jax.Array,
    A_wo: jax.Array,
    B_x: jax.Array,
    B_mem0: jax.Array,
    B_Wq: jax.Array,
    B_Wk: jax.Array,
    B_Wv: jax.Array,
    B_Wo: jax.Array,
    B_seg_len=SEG,
):
    assert B_seg_len == SEG and A_x.shape == (1, S, D)
    tr = lambda w: jnp.transpose(w, (1, 2, 0)).reshape(HB * DB, D)
    any_spec = pl.BlockSpec(memory_space=pl.ANY)
    vmem_spec = pl.BlockSpec(memory_space=pltpu.VMEM)
    out = pl.pallas_call(
        _kernel,
        out_shape=jax.ShapeDtypeStruct((S, D), BF16),
        in_specs=[any_spec, any_spec, vmem_spec, any_spec, vmem_spec,
                  any_spec, any_spec, any_spec, any_spec],
        out_specs=any_spec,
        scratch_shapes=[
            pltpu.VMEM((S, D), BF16),
            pltpu.VMEM((D, 3 * D), BF16),
            pltpu.VMEM((D, D), BF16),
            pltpu.VMEM((3, HB * DB, D), BF16),
            pltpu.VMEM((9 * NPAIR, D, 128), BF16),
            pltpu.VMEM((HB * DB, D), BF16),
            pltpu.VMEM((S, D), F32),
            pltpu.VMEM((S, D), F32),
            pltpu.VMEM((S, D), BF16),
            pltpu.VMEM((D, D), BF16),
            pltpu.VMEM((D, D), BF16),
            pltpu.VMEM((4, 2 * DA * 8, 256), F32),
            pltpu.VMEM((2 * DA, HA, 128), F32),
            pltpu.VMEM((8, 2 * D), F32),
            pltpu.VMEM((2 * DA, HA, D), F32),
            pltpu.VMEM((2 * DA * HA, D), BF16),
            pltpu.VMEM((NM, D), F32),
            pltpu.VMEM((NPAIR, 8, 9 * 128), F32),
            pltpu.VMEM((NPAIR, 8, 3 * 128), F32),
            pltpu.SemaphoreType.DMA((7,)),
        ],
        compiler_params=pltpu.CompilerParams(vmem_limit_bytes=120 * 1024 * 1024),
    )(A_x.reshape(S, D), A_wqkv, jnp.transpose(A_w_phi, (1, 2, 0)), A_wo,
      B_mem0.reshape(NM, D), tr(B_Wq), tr(B_Wk), tr(B_Wv), B_Wo.reshape(HB * DB, D))
    return out.reshape(1, S, D)
```

```python
import functools

import jax
import jax.numpy as jnp
import jax.experimental.pallas as pl
import jax.experimental.pallas.tpu as pltpu

F32 = jnp.float32
BF16 = jnp.bfloat16
U32 = jnp.uint32

S = 2048
D = 640
HA = 32
DA = 20
HB = 32
DB = 192
NM = 8
SEG = 32
NPAIR = HB // 2
TB = 512
LN_EPS = 1e-5

_NN = (((1,), (0,)), ((), ()))
_NT = (((1,), (1,)), ((), ()))


def _dot(a, b):
    return jax.lax.dot_general(a, b, _NN, preferred_element_type=F32)


def _dot_nt(a, b):
    return jax.lax.dot_general(a, b, _NT, preferred_element_type=F32)


def _ln(x):
    m = jnp.mean(x, axis=-1, keepdims=True)
    xc = x - m
    v = jnp.mean(xc * xc, axis=-1, keepdims=True)
    return xc * jax.lax.rsqrt(v + LN_EPS)


def _iota(shape, dim):
    return jax.lax.broadcasted_iota(jnp.int32, shape, dim)


def _div20(i):
    return (i * 3277) >> 16


def _kernel(x_hbm, wqkv_hbm, wphi_ref, wo_hbm, mem0_ref, wqt_hbm, wkt_hbm, wvt_hbm, bwo_hbm,
            out_hbm,
            xin, wqkv, woa, wt, wb, bwo, xres, xn32, xnb, wqp, wkpt, kvacc, zacc, zrow,
            kvwo32, kvwo, memv, sqkv, so, opend, sems):
    cp_x = pltpu.make_async_copy(x_hbm, xin, sems.at[0])
    cp_wqkv = pltpu.make_async_copy(wqkv_hbm, wqkv, sems.at[1])
    cp_wo = pltpu.make_async_copy(wo_hbm, woa, sems.at[2])
    cp_x.start()
    cp_wqkv.start()
    cp_wo.start()
    cp_big = [
        pltpu.make_async_copy(wqt_hbm, wt.at[0], sems.at[3]),
        pltpu.make_async_copy(wkt_hbm, wt.at[1], sems.at[4]),
        pltpu.make_async_copy(wvt_hbm, wt.at[2], sems.at[5]),
        pltpu.make_async_copy(bwo_hbm, wt.at[3], sems.at[6]),
    ]

    wphi = wphi_ref[...].astype(F32)
    wd = jnp.concatenate([wphi[:, f, :] for f in range(DA)], axis=1)
    wd = jnp.concatenate([wd, jnp.zeros((128 - DA, D), F32)], axis=0).astype(BF16)
    r = _iota((D, 128), 0)
    c = _iota((D, 128), 1)
    sel = jnp.where(r - _div20(r) * DA == c, 1.0, 0.0).astype(BF16)
    r = _iota((D, D), 0)
    c = _iota((D, D), 1)
    phi = jnp.where(_div20(r) == (c & (HA - 1)), _dot(sel, wd), 0.0).astype(BF16)

    cp_x.wait()
    cp_wqkv.wait()
    cp_wo.wait()
    for cp in cp_big:
        cp.start()

    wqp[...] = _dot(wqkv[:, 0:D], phi).astype(BF16)
    wkpt[...] = _dot(wqkv[:, D:2 * D], phi).T.astype(BF16)

    def init_blk(i, carry):
        rows = pl.ds(pl.multiple_of(i * 256, 256), 256)
        x = xin[rows, :].astype(F32)
        xres[rows, :] = x
        xnb[rows, :] = _ln(x).astype(BF16)
        return carry

    jax.lax.fori_loop(0, S // 256, init_blk, 0)

    def layer_a():
        kvacc[...] = jnp.zeros_like(kvacc)
        zacc[...] = jnp.zeros_like(zacc)

        def phase1(i, carry):
            rows = pl.ds(pl.multiple_of(i * TB, TB), TB)
            xn = xnb[rows, :]
            pkt = _dot_nt(wkpt[...], xn).reshape(DA, HA, TB)
            v = _dot(xn, wqkv[:, 2 * D:3 * D]).astype(BF16)
            for g in range(4):
                pk = pkt[:, 8 * g:8 * g + 8, :]
                mx = jnp.max(pk, axis=0, keepdims=True)
                mn = jnp.min(pk, axis=0, keepdims=True)
                ep = jnp.exp(pk - mx)
                en = jnp.exp(mn - pk)
                ep = ep * (1.0 / jnp.sum(ep, axis=0, keepdims=True))
                en = en * (1.0 / jnp.sum(en, axis=0, keepdims=True))
                ph = jnp.concatenate([ep, en], axis=0)
                zp = ph[:, :, 0:128]
                for t in range(1, TB // 128):
                    zp = zp + ph[:, :, t * 128:(t + 1) * 128]
                zacc[:, 8 * g:8 * g + 8, :] += zp
                lhs = ph.reshape(2 * DA * 8, TB).astype(BF16)
                kvacc[g] += _dot(lhs, v[:, 128 * g:128 * g + 256])
            return carry

        jax.lax.fori_loop(0, S // TB, phase1, 0)

        zt = zacc[...].reshape(2 * DA * HA, 128).T
        zrow[...] = jnp.broadcast_to(jnp.sum(zt, axis=0, keepdims=True), zrow.shape)
        rr = _iota((2 * DA * 8, 256), 0) & 7
        cc = _iota((2 * DA * 8, 256), 1)
        for g in range(4):
            keep = _div20(cc + 128 * g) == rr + 8 * g
            kvm = jnp.where(keep, kvacc[g], 0.0).astype(BF16)
            tg = _dot(kvm, woa[128 * g:128 * g + 256, :])
            kvwo32[:, 8 * g:8 * g + 8, :] = tg.reshape(2 * DA, 8, D)
        kvwo[...] = kvwo32[...].reshape(2 * DA * HA, D).astype(BF16)

        def lane_all(x, op):
            x = op(x, pltpu.roll(x, 32, 1))
            return op(x, pltpu.roll(x, 64, 1))

        def phase2(i, carry):
            rows = pl.ds(pl.multiple_of(i * TB, TB), TB)
            pq = _dot(xnb[rows, :], wqp[...])
            ts = [pq[:, 128 * t:128 * (t + 1)] for t in range(5)]
            mx = lane_all(functools.reduce(jnp.maximum, ts), jnp.maximum)
            mn = lane_all(functools.reduce(jnp.minimum, ts), jnp.minimum)
            ep = [jnp.exp(t - mx) for t in ts]
            en = [jnp.exp(mn - t) for t in ts]
            z = zrow[0:1, :]
            rp = 1.0 / lane_all(functools.reduce(jnp.add, ep), jnp.add)
            rn = 1.0 / lane_all(functools.reduce(jnp.add, en), jnp.add)
            tp = functools.reduce(
                jnp.add, [ep[t] * z[:, 128 * t:128 * (t + 1)] for t in range(5)])
            tn = functools.reduce(
                jnp.add, [en[t] * z[:, D + 128 * t:D + 128 * (t + 1)] for t in range(5)])
            rden = 1.0 / (lane_all(tp * rp + tn * rn, jnp.add) + 1e-6)
            cp_ = rp * rden
            cn_ = rn * rden
            lhs = jnp.concatenate(
                [(e * cp_).astype(BF16) for e in ep] + [(e * cn_).astype(BF16) for e in en],
                axis=1)
            xnew = xres[rows, :] + _dot(lhs, kvwo[...])
            xres[rows, :] = xnew
            xn32[rows, :] = _ln(xnew)
            return carry

        jax.lax.fori_loop(0, S // TB, phase2, 0)

    scale = DB ** (-0.5)

    def layer_b(layer):
        L = SEG + NM
        rr = _iota((L, 128), 0)
        cc = _iota((L, 128), 1)
        is_a = cc < L
        kx = jnp.where(is_a, cc, cc - (L + NM))
        is_memkey = (cc >= SEG) & (cc < SEG + 2 * NM)
        valid = cc < 2 * L
        allowed = valid & (is_memkey | (rr >= SEG) | (kx <= rr))
        fill = jnp.where(valid, -1000000000.0, -jnp.inf).astype(F32)
        lo64 = _iota((L, 128), 1) < 64

        def stack_keys(a, b):
            return jnp.concatenate([a, b[SEG:L], b[0:SEG]], axis=0).astype(BF16)

        def stack_rows(a, b):
            return jnp.concatenate([a[0:SEG], b[0:SEG], a[SEG:L], b[SEG:L]], axis=0).astype(BF16)

        def unstack_rows(r):
            a = jnp.concatenate([r[0:SEG], r[2 * SEG:2 * SEG + NM]], axis=0)
            b = jnp.concatenate([r[SEG:2 * SEG], r[2 * SEG + NM:2 * L]], axis=0)
            return a, b

        def expand(y):
            y0, y1, y2 = y[:, 0:128], y[:, 128:256], y[:, 256:384]
            return (stack_keys(y0, y2),
                    stack_keys(jnp.where(lo64, y1, 0.0), jnp.where(lo64, 0.0, y1)))

        def pad_lanes(s):
            return jnp.concatenate([s, jnp.zeros((s.shape[0], 128 - 2 * L), F32)], axis=1)

        def scores(q, k):
            sa, sb = unstack_rows(pad_lanes(_dot_nt(q[0], k[0])))
            s = jnp.where(is_a, sa, sb) + pad_lanes(_dot_nt(q[1], k[1]))
            s = jnp.where(allowed, s * scale, fill)
            ma = jnp.max(jnp.where(is_a, s, -jnp.inf), axis=1, keepdims=True)
            mb = jnp.max(jnp.where(is_a, -jnp.inf, s), axis=1, keepdims=True)
            e = jnp.exp(s - jnp.where(is_a, ma, mb))
            ea = jnp.where(is_a, e, 0.0)
            eb = jnp.where(is_a, 0.0, e)
            pa = ea * (1.0 / jnp.sum(ea, axis=1, keepdims=True))
            pb = eb * (1.0 / jnp.sum(eb, axis=1, keepdims=True))
            return stack_rows(pa, pb)[:, 0:2 * L], (pa + pb)[:, 0:2 * L].astype(BF16)

        def pv(p, v):
            o0, o2 = unstack_rows(_dot(p[0], v[0]))
            return jnp.concatenate([o0, _dot(p[1], v[1]), o2], axis=1)

        def step(h, even):
            def proj(j):
                w = jnp.concatenate(
                    [pltpu.bitcast(wb[9 * j + t], BF16) for t in range(9)], axis=1)
                if j == 0 and not even:
                    y = _dot(h[:, 0:128], w[0:128])
                    for t in range(1, 5):
                        y = _dot(h[:, 128 * t:128 * (t + 1)], w[128 * t:128 * (t + 1)]) + y
                else:
                    y = _dot(h, w)
                if even:
                    sqkv[j] = y[SEG:SEG + 8]
                    y = jnp.concatenate([y[0:SEG], y[SEG + 8:SEG + 16]], axis=0)
                else:
                    y = jnp.concatenate([sqkv[j], y], axis=0)
                q = (stack_rows(y[:, 0:128], y[:, 256:384]), y[:, 128:256].astype(BF16))
                return q, expand(y[:, 384:768]), expand(y[:, 768:1152])

            def fin(j, o):
                if even:
                    so[j] = o[24:SEG]
                    o = jnp.concatenate([o[0:24], o[SEG:L]], axis=0)
                else:
                    o = jnp.concatenate([o, so[j]], axis=0)
                return o.astype(BF16)

            qkv = [None] * NPAIR
            ps = [None] * NPAIR
            os_ = [None] * NPAIR

            def wo_chunk(c0, c1):
                w = pltpu.bitcast(bwo[192 * c0:192 * c1, :], BF16)
                return _dot(jnp.concatenate(os_[c0:c1], axis=1), w)

            fill_chunks = {NPAIR - 1: (0, 4), NPAIR: (4, 8), NPAIR + 1: (8, 11)}
            qkv[0] = proj(0)
            acc = None
            for j in range(NPAIR + 2):
                if j + 1 < NPAIR:
                    qkv[j + 1] = proj(j + 1)
                else:
                    c = wo_chunk(*fill_chunks[j])
                    acc = c if acc is None else c + acc
                if j < NPAIR:
                    ps[j] = scores(qkv[j][0], qkv[j][1])
                if j >= 2:
                    os_[j - 2] = fin(j - 2, pv(ps[j - 2], qkv[j - 2][2]))
            acc = wo_chunk(11, 14) + acc
            return wo_chunk(14, 16) + acc

        def finish_rows(base):
            xnew = xres[pl.ds(base, 64), :] + opend[...]
            xres[pl.ds(base, 64), :] = xnew
            xnb[pl.ds(base, 64), :] = _ln(xnew).astype(BF16)
            xin[pl.ds(base, 64), :] = xnew.astype(BF16)

        memv[...] = mem0_ref[...].astype(F32)
        opend[...] = jnp.zeros_like(opend)

        def body(i, carry):
            base = pl.multiple_of(i * 64, 64)
            xn = xn32[pl.ds(base, 64), :]
            h0 = jnp.concatenate([xn[0:40], memv[...]], axis=0).astype(BF16)
            finish_rows(pl.multiple_of(jnp.maximum(i - 1, 0) * 64, 64))
            o0 = step(h0, True)
            opend[0:24, :] = o0[0:24]
            h1 = jnp.concatenate([xn[40:64], o0[24:32]], axis=0).astype(BF16)
            o1 = step(h1, False)
            memv[...] = o1[32:40]
            opend[24:32, :] = o1[40:48]
            opend[32:64, :] = o1[0:32]
            return carry

        jax.lax.fori_loop(0, S // 64, body, 0)
        finish_rows(S - 64)

    def transpose_weights():
        for m in range(3):
            cp_big[m].wait()

            def tr(j, carry, m=m):
                for t in range(3):
                    off = pl.multiple_of(j * 384 + t * 128, 128)
                    wb[9 * j + 3 * m + t] = pltpu.bitcast(wt[m, pl.ds(off, 128), :].T, U32)
                return carry

            jax.lax.fori_loop(0, NPAIR, tr, 0)
        cp_big[3].wait()

        def cpo(j, carry):
            bwo[pl.ds(pl.multiple_of(j * 192, 192), 192), :] = pltpu.bitcast(
                wt[3, pl.ds(pl.multiple_of(j * 384, 384), 384), :], U32)
            return carry

        jax.lax.fori_loop(0, NPAIR, cpo, 0)

    def layer(l, carry):
        layer_a()

        @pl.when(l == 0)
        def _():
            transpose_weights()

        layer_b(l)
        return carry

    jax.lax.fori_loop(0, 2, layer, 0)

    cp_out = pltpu.make_async_copy(xin, out_hbm, sems.at[0])
    cp_out.start()
    cp_out.wait()


@functools.partial(jax.jit, static_argnames=("B_seg_len",))
def pallas_interleave_layers__linear_kernel_hedgehog__memory_aug_recurrent_mem_tr__prompt_kernel(
    A_x: jax.Array,
    A_wqkv: jax.Array,
    A_w_phi: jax.Array,
    A_wo: jax.Array,
    B_x: jax.Array,
    B_mem0: jax.Array,
    B_Wq: jax.Array,
    B_Wk: jax.Array,
    B_Wv: jax.Array,
    B_Wo: jax.Array,
    B_seg_len=SEG,
):
    assert B_seg_len == SEG and A_x.shape == (1, S, D)
    tr = lambda w: jnp.transpose(w, (1, 2, 0)).reshape(HB * DB, D)
    any_spec = pl.BlockSpec(memory_space=pl.ANY)
    vmem_spec = pl.BlockSpec(memory_space=pltpu.VMEM)
    out = pl.pallas_call(
        _kernel,
        out_shape=jax.ShapeDtypeStruct((S, D), BF16),
        in_specs=[any_spec, any_spec, vmem_spec, any_spec, vmem_spec,
                  any_spec, any_spec, any_spec, any_spec],
        out_specs=any_spec,
        scratch_shapes=[
            pltpu.VMEM((S, D), BF16),
            pltpu.VMEM((D, 3 * D), BF16),
            pltpu.VMEM((D, D), BF16),
            pltpu.VMEM((4, HB * DB, D), BF16),
            pltpu.VMEM((9 * NPAIR, D // 2, 128), U32),
            pltpu.VMEM((HB * DB // 2, D), U32),
            pltpu.VMEM((S, D), F32),
            pltpu.VMEM((S, D), F32),
            pltpu.VMEM((S, D), BF16),
            pltpu.VMEM((D, D), BF16),
            pltpu.VMEM((D, D), BF16),
            pltpu.VMEM((4, 2 * DA * 8, 256), F32),
            pltpu.VMEM((2 * DA, HA, 128), F32),
            pltpu.VMEM((8, 2 * D), F32),
            pltpu.VMEM((2 * DA, HA, D), F32),
            pltpu.VMEM((2 * DA * HA, D), BF16),
            pltpu.VMEM((NM, D), F32),
            pltpu.VMEM((NPAIR, 8, 9 * 128), F32),
            pltpu.VMEM((NPAIR, 8, 3 * 128), F32),
            pltpu.VMEM((64, D), F32),
            pltpu.SemaphoreType.DMA((7,)),
        ],
        compiler_params=pltpu.CompilerParams(vmem_limit_bytes=120 * 1024 * 1024),
    )(A_x.reshape(S, D), A_wqkv, jnp.transpose(A_w_phi, (1, 2, 0)), A_wo,
      B_mem0.reshape(NM, D), tr(B_Wq), tr(B_Wk), tr(B_Wv), B_Wo.reshape(HB * DB, D))
    return out.reshape(1, S, D)
```

```python
import functools

import jax
import jax.numpy as jnp
import jax.experimental.pallas as pl
import jax.experimental.pallas.tpu as pltpu

F32 = jnp.float32
BF16 = jnp.bfloat16
U32 = jnp.uint32

S = 2048
D = 640
HA = 32
DA = 20
HB = 32
DB = 192
NM = 8
SEG = 32
NPAIR = HB // 2
TB = 512
TC = 256
LN_EPS = 1e-5

_NN = (((1,), (0,)), ((), ()))
_NT = (((1,), (1,)), ((), ()))


def _dot(a, b):
    return jax.lax.dot_general(a, b, _NN, preferred_element_type=F32)


def _dot_nt(a, b):
    return jax.lax.dot_general(a, b, _NT, preferred_element_type=F32)


def _ln(x):
    m = jnp.mean(x, axis=-1, keepdims=True)
    xc = x - m
    v = jnp.mean(xc * xc, axis=-1, keepdims=True)
    return xc * jax.lax.rsqrt(v + LN_EPS)


def _iota(shape, dim):
    return jax.lax.broadcasted_iota(jnp.int32, shape, dim)


def _div20(i):
    return (i * 3277) >> 16


def _div40(i):
    return _div20(i) >> 1


def _kernel(x_hbm, wqkv_hbm, wphi_ref, wo_hbm, mem0_ref, wqt_hbm, wkt_hbm, wvt_hbm, bwo_hbm,
            out_hbm,
            xin, wqkv, woa, wt, wb, bwo, xres, xn32, xnb, wat, kvacc, phiq,
            memv, sqkv, so, opend, sems):
    cp_x = pltpu.make_async_copy(x_hbm, xin, sems.at[0])
    cp_wqkv = pltpu.make_async_copy(wqkv_hbm, wqkv, sems.at[1])
    cp_wo = pltpu.make_async_copy(wo_hbm, woa, sems.at[2])
    cp_wqkv.start()
    cp_x.start()
    cp_wo.start()
    cp_big = [
        pltpu.make_async_copy(wqt_hbm, wt.at[0], sems.at[3]),
        pltpu.make_async_copy(wkt_hbm, wt.at[1], sems.at[4]),
        pltpu.make_async_copy(wvt_hbm, wt.at[2], sems.at[5]),
        pltpu.make_async_copy(bwo_hbm, wt.at[3], sems.at[6]),
    ]

    wphi = wphi_ref[...].astype(F32)
    xw = jnp.concatenate([wphi[d] for d in range(DA)], axis=1)
    xw = jnp.concatenate([xw, jnp.zeros((32 - DA, D), F32)], axis=0).astype(BF16)
    r = _iota((D, D), 0)
    c = _iota((D, D), 1)
    perm = jnp.where((r & 31) * DA + (r >> 5) == c, 1.0, 0.0).astype(BF16)
    wf = _dot(xw, perm).astype(BF16)
    r = _iota((160, 32), 0)
    c = _iota((160, 32), 1)
    rsel = jnp.where(((r - _div40(r) * 40) >> 1) == c, 1.0, 0.0).astype(BF16)
    r = _iota((160, 128), 0)
    c = _iota((160, 128), 1)
    phit = []
    for t in range(5):
        keep = 2 * (_div40(r) + 3 * t) + (r & 1) == _div20(c + 128 * t)
        phit.append(jnp.where(keep, _dot(rsel, wf[:, 128 * t:128 * (t + 1)]), 0.0).astype(BF16))

    cp_wqkv.wait()
    cp_x.wait()
    cp_wo.wait()
    for cp in cp_big:
        cp.start()

    for m, dst in ((1, 0), (0, 1)):
        p = [_dot_nt(phit[t], wqkv[:, m * D + 128 * t:m * D + 128 * (t + 1)]) for t in range(5)]
        rows = [p[0][0:120]]
        for t in range(1, 5):
            rows += [p[t - 1][120:160] + p[t][0:40], p[t][40:120]]
        rows.append(p[4][120:160])
        wat[dst] = pltpu.bitcast(jnp.concatenate(rows, axis=0).astype(BF16), U32)
    wat[2] = pltpu.bitcast(wqkv[:, 2 * D:3 * D].T, U32)

    def init_blk(i, carry):
        rows = pl.ds(pl.multiple_of(i * 256, 256), 256)
        x = xin[rows, :].astype(F32)
        xres[rows, :] = x
        xnb[rows, :] = _ln(x).astype(BF16)
        return carry

    jax.lax.fori_loop(0, S // 256, init_blk, 0)

    def layer_a():
        kvacc[...] = jnp.zeros_like(kvacc)

        def sub_all(x, op):
            x = op(x, pltpu.roll(x, 2, 0))
            return op(x, pltpu.roll(x, 4, 0))

        def phi(p):
            ts = [p[8 * t:8 * (t + 1)] for t in range(5)]
            mx = sub_all(functools.reduce(jnp.maximum, ts), jnp.maximum)
            mn = sub_all(functools.reduce(jnp.minimum, ts), jnp.minimum)
            ep = [jnp.exp(t - mx) for t in ts]
            en = [jnp.exp(mn - t) for t in ts]
            rp = 1.0 / sub_all(functools.reduce(jnp.add, ep), jnp.add)
            rn = 1.0 / sub_all(functools.reduce(jnp.add, en), jnp.add)
            return jnp.concatenate([e * rp for e in ep] + [e * rn for e in en], axis=0).astype(BF16)

        def phase1(i, carry):
            off = pl.multiple_of(i * TB, TB)
            xn = xnb[pl.ds(off, TB), :]
            pk = _dot_nt(pltpu.bitcast(wat[0], BF16), xn)
            phik = [phi(pk[40 * j:40 * (j + 1)]) for j in range(16)]
            pq = _dot_nt(pltpu.bitcast(wat[1], BF16), xn)
            for j in range(16):
                phiq[j, :, pl.ds(off, TB)] = pltpu.bitcast(phi(pq[40 * j:40 * (j + 1)]), U32)
            hb = TB // 2
            vt = [_dot_nt(pltpu.bitcast(wat[2], BF16), xn[hb * u:hb * (u + 1)]) for u in range(2)]
            ones = jnp.ones((8, hb), F32)
            for u in range(2):
                for j in range(16):
                    lhs = jnp.concatenate([vt[u][40 * j:40 * (j + 1)], ones], axis=0).astype(BF16)
                    kvacc[j] = _dot_nt(lhs, phik[j][:, hb * u:hb * (u + 1)]) + kvacc[j]
            return carry

        jax.lax.fori_loop(0, S // TB, phase1, 0)

        rr = _iota((48, 80), 0)
        cc = _iota((48, 80), 1)
        keep = jnp.where(rr < 40, _div20(rr), (rr - 40) >> 2) == (cc & 1)
        kvm = [jnp.where(keep, kvacc[j], 0.0).astype(BF16) for j in range(16)]
        lo4 = _iota((8, TC), 0) < 4

        def num(b):
            parts = []
            for j in range(16):
                r = _dot(kvm[j], pltpu.bitcast(phiq[j, :, TC * b:TC * (b + 1)], BF16))
                rc = 1.0 / (r[40:48] + 1e-6)
                rc2 = pltpu.roll(rc, 4, 0)
                ra = jnp.where(lo4, rc, rc2)
                rb = jnp.where(lo4, rc2, rc)
                parts += [r[0:8] * ra, r[8:16] * ra, r[16:24] * rc, r[24:32] * rb, r[32:40] * rb]
            return jnp.concatenate(parts, axis=0).astype(BF16).T

        def out(b, o):
            rows = slice(TC * b, TC * (b + 1))
            xnew = xres[rows, :] + _dot(o, woa[...])
            xres[rows, :] = xnew
            xn32[rows, :] = _ln(xnew)

        nb = S // TC
        os_ = [None] * nb
        os_[0] = num(0)
        os_[1] = num(1)
        for b in range(nb):
            if b + 2 < nb:
                os_[b + 2] = num(b + 2)
            out(b, os_[b])

    scale = DB ** (-0.5)

    def layer_b(layer):
        L = SEG + NM
        rr = _iota((L, 128), 0)
        cc = _iota((L, 128), 1)
        is_a = cc < L
        kx = jnp.where(is_a, cc, cc - (L + NM))
        is_memkey = (cc >= SEG) & (cc < SEG + 2 * NM)
        valid = cc < 2 * L
        allowed = valid & (is_memkey | (rr >= SEG) | (kx <= rr))
        fill = jnp.where(valid, -1000000000.0, -jnp.inf).astype(F32)
        lo64 = _iota((L, 128), 1) < 64

        def stack_keys(a, b):
            return jnp.concatenate([a, b[SEG:L], b[0:SEG]], axis=0).astype(BF16)

        def stack_rows(a, b):
            return jnp.concatenate([a[0:SEG], b[0:SEG], a[SEG:L], b[SEG:L]], axis=0).astype(BF16)

        def unstack_rows(r):
            a = jnp.concatenate([r[0:SEG], r[2 * SEG:2 * SEG + NM]], axis=0)
            b = jnp.concatenate([r[SEG:2 * SEG], r[2 * SEG + NM:2 * L]], axis=0)
            return a, b

        def expand(y):
            y0, y1, y2 = y[:, 0:128], y[:, 128:256], y[:, 256:384]
            return (stack_keys(y0, y2),
                    stack_keys(jnp.where(lo64, y1, 0.0), jnp.where(lo64, 0.0, y1)))

        def pad_lanes(s):
            return jnp.concatenate([s, jnp.zeros((s.shape[0], 128 - 2 * L), F32)], axis=1)

        def scores(q, k):
            sa, sb = unstack_rows(pad_lanes(_dot_nt(q[0], k[0])))
            s = jnp.where(is_a, sa, sb) + pad_lanes(_dot_nt(q[1], k[1]))
            s = jnp.where(allowed, s * scale, fill)
            ma = jnp.max(jnp.where(is_a, s, -jnp.inf), axis=1, keepdims=True)
            mb = jnp.max(jnp.where(is_a, -jnp.inf, s), axis=1, keepdims=True)
            e = jnp.exp(s - jnp.where(is_a, ma, mb))
            ea = jnp.where(is_a, e, 0.0)
            eb = jnp.where(is_a, 0.0, e)
            pa = ea * (1.0 / jnp.sum(ea, axis=1, keepdims=True))
            pb = eb * (1.0 / jnp.sum(eb, axis=1, keepdims=True))
            return stack_rows(pa, pb)[:, 0:2 * L], (pa + pb)[:, 0:2 * L].astype(BF16)

        def pv(p, v):
            o0, o2 = unstack_rows(_dot(p[0], v[0]))
            return jnp.concatenate([o0, _dot(p[1], v[1]), o2], axis=1)

        def step(h, even):
            def proj(j):
                w = jnp.concatenate(
                    [pltpu.bitcast(wb[9 * j + t], BF16) for t in range(9)], axis=1)
                if j == 0 and not even:
                    y = _dot(h[:, 0:128], w[0:128])
                    for t in range(1, 5):
                        y = _dot(h[:, 128 * t:128 * (t + 1)], w[128 * t:128 * (t + 1)]) + y
                else:
                    y = _dot(h, w)
                if even:
                    sqkv[j] = y[SEG:SEG + 8]
                    y = jnp.concatenate([y[0:SEG], y[SEG + 8:SEG + 16]], axis=0)
                else:
                    y = jnp.concatenate([sqkv[j], y], axis=0)
                q = (stack_rows(y[:, 0:128], y[:, 256:384]), y[:, 128:256].astype(BF16))
                return q, expand(y[:, 384:768]), expand(y[:, 768:1152])

            def fin(j, o):
                if even:
                    so[j] = o[24:SEG]
                    o = jnp.concatenate([o[0:24], o[SEG:L]], axis=0)
                else:
                    o = jnp.concatenate([o, so[j]], axis=0)
                return o.astype(BF16)

            qkv = [None] * NPAIR
            ps = [None] * NPAIR
            os_ = [None] * NPAIR

            def wo_chunk(c0, c1):
                w = pltpu.bitcast(bwo[192 * c0:192 * c1, :], BF16)
                return _dot(jnp.concatenate(os_[c0:c1], axis=1), w)

            fill_chunks = {NPAIR - 1: (0, 4), NPAIR: (4, 8), NPAIR + 1: (8, 11)}
            qkv[0] = proj(0)
            acc = None
            for j in range(NPAIR + 2):
                if j + 1 < NPAIR:
                    qkv[j + 1] = proj(j + 1)
                else:
                    c = wo_chunk(*fill_chunks[j])
                    acc = c if acc is None else c + acc
                if j < NPAIR:
                    ps[j] = scores(qkv[j][0], qkv[j][1])
                if j >= 2:
                    os_[j - 2] = fin(j - 2, pv(ps[j - 2], qkv[j - 2][2]))
            acc = wo_chunk(11, 14) + acc
            return wo_chunk(14, 16) + acc

        def finish_rows(base):
            xnew = xres[pl.ds(base, 64), :] + opend[...]
            xres[pl.ds(base, 64), :] = xnew
            xnb[pl.ds(base, 64), :] = _ln(xnew).astype(BF16)
            xin[pl.ds(base, 64), :] = xnew.astype(BF16)

        memv[...] = mem0_ref[...].astype(F32)
        opend[...] = jnp.zeros_like(opend)

        def body(i, carry):
            base = pl.multiple_of(i * 64, 64)
            xn = xn32[pl.ds(base, 64), :]
            h0 = jnp.concatenate([xn[0:40], memv[...]], axis=0).astype(BF16)
            finish_rows(pl.multiple_of(jnp.maximum(i - 1, 0) * 64, 64))
            o0 = step(h0, True)
            opend[0:24, :] = o0[0:24]
            h1 = jnp.concatenate([xn[40:64], o0[24:32]], axis=0).astype(BF16)
            o1 = step(h1, False)
            memv[...] = o1[32:40]
            opend[24:32, :] = o1[40:48]
            opend[32:64, :] = o1[0:32]
            return carry

        jax.lax.fori_loop(0, S // 64, body, 0)
        finish_rows(S - 64)

    def transpose_weights():
        for m in range(3):
            cp_big[m].wait()

            def tr(j, carry, m=m):
                for t in range(3):
                    off = pl.multiple_of(j * 384 + t * 128, 128)
                    wb[9 * j + 3 * m + t] = pltpu.bitcast(wt[m, pl.ds(off, 128), :].T, U32)
                return carry

            jax.lax.fori_loop(0, NPAIR, tr, 0)
        cp_big[3].wait()

        def cpo(j, carry):
            bwo[pl.ds(pl.multiple_of(j * 192, 192), 192), :] = pltpu.bitcast(
                wt[3, pl.ds(pl.multiple_of(j * 384, 384), 384), :], U32)
            return carry

        jax.lax.fori_loop(0, NPAIR, cpo, 0)

    def layer(l, carry):
        layer_a()

        @pl.when(l == 0)
        def _():
            transpose_weights()

        layer_b(l)
        return carry

    jax.lax.fori_loop(0, 2, layer, 0)

    cp_out = pltpu.make_async_copy(xin, out_hbm, sems.at[0])
    cp_out.start()
    cp_out.wait()


@functools.partial(jax.jit, static_argnames=("B_seg_len",))
def pallas_interleave_layers__linear_kernel_hedgehog__memory_aug_recurrent_mem_tr__prompt_kernel(
    A_x: jax.Array,
    A_wqkv: jax.Array,
    A_w_phi: jax.Array,
    A_wo: jax.Array,
    B_x: jax.Array,
    B_mem0: jax.Array,
    B_Wq: jax.Array,
    B_Wk: jax.Array,
    B_Wv: jax.Array,
    B_Wo: jax.Array,
    B_seg_len=SEG,
):
    assert B_seg_len == SEG and A_x.shape == (1, S, D)
    tr = lambda w: jnp.transpose(w, (1, 2, 0)).reshape(HB * DB, D)
    any_spec = pl.BlockSpec(memory_space=pl.ANY)
    vmem_spec = pl.BlockSpec(memory_space=pltpu.VMEM)
    out = pl.pallas_call(
        _kernel,
        out_shape=jax.ShapeDtypeStruct((S, D), BF16),
        in_specs=[any_spec, any_spec, vmem_spec, any_spec, vmem_spec,
                  any_spec, any_spec, any_spec, any_spec],
        out_specs=any_spec,
        scratch_shapes=[
            pltpu.VMEM((S, D), BF16),
            pltpu.VMEM((D, 3 * D), BF16),
            pltpu.VMEM((D, D), BF16),
            pltpu.VMEM((4, HB * DB, D), BF16),
            pltpu.VMEM((9 * NPAIR, D // 2, 128), U32),
            pltpu.VMEM((HB * DB // 2, D), U32),
            pltpu.VMEM((S, D), F32),
            pltpu.VMEM((S, D), F32),
            pltpu.VMEM((S, D), BF16),
            pltpu.VMEM((3, D // 2, D), U32),
            pltpu.VMEM((16, 48, 80), F32),
            pltpu.VMEM((16, 40, S), U32),
            pltpu.VMEM((NM, D), F32),
            pltpu.VMEM((NPAIR, 8, 9 * 128), F32),
            pltpu.VMEM((NPAIR, 8, 3 * 128), F32),
            pltpu.VMEM((64, D), F32),
            pltpu.SemaphoreType.DMA((7,)),
        ],
        compiler_params=pltpu.CompilerParams(vmem_limit_bytes=120 * 1024 * 1024),
    )(A_x.reshape(S, D), A_wqkv, jnp.transpose(A_w_phi, (1, 2, 0)), A_wo,
      B_mem0.reshape(NM, D), tr(B_Wq), tr(B_Wk), tr(B_Wv), B_Wo.reshape(HB * DB, D))
    return out.reshape(1, S, D)
```

```python
import functools

import jax
import jax.numpy as jnp
import jax.experimental.pallas as pl
import jax.experimental.pallas.tpu as pltpu

F32 = jnp.float32
BF16 = jnp.bfloat16
U32 = jnp.uint32

S = 2048
D = 640
HA = 32
DA = 20
HB = 32
DB = 192
NM = 8
SEG = 32
NPAIR = HB // 2
TB = 512
TC = 256
UNROLL = 1
LN_EPS = 1e-5

_NN = (((1,), (0,)), ((), ()))
_NT = (((1,), (1,)), ((), ()))


def _dot(a, b):
    return jax.lax.dot_general(a, b, _NN, preferred_element_type=F32)


def _dot_nt(a, b):
    return jax.lax.dot_general(a, b, _NT, preferred_element_type=F32)


def _ln(x):
    m = jnp.mean(x, axis=-1, keepdims=True)
    xc = x - m
    v = jnp.mean(xc * xc, axis=-1, keepdims=True)
    return xc * jax.lax.rsqrt(v + LN_EPS)


def _iota(shape, dim):
    return jax.lax.broadcasted_iota(jnp.int32, shape, dim)


def _div20(i):
    return (i * 3277) >> 16


def _div40(i):
    return _div20(i) >> 1


def _kernel(x_hbm, wqkv_hbm, wphi_ref, wo_hbm, mem0_ref, wqt_hbm, wkt_hbm, wvt_hbm, bwo_hbm,
            out_hbm,
            xin, wqkv, woa, wt, wb, bwo, xres, xn32, xnb, wat, kvacc, phiq,
            memv, snext, sdef, opend, sems):
    cp_x = pltpu.make_async_copy(x_hbm, xin, sems.at[0])
    cp_wqkv = pltpu.make_async_copy(wqkv_hbm, wqkv, sems.at[1])
    cp_wo = pltpu.make_async_copy(wo_hbm, woa, sems.at[2])
    cp_wqkv.start()
    cp_x.start()
    cp_wo.start()
    cp_big = [
        pltpu.make_async_copy(wqt_hbm, wt.at[0], sems.at[3]),
        pltpu.make_async_copy(wkt_hbm, wt.at[1], sems.at[4]),
        pltpu.make_async_copy(wvt_hbm, wt.at[2], sems.at[5]),
        pltpu.make_async_copy(bwo_hbm, wt.at[3], sems.at[6]),
    ]

    wphi = wphi_ref[...].astype(F32)
    xw = jnp.concatenate([wphi[d] for d in range(DA)], axis=1)
    xw = jnp.concatenate([xw, jnp.zeros((32 - DA, D), F32)], axis=0).astype(BF16)
    r = _iota((D, D), 0)
    c = _iota((D, D), 1)
    perm = jnp.where((r & 31) * DA + (r >> 5) == c, 1.0, 0.0).astype(BF16)
    wf = _dot(xw, perm).astype(BF16)
    r = _iota((160, 32), 0)
    c = _iota((160, 32), 1)
    rsel = jnp.where(((r - _div40(r) * 40) >> 1) == c, 1.0, 0.0).astype(BF16)
    r = _iota((160, 128), 0)
    c = _iota((160, 128), 1)
    phit = []
    for t in range(5):
        keep = 2 * (_div40(r) + 3 * t) + (r & 1) == _div20(c + 128 * t)
        phit.append(jnp.where(keep, _dot(rsel, wf[:, 128 * t:128 * (t + 1)]), 0.0).astype(BF16))

    cp_wqkv.wait()
    cp_x.wait()
    cp_wo.wait()
    for cp in cp_big:
        cp.start()

    for m, dst in ((1, 0), (0, 1)):
        p = [_dot_nt(phit[t], wqkv[:, m * D + 128 * t:m * D + 128 * (t + 1)]) for t in range(5)]
        rows = [p[0][0:120]]
        for t in range(1, 5):
            rows += [p[t - 1][120:160] + p[t][0:40], p[t][40:120]]
        rows.append(p[4][120:160])
        wat[dst] = pltpu.bitcast(jnp.concatenate(rows, axis=0).astype(BF16), U32)
    wat[2] = pltpu.bitcast(wqkv[:, 2 * D:3 * D].T, U32)

    def init_blk(i, carry):
        rows = pl.ds(pl.multiple_of(i * 256, 256), 256)
        x = xin[rows, :].astype(F32)
        xres[rows, :] = x
        xnb[rows, :] = _ln(x).astype(BF16)
        return carry

    jax.lax.fori_loop(0, S // 256, init_blk, 0)

    def layer_a():
        kvacc[...] = jnp.zeros_like(kvacc)

        def sub_all(x, op):
            x = op(x, pltpu.roll(x, 2, 0))
            return op(x, pltpu.roll(x, 4, 0))

        def phi(p):
            ts = [p[8 * t:8 * (t + 1)] for t in range(5)]
            mx = sub_all(functools.reduce(jnp.maximum, ts), jnp.maximum)
            mn = sub_all(functools.reduce(jnp.minimum, ts), jnp.minimum)
            ep = [jnp.exp(t - mx) for t in ts]
            en = [jnp.exp(mn - t) for t in ts]
            rp = 1.0 / sub_all(functools.reduce(jnp.add, ep), jnp.add)
            rn = 1.0 / sub_all(functools.reduce(jnp.add, en), jnp.add)
            return jnp.concatenate([e * rp for e in ep] + [e * rn for e in en], axis=0).astype(BF16)

        def phase1(i, carry):
            off = pl.multiple_of(i * TB, TB)
            xn = xnb[pl.ds(off, TB), :]
            pk = _dot_nt(pltpu.bitcast(wat[0], BF16), xn)
            phik = [phi(pk[40 * j:40 * (j + 1)]) for j in range(16)]
            pq = _dot_nt(pltpu.bitcast(wat[1], BF16), xn)
            for j in range(16):
                phiq[j, :, pl.ds(off, TB)] = pltpu.bitcast(phi(pq[40 * j:40 * (j + 1)]), U32)
            hb = TB // 2
            vt = [_dot_nt(pltpu.bitcast(wat[2], BF16), xn[hb * u:hb * (u + 1)]) for u in range(2)]
            ones = jnp.ones((8, hb), F32)
            for u in range(2):
                for j in range(16):
                    lhs = jnp.concatenate([vt[u][40 * j:40 * (j + 1)], ones], axis=0).astype(BF16)
                    kvacc[j] = _dot_nt(lhs, phik[j][:, hb * u:hb * (u + 1)]) + kvacc[j]
            return carry

        jax.lax.fori_loop(0, S // TB, phase1, 0)

        rr = _iota((48, 80), 0)
        cc = _iota((48, 80), 1)
        keep = jnp.where(rr < 40, _div20(rr), (rr - 40) >> 2) == (cc & 1)
        kvm = [jnp.where(keep, kvacc[j], 0.0).astype(BF16) for j in range(16)]
        lo4 = _iota((8, TC), 0) < 4

        def num(b):
            parts = []
            for j in range(16):
                r = _dot(kvm[j], pltpu.bitcast(phiq[j, :, TC * b:TC * (b + 1)], BF16))
                rc = 1.0 / (r[40:48] + 1e-6)
                rc2 = pltpu.roll(rc, 4, 0)
                ra = jnp.where(lo4, rc, rc2)
                rb = jnp.where(lo4, rc2, rc)
                parts += [r[0:8] * ra, r[8:16] * ra, r[16:24] * rc, r[24:32] * rb, r[32:40] * rb]
            return jnp.concatenate(parts, axis=0).astype(BF16).T

        def out(b, o):
            rows = slice(TC * b, TC * (b + 1))
            xnew = xres[rows, :] + _dot(o, woa[...])
            xres[rows, :] = xnew
            xn32[rows, :] = _ln(xnew)

        nb = S // TC
        os_ = [None] * nb
        os_[0] = num(0)
        os_[1] = num(1)
        for b in range(nb):
            if b + 2 < nb:
                os_[b + 2] = num(b + 2)
            out(b, os_[b])

    scale = DB ** (-0.5)

    def layer_b(layer):
        L = SEG + NM
        NEG = -1000000000.0

        def masks(even):
            nrow = SEG if even else L + 8
            rr = _iota((nrow, 128), 0)
            cc = _iota((nrow, 128), 1)
            is_a = (cc < L) | ((cc >= 2 * L) & (cc < 2 * L + 16))
            kx = jnp.where(cc < L, cc, cc - (L + NM))
            is_memkey = (cc >= SEG) & (cc < SEG + 2 * NM)
            if even:
                valid = cc < 2 * L
                allowed = valid & (is_memkey | (rr >= 24) | (kx <= rr + 8))
            else:
                dk = (cc - 2 * L) & 15
                cur = (rr < L) & (cc < 2 * L)
                old = (rr >= L) & (cc >= 2 * L) & (cc < 2 * L + 32)
                valid = cur | old
                allowed = ((cur & (is_memkey | (rr >= SEG) | (kx <= rr)))
                           | (old & ((dk >= 8) | (dk <= rr - L))))
            return is_a, allowed, jnp.where(valid, NEG, -jnp.inf).astype(F32)

        all_masks = {True: masks(True), False: masks(False)}

        def lo64(y):
            return _iota(y.shape, 1) < 64

        def stack_keys(a, b):
            parts = [a[0:L], b[SEG:L], b[0:SEG]]
            if a.shape[0] > L:
                parts += [a[L:], b[L:]]
            return jnp.concatenate(parts, axis=0).astype(BF16)

        def expand(y):
            y0, y1, y2 = y[:, 0:128], y[:, 128:256], y[:, 256:384]
            return (stack_keys(y0, y2),
                    stack_keys(jnp.where(lo64(y1), y1, 0.0), jnp.where(lo64(y1), 0.0, y1)))

        def pad_lanes(s):
            return jnp.concatenate([s, jnp.zeros((s.shape[0], 128 - s.shape[1]), F32)], axis=1)

        def step(h, even, kmajor):
            is_a, allowed, fill = all_masks[even]
            nrow = SEG if even else L + 8
            nkey = 2 * L if even else 2 * L + 32

            def proj(j):
                w = jnp.concatenate(
                    [pltpu.bitcast(wb[9 * j + t], BF16) for t in range(9)], axis=1)
                if j == 0 and kmajor:
                    y = _dot(h[:, 0:128], w[0:128])
                    for t in range(1, 5):
                        y = _dot(h[:, 128 * t:128 * (t + 1)], w[128 * t:128 * (t + 1)]) + y
                else:
                    y = _dot(h, w)
                if even:
                    snext[j] = y[SEG:L]
                    sdef[j, 0:8, :] = y[0:8]
                    sdef[j, 8:16, 384:1152] = y[L:L + 8, 384:1152]
                    q = jnp.concatenate([y[8:SEG, 0:384], y[L:L + 8, 0:384]], axis=0)
                    kv = jnp.concatenate([y[0:SEG, 384:1152], y[L:L + 8, 384:1152]], axis=0)
                else:
                    q = jnp.concatenate(
                        [snext[j, :, 0:384], y[:, 0:384], sdef[j, 0:8, 0:384]], axis=0)
                    kv = jnp.concatenate(
                        [snext[j, :, 384:1152], y[:, 384:1152], sdef[j, :, 384:1152]], axis=0)
                q = q.astype(BF16)
                q = (jnp.concatenate([q[:, 0:128], q[:, 256:384]], axis=0), q[:, 128:256])
                return q, expand(kv[:, 0:384]), expand(kv[:, 384:768])

            def scores(q, k):
                s02 = pad_lanes(_dot_nt(q[0], k[0]))
                s = jnp.where(is_a, s02[0:nrow], s02[nrow:]) + pad_lanes(_dot_nt(q[1], k[1]))
                s = jnp.where(allowed, s * scale, fill)
                ma = jnp.max(jnp.where(is_a, s, -jnp.inf), axis=1, keepdims=True)
                mb = jnp.max(jnp.where(is_a, -jnp.inf, s), axis=1, keepdims=True)
                e = jnp.exp(s - jnp.where(is_a, ma, mb))
                ea = jnp.where(is_a, e, 0.0)
                eb = jnp.where(is_a, 0.0, e)
                pa = ea * (1.0 / jnp.sum(ea, axis=1, keepdims=True))
                pb = eb * (1.0 / jnp.sum(eb, axis=1, keepdims=True))
                return (jnp.concatenate([pa, pb], axis=0)[:, 0:nkey].astype(BF16),
                        (pa + pb)[:, 0:nkey].astype(BF16))

            def pv(p, v):
                o02 = _dot(p[0], v[0])
                return jnp.concatenate(
                    [o02[0:nrow], _dot(p[1], v[1]), o02[nrow:]], axis=1).astype(BF16)

            qkv = [None] * NPAIR
            ps = [None] * NPAIR
            os_ = [None] * NPAIR

            def wo_chunk(c0, c1):
                w = pltpu.bitcast(bwo[192 * c0:192 * c1, :], BF16)
                return _dot(jnp.concatenate(os_[c0:c1], axis=1), w)

            fill_chunks = {NPAIR - 1: (0, 4), NPAIR: (4, 8), NPAIR + 1: (8, 11)}
            qkv[0] = proj(0)
            acc = None
            for j in range(NPAIR + 2):
                if j + 1 < NPAIR:
                    qkv[j + 1] = proj(j + 1)
                else:
                    c = wo_chunk(*fill_chunks[j])
                    acc = c if acc is None else c + acc
                if j < NPAIR:
                    ps[j] = scores(qkv[j][0], qkv[j][1])
                if j >= 2:
                    os_[j - 2] = pv(ps[j - 2], qkv[j - 2][2])
            acc = wo_chunk(11, 14) + acc
            return wo_chunk(14, 16) + acc

        RB = 64 * UNROLL

        def finish_rows(base):
            xnew = xres[pl.ds(base, RB), :] + opend[...]
            xres[pl.ds(base, RB), :] = xnew
            xnb[pl.ds(base, RB), :] = _ln(xnew).astype(BF16)
            xin[pl.ds(base, RB), :] = xnew.astype(BF16)

        memv[...] = mem0_ref[...].astype(F32)
        opend[...] = jnp.zeros_like(opend)

        def body(i, carry):
            base = pl.multiple_of(i * RB, RB)
            finish_rows(pl.multiple_of(jnp.maximum(i - 1, 0) * RB, RB))
            mem = memv[...]
            for u in range(UNROLL):
                r0 = 64 * u
                h0 = jnp.concatenate([xn32[pl.ds(base + r0, 40), :], mem], axis=0).astype(BF16)
                o0 = step(h0, True, u > 0)
                opend[r0 + 8:r0 + 32, :] = o0[0:24]
                h1 = jnp.concatenate(
                    [xn32[pl.ds(base + r0 + 40, 24), :], o0[24:32]], axis=0).astype(BF16)
                o1 = step(h1, False, True)
                mem = o1[32:40]
                opend[r0:r0 + 8, :] = o1[40:48]
                opend[r0 + 32:r0 + 64, :] = o1[0:32]
            memv[...] = mem
            return carry

        jax.lax.fori_loop(0, S // RB, body, 0)
        finish_rows(S - RB)

    def transpose_weights():
        for m in range(3):
            cp_big[m].wait()

            def tr(j, carry, m=m):
                for t in range(3):
                    off = pl.multiple_of(j * 384 + t * 128, 128)
                    wb[9 * j + 3 * m + t] = pltpu.bitcast(wt[m, pl.ds(off, 128), :].T, U32)
                return carry

            jax.lax.fori_loop(0, NPAIR, tr, 0)
        cp_big[3].wait()

        def cpo(j, carry):
            bwo[pl.ds(pl.multiple_of(j * 192, 192), 192), :] = pltpu.bitcast(
                wt[3, pl.ds(pl.multiple_of(j * 384, 384), 384), :], U32)
            return carry

        jax.lax.fori_loop(0, NPAIR, cpo, 0)

    def layer(l, carry):
        layer_a()

        @pl.when(l == 0)
        def _():
            transpose_weights()

        layer_b(l)
        return carry

    jax.lax.fori_loop(0, 2, layer, 0)

    cp_out = pltpu.make_async_copy(xin, out_hbm, sems.at[0])
    cp_out.start()
    cp_out.wait()


@functools.partial(jax.jit, static_argnames=("B_seg_len",))
def pallas_interleave_layers__linear_kernel_hedgehog__memory_aug_recurrent_mem_tr__prompt_kernel(
    A_x: jax.Array,
    A_wqkv: jax.Array,
    A_w_phi: jax.Array,
    A_wo: jax.Array,
    B_x: jax.Array,
    B_mem0: jax.Array,
    B_Wq: jax.Array,
    B_Wk: jax.Array,
    B_Wv: jax.Array,
    B_Wo: jax.Array,
    B_seg_len=SEG,
):
    assert B_seg_len == SEG and A_x.shape == (1, S, D)
    tr = lambda w: jnp.transpose(w, (1, 2, 0)).reshape(HB * DB, D)
    any_spec = pl.BlockSpec(memory_space=pl.ANY)
    vmem_spec = pl.BlockSpec(memory_space=pltpu.VMEM)
    out = pl.pallas_call(
        _kernel,
        out_shape=jax.ShapeDtypeStruct((S, D), BF16),
        in_specs=[any_spec, any_spec, vmem_spec, any_spec, vmem_spec,
                  any_spec, any_spec, any_spec, any_spec],
        out_specs=any_spec,
        scratch_shapes=[
            pltpu.VMEM((S, D), BF16),
            pltpu.VMEM((D, 3 * D), BF16),
            pltpu.VMEM((D, D), BF16),
            pltpu.VMEM((4, HB * DB, D), BF16),
            pltpu.VMEM((9 * NPAIR, D // 2, 128), U32),
            pltpu.VMEM((HB * DB // 2, D), U32),
            pltpu.VMEM((S, D), F32),
            pltpu.VMEM((S, D), F32),
            pltpu.VMEM((S, D), BF16),
            pltpu.VMEM((3, D // 2, D), U32),
            pltpu.VMEM((16, 48, 80), F32),
            pltpu.VMEM((16, 40, S), U32),
            pltpu.VMEM((NM, D), F32),
            pltpu.VMEM((NPAIR, 8, 9 * 128), F32),
            pltpu.VMEM((NPAIR, 16, 9 * 128), F32),
            pltpu.VMEM((64 * UNROLL, D), F32),
            pltpu.SemaphoreType.DMA((7,)),
        ],
        compiler_params=pltpu.CompilerParams(vmem_limit_bytes=120 * 1024 * 1024),
    )(A_x.reshape(S, D), A_wqkv, jnp.transpose(A_w_phi, (1, 2, 0)), A_wo,
      B_mem0.reshape(NM, D), tr(B_Wq), tr(B_Wk), tr(B_Wv), B_Wo.reshape(HB * DB, D))
    return out.reshape(1, S, D)
```

```python
import functools

import jax
import jax.numpy as jnp
import jax.experimental.pallas as pl
import jax.experimental.pallas.tpu as pltpu

F32 = jnp.float32
BF16 = jnp.bfloat16
U32 = jnp.uint32

S = 2048
D = 640
HA = 32
DA = 20
HB = 32
DB = 192
NM = 8
SEG = 32
NPAIR = HB // 2
TB = 512
TC = 256
UNROLL = 1
NXC = 8
NOC = 4
LN_EPS = 1e-5

_NN = (((1,), (0,)), ((), ()))
_NT = (((1,), (1,)), ((), ()))


def _dot(a, b):
    return jax.lax.dot_general(a, b, _NN, preferred_element_type=F32)


def _dot_nt(a, b):
    return jax.lax.dot_general(a, b, _NT, preferred_element_type=F32)


def _ln(x):
    m = jnp.mean(x, axis=-1, keepdims=True)
    xc = x - m
    v = jnp.mean(xc * xc, axis=-1, keepdims=True)
    return xc * jax.lax.rsqrt(v + LN_EPS)


def _iota(shape, dim):
    return jax.lax.broadcasted_iota(jnp.int32, shape, dim)


def _div20(i):
    return (i * 3277) >> 16


def _div40(i):
    return _div20(i) >> 1


def _kernel(x_hbm, wqkv_hbm, wphi_hbm, wo_hbm, mem0_hbm, wqt_hbm, wkt_hbm, wvt_hbm, bwo_hbm,
            out_hbm,
            wphi_ref, mem0_ref, xin, wqkv, woa, wt, wb, bwo, xres, xn32, xnb, wat, kvacc, phiq,
            memv, snext, sdef, opend, sems, xsems, osems):
    XC = S // NXC
    cp_phi = pltpu.make_async_copy(wphi_hbm, wphi_ref, sems.at[0])
    cp_wqkv = pltpu.make_async_copy(wqkv_hbm, wqkv, sems.at[1])

    def cp_x(c):
        rows = pl.ds(pl.multiple_of(c * XC, XC), XC)
        return pltpu.make_async_copy(x_hbm.at[rows], xin.at[rows], xsems.at[c])

    cp_wo = pltpu.make_async_copy(wo_hbm, woa, sems.at[2])
    cp_mem = pltpu.make_async_copy(mem0_hbm, mem0_ref, sems.at[3])
    cp_big = [
        pltpu.make_async_copy(wqt_hbm, wt.at[0], sems.at[4]),
        pltpu.make_async_copy(wkt_hbm, wt.at[1], sems.at[5]),
        pltpu.make_async_copy(wvt_hbm, wt.at[2], sems.at[6]),
    ]
    OC = HB * DB // NOC

    def cp_bwo(c):
        rows = pl.ds(pl.multiple_of(c * OC, OC), OC)
        return pltpu.make_async_copy(bwo_hbm.at[rows], wt.at[3, rows], osems.at[c])

    def start_first(c, carry):
        @pl.when(c == 0)
        def _():
            cp_phi.start()

        @pl.when(c == 1)
        def _():
            cp_wqkv.start()

        @pl.when(c >= 2)
        def _():
            cp_x(c - 2).start()

        return carry

    jax.lax.fori_loop(0, NXC + 2, start_first, 0)
    cp_phi.wait()

    wphi = wphi_ref[...].astype(F32)
    xw = jnp.concatenate([wphi[d] for d in range(DA)], axis=1)
    xw = jnp.concatenate([xw, jnp.zeros((32 - DA, D), F32)], axis=0).astype(BF16)
    r = _iota((D, D), 0)
    c = _iota((D, D), 1)
    perm = jnp.where((r & 31) * DA + (r >> 5) == c, 1.0, 0.0).astype(BF16)
    wf = _dot(xw, perm).astype(BF16)
    r = _iota((160, 32), 0)
    c = _iota((160, 32), 1)
    rsel = jnp.where(((r - _div40(r) * 40) >> 1) == c, 1.0, 0.0).astype(BF16)
    r = _iota((160, 128), 0)
    c = _iota((160, 128), 1)
    phit = []
    for t in range(5):
        keep = 2 * (_div40(r) + 3 * t) + (r & 1) == _div20(c + 128 * t)
        phit.append(jnp.where(keep, _dot(rsel, wf[:, 128 * t:128 * (t + 1)]), 0.0).astype(BF16))

    cp_wqkv.wait()
    cp_big[0].start()
    for m, dst in ((1, 0), (0, 1)):
        p = [_dot_nt(phit[t], wqkv[:, m * D + 128 * t:m * D + 128 * (t + 1)]) for t in range(5)]
        rows = [p[0][0:120]]
        for t in range(1, 5):
            rows += [p[t - 1][120:160] + p[t][0:40], p[t][40:120]]
        rows.append(p[4][120:160])
        wat[dst] = pltpu.bitcast(jnp.concatenate(rows, axis=0).astype(BF16), U32)
    wat[2] = pltpu.bitcast(wqkv[:, 2 * D:3 * D].T, U32)

    def init_blk(i, carry):
        cp_x(i).wait()
        for u in range(XC // 64):
            off = pl.multiple_of(i * XC + u * 64, 64)
            x = xin[pl.ds(off, 64), :].astype(F32)
            xres[pl.ds(off, 64), :] = x
            xnb[pl.ds(pl.multiple_of(off // 2, 32), 32), :] = pltpu.bitcast(_ln(x).astype(BF16), U32)
        return carry

    jax.lax.fori_loop(0, NXC, init_blk, 0)
    cp_big[1].start()

    def transpose_tiles(src, dst, jlo, jhi):
        for j in range(jlo, jhi):
            for t in range(3):
                off = j * 384 + t * 128
                wb[9 * j + 3 * dst + t] = pltpu.bitcast(wt[src, off:off + 128, :].T, U32)

    def layer_a(l):
        kvacc[...] = jnp.zeros_like(kvacc)

        def sub_all(x, op):
            x = op(x, pltpu.roll(x, 2, 0))
            return op(x, pltpu.roll(x, 4, 0))

        def phi(p):
            ts = [p[8 * t:8 * (t + 1)] for t in range(5)]
            mx = sub_all(functools.reduce(jnp.maximum, ts), jnp.maximum)
            mn = sub_all(functools.reduce(jnp.minimum, ts), jnp.minimum)
            ep = [jnp.exp(t - mx) for t in ts]
            en = [jnp.exp(mn - t) for t in ts]
            rp = 1.0 / sub_all(functools.reduce(jnp.add, ep), jnp.add)
            rn = 1.0 / sub_all(functools.reduce(jnp.add, en), jnp.add)
            return jnp.concatenate([e * rp for e in ep] + [e * rn for e in en], axis=0).astype(BF16)

        def phase1(i, carry):
            @pl.when(jnp.logical_and(l == 0, i == 0))
            def _():
                cp_wo.start()
                cp_mem.start()

            @pl.when(jnp.logical_and(l == 0, i == 1))
            def _():
                cp_big[2].start()

            @pl.when(jnp.logical_and(l == 0, i == 2))
            def _():
                for c in range(NOC):
                    cp_bwo(c).start()
                cp_big[0].wait()

            @pl.when(jnp.logical_and(l == 0, i == 3))
            def _():
                cp_big[1].wait()

            transpose_tiles(jnp.where(i < 2, 3, i - 2), jnp.where(i < 2, 2, i - 2), 0, NPAIR)
            off = pl.multiple_of(i * TB, TB)
            xn = pltpu.bitcast(xnb[pl.ds(pl.multiple_of(i * (TB // 2), TB // 2), TB // 2), :], BF16)
            pk = _dot_nt(pltpu.bitcast(wat[0], BF16), xn)
            phik = [phi(pk[40 * j:40 * (j + 1)]) for j in range(16)]
            pq = _dot_nt(pltpu.bitcast(wat[1], BF16), xn)
            for j in range(16):
                phiq[j, :, pl.ds(off, TB)] = pltpu.bitcast(phi(pq[40 * j:40 * (j + 1)]), U32)
            hb = TB // 2
            vt = [_dot_nt(pltpu.bitcast(wat[2], BF16), xn[hb * u:hb * (u + 1)]) for u in range(2)]
            ones = jnp.ones((8, hb), F32)
            for u in range(2):
                for j in range(16):
                    lhs = jnp.concatenate([vt[u][40 * j:40 * (j + 1)], ones], axis=0).astype(BF16)
                    kvacc[j] = _dot_nt(lhs, phik[j][:, hb * u:hb * (u + 1)]) + kvacc[j]
            return carry

        jax.lax.fori_loop(0, S // TB, phase1, 0)

        @pl.when(l == 0)
        def _():
            cp_wo.wait()
            cp_mem.wait()

        rr = _iota((48, 80), 0)
        cc = _iota((48, 80), 1)
        keep = jnp.where(rr < 40, _div20(rr), (rr - 40) >> 2) == (cc & 1)
        kvm = [jnp.where(keep, kvacc[j], 0.0).astype(BF16) for j in range(16)]
        lo4 = _iota((8, TC), 0) < 4

        def num(b):
            parts = []
            for j in range(16):
                r = _dot(kvm[j], pltpu.bitcast(phiq[j, :, TC * b:TC * (b + 1)], BF16))
                rc = 1.0 / (r[40:48] + 1e-6)
                rc2 = pltpu.roll(rc, 4, 0)
                ra = jnp.where(lo4, rc, rc2)
                rb = jnp.where(lo4, rc2, rc)
                parts += [r[0:8] * ra, r[8:16] * ra, r[16:24] * rc, r[24:32] * rb, r[32:40] * rb]
            return jnp.concatenate(parts, axis=0).astype(BF16).T

        def out(b, o):
            rows = slice(TC * b, TC * (b + 1))
            xnew = xres[rows, :] + _dot(o, woa[...])
            xres[rows, :] = xnew
            xn32[rows, :] = _ln(xnew)

        nb = S // TC
        os_ = [None] * nb
        os_[0] = num(0)
        os_[1] = num(1)
        for b in range(nb):
            if b == 2:
                @pl.when(l == 0)
                def _():
                    cp_big[2].wait()
            if b >= 2:
                transpose_tiles(2, 2, (b - 2) * NPAIR // 6, (b - 1) * NPAIR // 6)
            if b + 2 < nb:
                os_[b + 2] = num(b + 2)
            out(b, os_[b])

        @pl.when(l == 0)
        def _():
            def cpo(c, carry):
                cp_bwo(c).wait()
                for u in range(OC // 384):
                    off = pl.multiple_of(c * OC + u * 384, 384)
                    bwo[pl.ds(pl.multiple_of(off // 2, 192), 192), :] = pltpu.bitcast(
                        wt[3, pl.ds(off, 384), :], U32)
                return carry

            jax.lax.fori_loop(0, NOC, cpo, 0)

    scale = DB ** (-0.5)

    def layer_b(layer):
        L = SEG + NM
        NEG = -1000000000.0

        def masks(even):
            nrow = SEG if even else L + 8
            rr = _iota((nrow, 128), 0)
            cc = _iota((nrow, 128), 1)
            is_a = (cc < L) | ((cc >= 2 * L) & (cc < 2 * L + 16))
            kx = jnp.where(cc < L, cc, cc - (L + NM))
            is_memkey = (cc >= SEG) & (cc < SEG + 2 * NM)
            if even:
                valid = cc < 2 * L
                allowed = valid & (is_memkey | (rr >= 24) | (kx <= rr + 8))
            else:
                dk = (cc - 2 * L) & 15
                cur = (rr < L) & (cc < 2 * L)
                old = (rr >= L) & (cc >= 2 * L) & (cc < 2 * L + 32)
                valid = cur | old
                allowed = ((cur & (is_memkey | (rr >= SEG) | (kx <= rr)))
                           | (old & ((dk >= 8) | (dk <= rr - L))))
            return is_a, allowed, jnp.where(valid, NEG, -jnp.inf).astype(F32)

        all_masks = {True: masks(True), False: masks(False)}

        def lo64(y):
            return _iota(y.shape, 1) < 64

        def stack_keys(a, b):
            parts = [a[0:L], b[SEG:L], b[0:SEG]]
            if a.shape[0] > L:
                parts += [a[L:], b[L:]]
            return jnp.concatenate(parts, axis=0).astype(BF16)

        def expand(y):
            y0, y1, y2 = y[:, 0:128], y[:, 128:256], y[:, 256:384]
            return (stack_keys(y0, y2),
                    stack_keys(jnp.where(lo64(y1), y1, 0.0), jnp.where(lo64(y1), 0.0, y1)))

        def pad_lanes(s):
            return jnp.concatenate([s, jnp.zeros((s.shape[0], 128 - s.shape[1]), F32)], axis=1)

        def step(h, even, kmajor):
            is_a, allowed, fill = all_masks[even]
            nrow = SEG if even else L + 8
            nkey = 2 * L if even else 2 * L + 32

            def proj(j):
                w = jnp.concatenate(
                    [pltpu.bitcast(wb[9 * j + t], BF16) for t in range(9)], axis=1)
                if j == 0 and kmajor:
                    y = _dot(h[:, 0:128], w[0:128])
                    for t in range(1, 5):
                        y = _dot(h[:, 128 * t:128 * (t + 1)], w[128 * t:128 * (t + 1)]) + y
                else:
                    y = _dot(h, w)
                if even:
                    snext[j] = y[SEG:L]
                    sdef[j, 0:8, :] = y[0:8]
                    sdef[j, 8:16, 384:1152] = y[L:L + 8, 384:1152]
                    q = jnp.concatenate([y[8:SEG, 0:384], y[L:L + 8, 0:384]], axis=0)
                    kv = jnp.concatenate([y[0:SEG, 384:1152], y[L:L + 8, 384:1152]], axis=0)
                else:
                    q = jnp.concatenate(
                        [snext[j, :, 0:384], y[:, 0:384], sdef[j, 0:8, 0:384]], axis=0)
                    kv = jnp.concatenate(
                        [snext[j, :, 384:1152], y[:, 384:1152], sdef[j, :, 384:1152]], axis=0)
                q = q.astype(BF16)
                q = (jnp.concatenate([q[:, 0:128], q[:, 256:384]], axis=0), q[:, 128:256])
                return q, expand(kv[:, 0:384]), expand(kv[:, 384:768])

            def scores(q, k):
                s02 = pad_lanes(_dot_nt(q[0], k[0]))
                s = jnp.where(is_a, s02[0:nrow], s02[nrow:]) + pad_lanes(_dot_nt(q[1], k[1]))
                s = jnp.where(allowed, s * scale, fill)
                ma = jnp.max(jnp.where(is_a, s, -jnp.inf), axis=1, keepdims=True)
                mb = jnp.max(jnp.where(is_a, -jnp.inf, s), axis=1, keepdims=True)
                e = jnp.exp(s - jnp.where(is_a, ma, mb))
                ea = jnp.where(is_a, e, 0.0)
                eb = jnp.where(is_a, 0.0, e)
                pa = ea * (1.0 / jnp.sum(ea, axis=1, keepdims=True))
                pb = eb * (1.0 / jnp.sum(eb, axis=1, keepdims=True))
                return (jnp.concatenate([pa, pb], axis=0)[:, 0:nkey].astype(BF16),
                        (pa + pb)[:, 0:nkey].astype(BF16))

            def pv(p, v):
                o02 = _dot(p[0], v[0])
                return jnp.concatenate(
                    [o02[0:nrow], _dot(p[1], v[1]), o02[nrow:]], axis=1).astype(BF16)

            qkv = [None] * NPAIR
            ps = [None] * NPAIR
            os_ = [None] * NPAIR

            def wo_chunk(c0, c1):
                w = pltpu.bitcast(bwo[192 * c0:192 * c1, :], BF16)
                return _dot(jnp.concatenate(os_[c0:c1], axis=1), w)

            fill_chunks = {NPAIR - 1: (0, 4), NPAIR: (4, 8), NPAIR + 1: (8, 11)}
            qkv[0] = proj(0)
            acc = None
            for j in range(NPAIR + 2):
                if j + 1 < NPAIR:
                    qkv[j + 1] = proj(j + 1)
                else:
                    c = wo_chunk(*fill_chunks[j])
                    acc = c if acc is None else c + acc
                if j < NPAIR:
                    ps[j] = scores(qkv[j][0], qkv[j][1])
                if j >= 2:
                    os_[j - 2] = pv(ps[j - 2], qkv[j - 2][2])
            acc = wo_chunk(11, 14) + acc
            return wo_chunk(14, 16) + acc

        RB = 64 * UNROLL

        def finish_rows(base):
            xnew = xres[pl.ds(base, RB), :] + opend[...]
            xres[pl.ds(base, RB), :] = xnew
            xnb[pl.ds(pl.multiple_of(base // 2, RB // 2), RB // 2), :] = pltpu.bitcast(
                _ln(xnew).astype(BF16), U32)
            xin[pl.ds(base, RB), :] = xnew.astype(BF16)

        memv[...] = mem0_ref[...].astype(F32)
        opend[...] = jnp.zeros_like(opend)

        def body(i, carry):
            base = pl.multiple_of(i * RB, RB)
            finish_rows(pl.multiple_of(jnp.maximum(i - 1, 0) * RB, RB))
            mem = memv[...]
            for u in range(UNROLL):
                r0 = 64 * u
                h0 = jnp.concatenate([xn32[pl.ds(base + r0, 40), :], mem], axis=0).astype(BF16)
                o0 = step(h0, True, u > 0)
                opend[r0 + 8:r0 + 32, :] = o0[0:24]
                h1 = jnp.concatenate(
                    [xn32[pl.ds(base + r0 + 40, 24), :], o0[24:32]], axis=0).astype(BF16)
                o1 = step(h1, False, True)
                mem = o1[32:40]
                opend[r0:r0 + 8, :] = o1[40:48]
                opend[r0 + 32:r0 + 64, :] = o1[0:32]
            memv[...] = mem
            return carry

        jax.lax.fori_loop(0, S // RB, body, 0)
        finish_rows(S - RB)

    def layer(l, carry):
        layer_a(l)
        layer_b(l)
        return carry

    jax.lax.fori_loop(0, 2, layer, 0)

    cp_out = pltpu.make_async_copy(xin, out_hbm, sems.at[0])
    cp_out.start()
    cp_out.wait()


@functools.partial(jax.jit, static_argnames=("B_seg_len",))
def pallas_interleave_layers__linear_kernel_hedgehog__memory_aug_recurrent_mem_tr__prompt_kernel(
    A_x: jax.Array,
    A_wqkv: jax.Array,
    A_w_phi: jax.Array,
    A_wo: jax.Array,
    B_x: jax.Array,
    B_mem0: jax.Array,
    B_Wq: jax.Array,
    B_Wk: jax.Array,
    B_Wv: jax.Array,
    B_Wo: jax.Array,
    B_seg_len=SEG,
):
    assert B_seg_len == SEG and A_x.shape == (1, S, D)
    tr = lambda w: jnp.transpose(w, (1, 2, 0)).reshape(HB * DB, D)
    any_spec = pl.BlockSpec(memory_space=pl.ANY)
    out = pl.pallas_call(
        _kernel,
        out_shape=jax.ShapeDtypeStruct((S, D), BF16),
        in_specs=[any_spec] * 9,
        out_specs=any_spec,
        scratch_shapes=[
            pltpu.VMEM((DA, DA, HA), BF16),
            pltpu.VMEM((NM, D), BF16),
            pltpu.VMEM((S, D), BF16),
            pltpu.VMEM((D, 3 * D), BF16),
            pltpu.VMEM((D, D), BF16),
            pltpu.VMEM((4, HB * DB, D), BF16),
            pltpu.VMEM((9 * NPAIR, D // 2, 128), U32),
            pltpu.VMEM((HB * DB // 2, D), U32),
            pltpu.VMEM((S, D), F32),
            pltpu.VMEM((S, D), F32),
            pltpu.VMEM((S // 2, D), U32),
            pltpu.VMEM((3, D // 2, D), U32),
            pltpu.VMEM((16, 48, 80), F32),
            pltpu.VMEM((16, 40, S), U32),
            pltpu.VMEM((NM, D), F32),
            pltpu.VMEM((NPAIR, 8, 9 * 128), F32),
            pltpu.VMEM((NPAIR, 16, 9 * 128), F32),
            pltpu.VMEM((64 * UNROLL, D), F32),
            pltpu.SemaphoreType.DMA((7,)),
            pltpu.SemaphoreType.DMA((NXC,)),
            pltpu.SemaphoreType.DMA((NOC,)),
        ],
        compiler_params=pltpu.CompilerParams(vmem_limit_bytes=120 * 1024 * 1024),
    )(A_x.reshape(S, D), A_wqkv, jnp.transpose(A_w_phi, (1, 2, 0)), A_wo,
      B_mem0.reshape(NM, D), tr(B_Wq), tr(B_Wk), tr(B_Wv), B_Wo.reshape(HB * DB, D))
    return out.reshape(1, S, D)
```

```python
import functools

import jax
import jax.numpy as jnp
import jax.experimental.pallas as pl
import jax.experimental.pallas.tpu as pltpu

F32 = jnp.float32
BF16 = jnp.bfloat16
U32 = jnp.uint32

S = 2048
D = 640
HA = 32
DA = 20
HB = 32
DB = 192
NM = 8
SEG = 32
NPAIR = HB // 2
TB = 512
TC = 256
UNROLL = 1
NXC = 8
NOC = 4
LN_EPS = 1e-5

_NN = (((1,), (0,)), ((), ()))
_NT = (((1,), (1,)), ((), ()))


def _dot(a, b):
    return jax.lax.dot_general(a, b, _NN, preferred_element_type=F32)


def _dot_nt(a, b):
    return jax.lax.dot_general(a, b, _NT, preferred_element_type=F32)


def _ln(x):
    m = jnp.mean(x, axis=-1, keepdims=True)
    xc = x - m
    v = jnp.mean(xc * xc, axis=-1, keepdims=True)
    return xc * jax.lax.rsqrt(v + LN_EPS)


def _iota(shape, dim):
    return jax.lax.broadcasted_iota(jnp.int32, shape, dim)


def _div20(i):
    return (i * 3277) >> 16


def _div40(i):
    return _div20(i) >> 1


def _kernel(x_hbm, wqkv_hbm, wphi_hbm, wo_hbm, mem0_hbm, wqt_hbm, wkt_hbm, wvt_hbm, bwo_hbm,
            out_hbm,
            wphi_ref, mem0_ref, xin, wqkv, woa, wt, wb, bwo, xres, xn32, xnb, wat, kvacc, phiq,
            memv, snext, sdef, opend, sems, xsems, osems):
    XC = S // NXC
    cp_phi = pltpu.make_async_copy(wphi_hbm, wphi_ref, sems.at[0])
    cp_wqkv = pltpu.make_async_copy(wqkv_hbm, wqkv, sems.at[1])

    def cp_x(c):
        rows = pl.ds(pl.multiple_of(c * XC, XC), XC)
        return pltpu.make_async_copy(x_hbm.at[rows], xin.at[rows], xsems.at[c])

    cp_wo = pltpu.make_async_copy(wo_hbm, woa, sems.at[2])
    cp_mem = pltpu.make_async_copy(mem0_hbm, mem0_ref, sems.at[3])
    cp_big = [
        pltpu.make_async_copy(wqt_hbm, wt.at[0], sems.at[4]),
        pltpu.make_async_copy(wkt_hbm, wt.at[1], sems.at[5]),
        pltpu.make_async_copy(wvt_hbm, wt.at[2], sems.at[6]),
    ]
    OC = HB * DB // NOC

    def cp_bwo(c):
        rows = pl.ds(pl.multiple_of(c * OC, OC), OC)
        return pltpu.make_async_copy(bwo_hbm.at[rows], wt.at[3, rows], osems.at[c])

    def start_first(c, carry):
        @pl.when(c == 0)
        def _():
            cp_phi.start()

        @pl.when(c == 1)
        def _():
            cp_wqkv.start()

        @pl.when(c >= 2)
        def _():
            cp_x(c - 2).start()

        return carry

    jax.lax.fori_loop(0, NXC + 2, start_first, 0)
    cp_phi.wait()

    wphi = wphi_ref[...].astype(F32)
    xw = jnp.concatenate([wphi[d] for d in range(DA)], axis=1)
    xw = jnp.concatenate([xw, jnp.zeros((32 - DA, D), F32)], axis=0).astype(BF16)
    r = _iota((D, D), 0)
    c = _iota((D, D), 1)
    perm = jnp.where((r & 31) * DA + (r >> 5) == c, 1.0, 0.0).astype(BF16)
    wf = _dot(xw, perm).astype(BF16)
    r = _iota((160, 32), 0)
    c = _iota((160, 32), 1)
    rsel = jnp.where(((r - _div40(r) * 40) >> 1) == c, 1.0, 0.0).astype(BF16)
    r = _iota((160, 128), 0)
    c = _iota((160, 128), 1)
    phit = []
    for t in range(5):
        keep = 2 * (_div40(r) + 3 * t) + (r & 1) == _div20(c + 128 * t)
        phit.append(jnp.where(keep, _dot(rsel, wf[:, 128 * t:128 * (t + 1)]), 0.0).astype(BF16))

    cp_wqkv.wait()
    cp_big[0].start()
    for m, dst in ((1, 0), (0, 1)):
        p = [_dot_nt(phit[t], wqkv[:, m * D + 128 * t:m * D + 128 * (t + 1)]) for t in range(5)]
        rows = [p[0][0:120]]
        for t in range(1, 5):
            rows += [p[t - 1][120:160] + p[t][0:40], p[t][40:120]]
        rows.append(p[4][120:160])
        wat[dst] = pltpu.bitcast(jnp.concatenate(rows, axis=0).astype(BF16), U32)
    wat[2] = pltpu.bitcast(wqkv[:, 2 * D:3 * D].T, U32)

    def init_blk(i, carry):
        cp_x(i).wait()
        for u in range(XC // 64):
            off = pl.multiple_of(i * XC + u * 64, 64)
            x = xin[pl.ds(off, 64), :].astype(F32)
            xres[pl.ds(off, 64), :] = x
            xnb[pl.ds(pl.multiple_of(off // 2, 32), 32), :] = pltpu.bitcast(_ln(x).astype(BF16), U32)
        return carry

    jax.lax.fori_loop(0, NXC, init_blk, 0)
    cp_big[1].start()

    def transpose_tiles(src, dst, jlo, jhi):
        for j in range(jlo, jhi):
            for t in range(3):
                off = j * 384 + t * 128
                wb[9 * j + 3 * dst + t] = pltpu.bitcast(wt[src, off:off + 128, :].T, U32)

    def layer_a(l):
        kvacc[...] = jnp.zeros_like(kvacc)

        def sub_all(x, op):
            x = op(x, pltpu.roll(x, 2, 0))
            return op(x, pltpu.roll(x, 4, 0))

        def phi(p):
            ts = [p[8 * t:8 * (t + 1)] for t in range(5)]
            mx = sub_all(functools.reduce(jnp.maximum, ts), jnp.maximum)
            mn = sub_all(functools.reduce(jnp.minimum, ts), jnp.minimum)
            ep = [jnp.exp(t - mx) for t in ts]
            en = [jnp.exp(mn - t) for t in ts]
            rp = 1.0 / sub_all(functools.reduce(jnp.add, ep), jnp.add)
            rn = 1.0 / sub_all(functools.reduce(jnp.add, en), jnp.add)
            return jnp.concatenate([e * rp for e in ep] + [e * rn for e in en], axis=0).astype(BF16)

        def phase1(i, carry):
            @pl.when(jnp.logical_and(l == 0, i == 0))
            def _():
                cp_wo.start()
                cp_mem.start()

            @pl.when(jnp.logical_and(l == 0, i == 1))
            def _():
                cp_big[2].start()

            @pl.when(jnp.logical_and(l == 0, i == 2))
            def _():
                for c in range(NOC):
                    cp_bwo(c).start()
                cp_big[0].wait()

            @pl.when(jnp.logical_and(l == 0, i == 3))
            def _():
                cp_big[1].wait()

            transpose_tiles(jnp.where(i < 2, 3, i - 2), jnp.where(i < 2, 2, i - 2), 0, NPAIR)
            off = pl.multiple_of(i * TB, TB)
            xn = pltpu.bitcast(xnb[pl.ds(pl.multiple_of(i * (TB // 2), TB // 2), TB // 2), :], BF16)
            pk = _dot_nt(pltpu.bitcast(wat[0], BF16), xn)
            phik = [phi(pk[40 * j:40 * (j + 1)]) for j in range(16)]
            pq = _dot_nt(pltpu.bitcast(wat[1], BF16), xn)
            for j in range(16):
                phiq[j, :, pl.ds(off, TB)] = pltpu.bitcast(phi(pq[40 * j:40 * (j + 1)]), U32)
            hb = TB // 2
            vt = [_dot_nt(pltpu.bitcast(wat[2], BF16), xn[hb * u:hb * (u + 1)]) for u in range(2)]
            ones = jnp.ones((8, hb), F32)
            for u in range(2):
                for j in range(16):
                    lhs = jnp.concatenate([vt[u][40 * j:40 * (j + 1)], ones], axis=0).astype(BF16)
                    kvacc[j] = _dot_nt(lhs, phik[j][:, hb * u:hb * (u + 1)]) + kvacc[j]
            return carry

        jax.lax.fori_loop(0, S // TB, phase1, 0)

        @pl.when(l == 0)
        def _():
            cp_wo.wait()
            cp_mem.wait()

        rr = _iota((48, 80), 0)
        cc = _iota((48, 80), 1)
        keep = jnp.where(rr < 40, _div20(rr), (rr - 40) >> 2) == (cc & 1)
        kvm = [jnp.where(keep, kvacc[j], 0.0).astype(BF16) for j in range(16)]
        lo4 = _iota((8, TC), 0) < 4

        def num(b):
            parts = []
            for j in range(16):
                r = _dot(kvm[j], pltpu.bitcast(phiq[j, :, TC * b:TC * (b + 1)], BF16))
                rc = 1.0 / (r[40:48] + 1e-6)
                rc2 = pltpu.roll(rc, 4, 0)
                ra = jnp.where(lo4, rc, rc2)
                rb = jnp.where(lo4, rc2, rc)
                parts += [r[0:8] * ra, r[8:16] * ra, r[16:24] * rc, r[24:32] * rb, r[32:40] * rb]
            return jnp.concatenate(parts, axis=0).astype(BF16).T

        def out(b, o):
            rows = slice(TC * b, TC * (b + 1))
            xnew = xres[rows, :] + _dot(o, woa[...])
            xres[rows, :] = xnew
            xn32[rows, :] = _ln(xnew)

        nb = S // TC
        os_ = [None] * nb
        os_[0] = num(0)
        os_[1] = num(1)
        for b in range(nb):
            if b == 2:
                @pl.when(l == 0)
                def _():
                    cp_big[2].wait()
            if b >= 2:
                transpose_tiles(2, 2, (b - 2) * NPAIR // 6, (b - 1) * NPAIR // 6)
            if b + 2 < nb:
                os_[b + 2] = num(b + 2)
            out(b, os_[b])

        @pl.when(l == 0)
        def _():
            def cpo(c, carry):
                cp_bwo(c).wait()
                for u in range(OC // 384):
                    off = pl.multiple_of(c * OC + u * 384, 384)
                    bwo[pl.ds(pl.multiple_of(off // 2, 192), 192), :] = pltpu.bitcast(
                        wt[3, pl.ds(off, 384), :], U32)
                return carry

            jax.lax.fori_loop(0, NOC, cpo, 0)

    scale = DB ** (-0.5)

    def layer_b(layer):
        L = SEG + NM
        NEG = -1000000000.0

        def masks(even):
            nrow = SEG if even else L + 8
            rr = _iota((nrow, 128), 0)
            cc = _iota((nrow, 128), 1)
            is_a = (cc < L) | ((cc >= 2 * L) & (cc < 2 * L + 16))
            kx = jnp.where(cc < L, cc, cc - (L + NM))
            is_memkey = (cc >= SEG) & (cc < SEG + 2 * NM)
            if even:
                valid = cc < 2 * L
                allowed = valid & (is_memkey | (rr >= 24) | (kx <= rr + 8))
            else:
                dk = (cc - 2 * L) & 15
                cur = (rr < L) & (cc < 2 * L)
                old = (rr >= L) & (cc >= 2 * L) & (cc < 2 * L + 32)
                valid = cur | old
                allowed = ((cur & (is_memkey | (rr >= SEG) | (kx <= rr)))
                           | (old & ((dk >= 8) | (dk <= rr - L))))
            return is_a, allowed, jnp.where(valid, NEG, -jnp.inf).astype(F32)

        all_masks = {True: masks(True), False: masks(False)}

        def lo64(y):
            return _iota(y.shape, 1) < 64

        def stack_keys(a, b):
            parts = [a[0:L], b[SEG:L], b[0:SEG]]
            if a.shape[0] > L:
                parts += [a[L:], b[L:]]
            return jnp.concatenate(parts, axis=0).astype(BF16)

        def expand(y):
            y0, y1, y2 = y[:, 0:128], y[:, 128:256], y[:, 256:384]
            return (stack_keys(y0, y2),
                    stack_keys(jnp.where(lo64(y1), y1, 0.0), jnp.where(lo64(y1), 0.0, y1)))

        def pad_lanes(s):
            return jnp.concatenate([s, jnp.zeros((s.shape[0], 128 - s.shape[1]), F32)], axis=1)

        def step(h, even, kmajor):
            is_a, allowed, fill = all_masks[even]
            nrow = SEG if even else L + 8
            nkey = 2 * L if even else 2 * L + 32

            def proj(j):
                w = jnp.concatenate(
                    [pltpu.bitcast(wb[9 * j + t], BF16) for t in range(9)], axis=1)
                if j == 0 and kmajor:
                    y = _dot(h[:, 0:128], w[0:128])
                    for t in range(1, 5):
                        y = _dot(h[:, 128 * t:128 * (t + 1)], w[128 * t:128 * (t + 1)]) + y
                else:
                    y = _dot(h, w)
                if even:
                    snext[j] = y[SEG:L]
                    sdef[j, 0:8, :] = y[0:8]
                    sdef[j, 8:16, 384:1152] = y[L:L + 8, 384:1152]
                    q = jnp.concatenate([y[8:SEG, 0:384], y[L:L + 8, 0:384]], axis=0)
                    kv = jnp.concatenate([y[0:SEG, 384:1152], y[L:L + 8, 384:1152]], axis=0)
                else:
                    q = jnp.concatenate(
                        [snext[j, :, 0:384], y[:, 0:384], sdef[j, 0:8, 0:384]], axis=0)
                    kv = jnp.concatenate(
                        [snext[j, :, 384:1152], y[:, 384:1152], sdef[j, :, 384:1152]], axis=0)
                q = q.astype(BF16)
                q = (jnp.concatenate([q[:, 0:128], q[:, 256:384]], axis=0), q[:, 128:256])
                return q, expand(kv[:, 0:384]), expand(kv[:, 384:768])

            def scores(q, k):
                s02 = pad_lanes(_dot_nt(q[0], k[0]))
                s = jnp.where(is_a, s02[0:nrow], s02[nrow:]) + pad_lanes(_dot_nt(q[1], k[1]))
                s = jnp.where(allowed, s * scale, fill)
                ma = jnp.max(jnp.where(is_a, s, -jnp.inf), axis=1, keepdims=True)
                mb = jnp.max(jnp.where(is_a, -jnp.inf, s), axis=1, keepdims=True)
                e = jnp.exp(s - jnp.where(is_a, ma, mb))
                ea = jnp.where(is_a, e, 0.0)
                eb = jnp.where(is_a, 0.0, e)
                pa = ea * (1.0 / jnp.sum(ea, axis=1, keepdims=True))
                pb = eb * (1.0 / jnp.sum(eb, axis=1, keepdims=True))
                return (jnp.concatenate([pa, pb], axis=0)[:, 0:nkey].astype(BF16),
                        (pa + pb)[:, 0:nkey].astype(BF16))

            def pv(p, v):
                o02 = _dot(p[0], v[0])
                return jnp.concatenate(
                    [o02[0:nrow], _dot(p[1], v[1]), o02[nrow:]], axis=1).astype(BF16)

            qkv = [None] * NPAIR
            ps = [None] * NPAIR
            os_ = [None] * NPAIR

            def wo_chunk(c0, c1):
                w = pltpu.bitcast(bwo[192 * c0:192 * c1, :], BF16)
                return _dot(jnp.concatenate(os_[c0:c1], axis=1), w)

            fill_chunks = {NPAIR - 1: (0, 4), NPAIR: (4, 8), NPAIR + 1: (8, 11)}
            qkv[0] = proj(0)
            acc = None
            for j in range(NPAIR + 2):
                if j + 1 < NPAIR:
                    qkv[j + 1] = proj(j + 1)
                else:
                    c = wo_chunk(*fill_chunks[j])
                    acc = c if acc is None else c + acc
                if j < NPAIR:
                    ps[j] = scores(qkv[j][0], qkv[j][1])
                if j >= 2:
                    os_[j - 2] = pv(ps[j - 2], qkv[j - 2][2])
            acc = wo_chunk(11, 14) + acc
            return wo_chunk(14, 16) + acc

        RB = 64 * UNROLL

        def finish_rows(base):
            xnew = xres[pl.ds(base, RB), :] + opend[...]
            xres[pl.ds(base, RB), :] = xnew
            xnb[pl.ds(pl.multiple_of(base // 2, RB // 2), RB // 2), :] = pltpu.bitcast(
                _ln(xnew).astype(BF16), U32)
            xin[pl.ds(base, RB), :] = xnew.astype(BF16)

        memv[...] = mem0_ref[...].astype(F32)
        opend[...] = jnp.zeros_like(opend)

        def body(i, carry):
            base = pl.multiple_of(i * RB, RB)

            @pl.when(jnp.logical_and(layer == 1, i >= 2))
            def _():
                rows = pl.ds(pl.multiple_of((i - 2) * RB, RB), RB)
                pltpu.make_async_copy(xin.at[rows], out_hbm.at[rows], sems.at[0]).start()

            finish_rows(pl.multiple_of(jnp.maximum(i - 1, 0) * RB, RB))
            mem = memv[...]
            for u in range(UNROLL):
                r0 = 64 * u
                h0 = jnp.concatenate([xn32[pl.ds(base + r0, 40), :], mem], axis=0).astype(BF16)
                o0 = step(h0, True, u > 0)
                opend[r0 + 8:r0 + 32, :] = o0[0:24]
                h1 = jnp.concatenate(
                    [xn32[pl.ds(base + r0 + 40, 24), :], o0[24:32]], axis=0).astype(BF16)
                o1 = step(h1, False, True)
                mem = o1[32:40]
                opend[r0:r0 + 8, :] = o1[40:48]
                opend[r0 + 32:r0 + 64, :] = o1[0:32]
            memv[...] = mem
            return carry

        jax.lax.fori_loop(0, S // RB, body, 0)
        finish_rows(S - RB)

    def layer(l, carry):
        layer_a(l)
        layer_b(l)
        return carry

    jax.lax.fori_loop(0, 2, layer, 0)

    last = pl.ds(S - 128 * UNROLL, 128 * UNROLL)
    pltpu.make_async_copy(xin.at[last], out_hbm.at[last], sems.at[0]).start()
    pltpu.make_async_copy(xin, out_hbm, sems.at[0]).wait()


@functools.partial(jax.jit, static_argnames=("B_seg_len",))
def pallas_interleave_layers__linear_kernel_hedgehog__memory_aug_recurrent_mem_tr__prompt_kernel(
    A_x: jax.Array,
    A_wqkv: jax.Array,
    A_w_phi: jax.Array,
    A_wo: jax.Array,
    B_x: jax.Array,
    B_mem0: jax.Array,
    B_Wq: jax.Array,
    B_Wk: jax.Array,
    B_Wv: jax.Array,
    B_Wo: jax.Array,
    B_seg_len=SEG,
):
    assert B_seg_len == SEG and A_x.shape == (1, S, D)
    tr = lambda w: jnp.transpose(w, (1, 2, 0)).reshape(HB * DB, D)
    any_spec = pl.BlockSpec(memory_space=pl.ANY)
    out = pl.pallas_call(
        _kernel,
        out_shape=jax.ShapeDtypeStruct((S, D), BF16),
        in_specs=[any_spec] * 9,
        out_specs=any_spec,
        scratch_shapes=[
            pltpu.VMEM((DA, DA, HA), BF16),
            pltpu.VMEM((NM, D), BF16),
            pltpu.VMEM((S, D), BF16),
            pltpu.VMEM((D, 3 * D), BF16),
            pltpu.VMEM((D, D), BF16),
            pltpu.VMEM((4, HB * DB, D), BF16),
            pltpu.VMEM((9 * NPAIR, D // 2, 128), U32),
            pltpu.VMEM((HB * DB // 2, D), U32),
            pltpu.VMEM((S, D), F32),
            pltpu.VMEM((S, D), F32),
            pltpu.VMEM((S // 2, D), U32),
            pltpu.VMEM((3, D // 2, D), U32),
            pltpu.VMEM((16, 48, 80), F32),
            pltpu.VMEM((16, 40, S), U32),
            pltpu.VMEM((NM, D), F32),
            pltpu.VMEM((NPAIR, 8, 9 * 128), F32),
            pltpu.VMEM((NPAIR, 16, 9 * 128), F32),
            pltpu.VMEM((64 * UNROLL, D), F32),
            pltpu.SemaphoreType.DMA((7,)),
            pltpu.SemaphoreType.DMA((NXC,)),
            pltpu.SemaphoreType.DMA((NOC,)),
        ],
        compiler_params=pltpu.CompilerParams(vmem_limit_bytes=120 * 1024 * 1024),
    )(A_x.reshape(S, D), A_wqkv, jnp.transpose(A_w_phi, (1, 2, 0)), A_wo,
      B_mem0.reshape(NM, D), tr(B_Wq), tr(B_Wk), tr(B_Wv), B_Wo.reshape(HB * DB, D))
    return out.reshape(1, S, D)
```

```python
import functools

import jax
import jax.numpy as jnp
import jax.experimental.pallas as pl
import jax.experimental.pallas.tpu as pltpu

F32 = jnp.float32
BF16 = jnp.bfloat16
U32 = jnp.uint32

S = 2048
D = 640
HA = 32
DA = 20
HB = 32
DB = 192
NM = 8
SEG = 32
NPAIR = HB // 2
TB = 512
TC = 256
UNROLL = 2
RB = 64 * UNROLL
NXC = 8
NOC = 4
LN_EPS = 1e-5

_NN = (((1,), (0,)), ((), ()))
_NT = (((1,), (1,)), ((), ()))


def _dot(a, b):
    return jax.lax.dot_general(a, b, _NN, preferred_element_type=F32)


def _dot_nt(a, b):
    return jax.lax.dot_general(a, b, _NT, preferred_element_type=F32)


def _ln(x):
    m = jnp.mean(x, axis=-1, keepdims=True)
    xc = x - m
    v = jnp.mean(xc * xc, axis=-1, keepdims=True)
    return xc * jax.lax.rsqrt(v + LN_EPS)


def _iota(shape, dim):
    return jax.lax.broadcasted_iota(jnp.int32, shape, dim)


def _div20(i):
    return (i * 3277) >> 16


def _div40(i):
    return _div20(i) >> 1


def _kernel(x_hbm, wqkv_hbm, wphi_hbm, wo_hbm, mem0_hbm, wqt_hbm, wkt_hbm, wvt_hbm, bwo_hbm,
            out_hbm,
            wphi_ref, mem0_ref, xin, wqkv, woa, wt, wb, bwo, xres, xn32, xnb, wat, kvacc, phiq, obuf,
            memv, snext, sdef, opend, sems, xsems, osems):
    XC = S // NXC
    cp_phi = pltpu.make_async_copy(wphi_hbm, wphi_ref, sems.at[0])
    cp_wqkv = pltpu.make_async_copy(wqkv_hbm, wqkv, sems.at[1])

    def cp_x(c):
        rows = pl.ds(pl.multiple_of(c * XC, XC), XC)
        return pltpu.make_async_copy(x_hbm.at[rows], xin.at[rows], xsems.at[c])

    cp_wo = pltpu.make_async_copy(wo_hbm, woa, sems.at[2])
    cp_mem = pltpu.make_async_copy(mem0_hbm, mem0_ref, sems.at[3])
    cp_big = [
        pltpu.make_async_copy(wqt_hbm, wt.at[0], sems.at[4]),
        pltpu.make_async_copy(wkt_hbm, wt.at[1], sems.at[5]),
        pltpu.make_async_copy(wvt_hbm, wt.at[2], sems.at[6]),
    ]
    OC = HB * DB // NOC

    def cp_bwo(c):
        rows = pl.ds(pl.multiple_of(c * OC, OC), OC)
        return pltpu.make_async_copy(bwo_hbm.at[rows], wt.at[3, rows], osems.at[c])

    def start_first(c, carry):
        @pl.when(c == 0)
        def _():
            cp_phi.start()

        @pl.when(c == 1)
        def _():
            cp_wqkv.start()

        @pl.when(c >= 2)
        def _():
            cp_x(c - 2).start()

        return carry

    jax.lax.fori_loop(0, NXC + 2, start_first, 0)
    cp_phi.wait()

    wphi = wphi_ref[...].astype(F32)
    xw = jnp.concatenate([wphi[d] for d in range(DA)], axis=1)
    xw = jnp.concatenate([xw, jnp.zeros((32 - DA, D), F32)], axis=0).astype(BF16)
    r = _iota((D, D), 0)
    c = _iota((D, D), 1)
    perm = jnp.where((r & 31) * DA + (r >> 5) == c, 1.0, 0.0).astype(BF16)
    wf = _dot(xw, perm).astype(BF16)
    r = _iota((160, 32), 0)
    c = _iota((160, 32), 1)
    rsel = jnp.where(((r - _div40(r) * 40) >> 1) == c, 1.0, 0.0).astype(BF16)
    r = _iota((160, 128), 0)
    c = _iota((160, 128), 1)
    phit = []
    for t in range(5):
        keep = 2 * (_div40(r) + 3 * t) + (r & 1) == _div20(c + 128 * t)
        phit.append(jnp.where(keep, _dot(rsel, wf[:, 128 * t:128 * (t + 1)]), 0.0).astype(BF16))

    cp_wqkv.wait()
    cp_big[0].start()
    for m, dst in ((1, 0), (0, 1)):
        p = [_dot_nt(phit[t], wqkv[:, m * D + 128 * t:m * D + 128 * (t + 1)]) for t in range(5)]
        rows = [p[0][0:120]]
        for t in range(1, 5):
            rows += [p[t - 1][120:160] + p[t][0:40], p[t][40:120]]
        rows.append(p[4][120:160])
        wat[dst] = pltpu.bitcast(jnp.concatenate(rows, axis=0).astype(BF16), U32)
    wat[2] = pltpu.bitcast(wqkv[:, 2 * D:3 * D].T, U32)

    def init_blk(i, carry):
        cp_x(i).wait()
        for u in range(XC // 64):
            off = pl.multiple_of(i * XC + u * 64, 64)
            x = xin[pl.ds(off, 64), :].astype(F32)
            xres[pl.ds(off, 64), :] = x
            xnb[pl.ds(pl.multiple_of(off // 2, 32), 32), :] = pltpu.bitcast(_ln(x).astype(BF16), U32)
        return carry

    jax.lax.fori_loop(0, NXC, init_blk, 0)
    cp_big[1].start()

    def transpose_tiles(src, dst, j0, n):
        for j in range(n):
            for t in range(3):
                off = (j0 + j) * 384 + t * 128
                if not isinstance(off, int):
                    off = pl.multiple_of(off, 128)
                wb[9 * (j0 + j) + 3 * dst + t] = pltpu.bitcast(wt[src, pl.ds(off, 128), :].T, U32)

    def layer_a(l):
        kvacc[...] = jnp.zeros_like(kvacc)

        def sub_all(x, op):
            x = op(x, pltpu.roll(x, 2, 0))
            return op(x, pltpu.roll(x, 4, 0))

        def phi(p):
            ts = [p[8 * t:8 * (t + 1)] for t in range(5)]
            mx = sub_all(functools.reduce(jnp.maximum, ts), jnp.maximum)
            mn = sub_all(functools.reduce(jnp.minimum, ts), jnp.minimum)
            ep = [jnp.exp(t - mx) for t in ts]
            en = [jnp.exp(mn - t) for t in ts]
            rp = 1.0 / sub_all(functools.reduce(jnp.add, ep), jnp.add)
            rn = 1.0 / sub_all(functools.reduce(jnp.add, en), jnp.add)
            return jnp.concatenate([e * rp for e in ep] + [e * rn for e in en], axis=0).astype(BF16)

        def phase1(i, carry):
            @pl.when(jnp.logical_and(l == 0, i == 0))
            def _():
                cp_wo.start()
                cp_mem.start()

            @pl.when(jnp.logical_and(l == 0, i == 1))
            def _():
                cp_big[2].start()

            @pl.when(jnp.logical_and(l == 0, i == 2))
            def _():
                for c in range(NOC):
                    cp_bwo(c).start()
                cp_big[0].wait()

            @pl.when(jnp.logical_and(l == 0, i == 3))
            def _():
                cp_big[1].wait()

            transpose_tiles(jnp.where(i < 2, 3, i - 2), jnp.where(i < 2, 2, i - 2), 0, NPAIR)
            off = pl.multiple_of(i * TB, TB)
            xn = pltpu.bitcast(xnb[pl.ds(pl.multiple_of(i * (TB // 2), TB // 2), TB // 2), :], BF16)
            pk = _dot_nt(pltpu.bitcast(wat[0], BF16), xn)
            phik = [phi(pk[40 * j:40 * (j + 1)]) for j in range(16)]
            pq = _dot_nt(pltpu.bitcast(wat[1], BF16), xn)
            for j in range(16):
                phiq[j, :, pl.ds(off, TB)] = pltpu.bitcast(phi(pq[40 * j:40 * (j + 1)]), U32)
            hb = TB // 2
            vt = [_dot_nt(pltpu.bitcast(wat[2], BF16), xn[hb * u:hb * (u + 1)]) for u in range(2)]
            ones = jnp.ones((8, hb), F32)
            for u in range(2):
                for j in range(16):
                    lhs = jnp.concatenate([vt[u][40 * j:40 * (j + 1)], ones], axis=0).astype(BF16)
                    kvacc[j] = _dot_nt(lhs, phik[j][:, hb * u:hb * (u + 1)]) + kvacc[j]
            return carry

        jax.lax.fori_loop(0, S // TB, phase1, 0)

        rr = _iota((48, 80), 0)
        cc = _iota((48, 80), 1)
        keep = jnp.where(rr < 40, _div20(rr), (rr - 40) >> 2) == (cc & 1)
        kvm = [jnp.where(keep, kvacc[j], 0.0).astype(BF16) for j in range(16)]
        lo4 = _iota((8, TC), 0) < 4

        def num(b):
            parts = []
            for j in range(16):
                r = _dot(kvm[j], pltpu.bitcast(phiq[j, :, TC * b:TC * (b + 1)], BF16))
                rc = 1.0 / (r[40:48] + 1e-6)
                rc2 = pltpu.roll(rc, 4, 0)
                ra = jnp.where(lo4, rc, rc2)
                rb = jnp.where(lo4, rc2, rc)
                parts += [r[0:8] * ra, r[8:16] * ra, r[16:24] * rc, r[24:32] * rb, r[32:40] * rb]
            return jnp.concatenate(parts, axis=0).astype(BF16).T

        for b in range(S // TC):
            obuf[TC // 2 * b:TC // 2 * (b + 1), :] = pltpu.bitcast(num(b), U32)

        @pl.when(l == 0)
        def _():
            cp_wo.wait()
            cp_mem.wait()
            cp_big[2].wait()

        def out(i, carry):
            transpose_tiles(2, 2, i * (NPAIR // 4), NPAIR // 4)
            xn32[0:RB, :] = _ln(xres[0:RB, :])
            rows = pl.ds(pl.multiple_of(i * TB, TB), TB)
            o = pltpu.bitcast(obuf[pl.ds(pl.multiple_of(i * (TB // 2), TB // 2), TB // 2), :], BF16)
            xres[rows, :] = _dot(o, woa[...]) + xres[rows, :]
            return carry

        jax.lax.fori_loop(0, S // TB, out, 0)

        @pl.when(l == 0)
        def _():
            def cpo(c, carry):
                cp_bwo(c).wait()
                for u in range(OC // 384):
                    off = pl.multiple_of(c * OC + u * 384, 384)
                    bwo[pl.ds(pl.multiple_of(off // 2, 192), 192), :] = pltpu.bitcast(
                        wt[3, pl.ds(off, 384), :], U32)
                return carry

            jax.lax.fori_loop(0, NOC, cpo, 0)

    scale = DB ** (-0.5)

    def layer_b(layer):
        L = SEG + NM
        NEG = -1000000000.0

        def masks(even):
            nrow = SEG if even else L + 8
            rr = _iota((nrow, 128), 0)
            cc = _iota((nrow, 128), 1)
            is_a = (cc < L) | ((cc >= 2 * L) & (cc < 2 * L + 16))
            kx = jnp.where(cc < L, cc, cc - (L + NM))
            is_memkey = (cc >= SEG) & (cc < SEG + 2 * NM)
            if even:
                valid = cc < 2 * L
                allowed = valid & (is_memkey | (rr >= 24) | (kx <= rr + 8))
            else:
                dk = (cc - 2 * L) & 15
                cur = (rr < L) & (cc < 2 * L)
                old = (rr >= L) & (cc >= 2 * L) & (cc < 2 * L + 32)
                valid = cur | old
                allowed = ((cur & (is_memkey | (rr >= SEG) | (kx <= rr)))
                           | (old & ((dk >= 8) | (dk <= rr - L))))
            return is_a, allowed, jnp.where(valid, NEG, -jnp.inf).astype(F32)

        all_masks = {True: masks(True), False: masks(False)}

        def lo64(y):
            return _iota(y.shape, 1) < 64

        def stack_keys(a, b):
            parts = [a[0:L], b[SEG:L], b[0:SEG]]
            if a.shape[0] > L:
                parts += [a[L:], b[L:]]
            return jnp.concatenate(parts, axis=0).astype(BF16)

        def expand(y):
            y0, y1, y2 = y[:, 0:128], y[:, 128:256], y[:, 256:384]
            return (stack_keys(y0, y2),
                    stack_keys(jnp.where(lo64(y1), y1, 0.0), jnp.where(lo64(y1), 0.0, y1)))

        def pad_lanes(s):
            return jnp.concatenate([s, jnp.zeros((s.shape[0], 128 - s.shape[1]), F32)], axis=1)

        def step(h, even, kmajor):
            is_a, allowed, fill = all_masks[even]
            nrow = SEG if even else L + 8
            nkey = 2 * L if even else 2 * L + 32

            def proj(j):
                w = jnp.concatenate(
                    [pltpu.bitcast(wb[9 * j + t], BF16) for t in range(9)], axis=1)
                if j == 0 and kmajor:
                    y = _dot(h[:, 0:128], w[0:128])
                    for t in range(1, 5):
                        y = _dot(h[:, 128 * t:128 * (t + 1)], w[128 * t:128 * (t + 1)]) + y
                else:
                    y = _dot(h, w)
                if even:
                    snext[j] = y[SEG:L]
                    sdef[j, 0:8, :] = y[0:8]
                    sdef[j, 8:16, 384:1152] = y[L:L + 8, 384:1152]
                    q = jnp.concatenate([y[8:SEG, 0:384], y[L:L + 8, 0:384]], axis=0)
                    kv = jnp.concatenate([y[0:SEG, 384:1152], y[L:L + 8, 384:1152]], axis=0)
                else:
                    q = jnp.concatenate(
                        [snext[j, :, 0:384], y[:, 0:384], sdef[j, 0:8, 0:384]], axis=0)
                    kv = jnp.concatenate(
                        [snext[j, :, 384:1152], y[:, 384:1152], sdef[j, :, 384:1152]], axis=0)
                q = q.astype(BF16)
                q = (jnp.concatenate([q[:, 0:128], q[:, 256:384]], axis=0), q[:, 128:256])
                return q, expand(kv[:, 0:384]), expand(kv[:, 384:768])

            def scores(q, k):
                s02 = pad_lanes(_dot_nt(q[0], k[0]))
                s = jnp.where(is_a, s02[0:nrow], s02[nrow:]) + pad_lanes(_dot_nt(q[1], k[1]))
                s = jnp.where(allowed, s * scale, fill)
                ma = jnp.max(jnp.where(is_a, s, -jnp.inf), axis=1, keepdims=True)
                mb = jnp.max(jnp.where(is_a, -jnp.inf, s), axis=1, keepdims=True)
                e = jnp.exp(s - jnp.where(is_a, ma, mb))
                ea = jnp.where(is_a, e, 0.0)
                eb = jnp.where(is_a, 0.0, e)
                pa = ea * (1.0 / jnp.sum(ea, axis=1, keepdims=True))
                pb = eb * (1.0 / jnp.sum(eb, axis=1, keepdims=True))
                return (jnp.concatenate([pa, pb], axis=0)[:, 0:nkey].astype(BF16),
                        (pa + pb)[:, 0:nkey].astype(BF16))

            def pv(p, v):
                o02 = _dot(p[0], v[0])
                return jnp.concatenate(
                    [o02[0:nrow], _dot(p[1], v[1]), o02[nrow:]], axis=1).astype(BF16)

            qkv = [None] * NPAIR
            ps = [None] * NPAIR
            os_ = [None] * NPAIR

            def wo_chunk(c0, c1):
                w = pltpu.bitcast(bwo[192 * c0:192 * c1, :], BF16)
                return _dot(jnp.concatenate(os_[c0:c1], axis=1), w)

            lag = NPAIR if even else 4
            cuts = (0, 4, 8, 11, 14, 16) if even else (11, 12, 13, 14, 15, 16)
            qkv[0] = proj(0)
            acc = None
            for j in range(NPAIR + 2):
                c = None
                if j + 1 < NPAIR:
                    qkv[j + 1] = proj(j + 1)
                    if j >= lag:
                        c = wo_chunk(j - lag, j - lag + 1)
                else:
                    c = wo_chunk(cuts[j + 1 - NPAIR], cuts[j + 2 - NPAIR])
                if c is not None:
                    acc = c if acc is None else c + acc
                if j < NPAIR:
                    ps[j] = scores(qkv[j][0], qkv[j][1])
                if j >= 2:
                    os_[j - 2] = pv(ps[j - 2], qkv[j - 2][2])
            acc = wo_chunk(cuts[3], cuts[4]) + acc
            return wo_chunk(cuts[4], cuts[5]) + acc

        def finish_rows(base):
            xnew = xres[pl.ds(base, RB), :] + opend[...]
            xres[pl.ds(base, RB), :] = xnew
            xnb[pl.ds(pl.multiple_of(base // 2, RB // 2), RB // 2), :] = pltpu.bitcast(
                _ln(xnew).astype(BF16), U32)
            xin[pl.ds(base, RB), :] = xnew.astype(BF16)

        memv[...] = mem0_ref[...].astype(F32)
        opend[...] = jnp.zeros_like(opend)

        def body(i, carry):
            base = pl.multiple_of(i * RB, RB)

            @pl.when(jnp.logical_and(layer == 1, i >= 2))
            def _():
                rows = pl.ds(pl.multiple_of((i - 2) * RB, RB), RB)
                pltpu.make_async_copy(xin.at[rows], out_hbm.at[rows], sems.at[0]).start()

            finish_rows(pl.multiple_of(jnp.maximum(i - 1, 0) * RB, RB))
            mem = memv[...]
            for u in range(UNROLL):
                r0 = 64 * u
                h0 = jnp.concatenate([xn32[pl.ds(base + r0, 40), :], mem], axis=0).astype(BF16)
                o0 = step(h0, True, u > 0)
                opend[r0 + 8:r0 + 32, :] = o0[0:24]
                h1 = jnp.concatenate(
                    [xn32[pl.ds(base + r0 + 40, 24), :], o0[24:32]], axis=0).astype(BF16)
                o1 = step(h1, False, True)
                mem = o1[32:40]
                opend[r0:r0 + 8, :] = o1[40:48]
                opend[r0 + 32:r0 + 64, :] = o1[0:32]
            memv[...] = mem
            nxt = pl.ds(pl.multiple_of(jnp.minimum(i + 1, S // RB - 1) * RB, RB), RB)
            xn32[nxt, :] = _ln(xres[nxt, :])
            return carry

        jax.lax.fori_loop(0, S // RB, body, 0)
        finish_rows(S - RB)

    def layer(l, carry):
        layer_a(l)
        layer_b(l)
        return carry

    jax.lax.fori_loop(0, 2, layer, 0)

    last = pl.ds(S - 128 * UNROLL, 128 * UNROLL)
    pltpu.make_async_copy(xin.at[last], out_hbm.at[last], sems.at[0]).start()
    pltpu.make_async_copy(xin, out_hbm, sems.at[0]).wait()


@functools.partial(jax.jit, static_argnames=("B_seg_len",))
def pallas_interleave_layers__linear_kernel_hedgehog__memory_aug_recurrent_mem_tr__prompt_kernel(
    A_x: jax.Array,
    A_wqkv: jax.Array,
    A_w_phi: jax.Array,
    A_wo: jax.Array,
    B_x: jax.Array,
    B_mem0: jax.Array,
    B_Wq: jax.Array,
    B_Wk: jax.Array,
    B_Wv: jax.Array,
    B_Wo: jax.Array,
    B_seg_len=SEG,
):
    assert B_seg_len == SEG and A_x.shape == (1, S, D)
    tr = lambda w: jnp.transpose(w, (1, 2, 0)).reshape(HB * DB, D)
    any_spec = pl.BlockSpec(memory_space=pl.ANY)
    out = pl.pallas_call(
        _kernel,
        out_shape=jax.ShapeDtypeStruct((S, D), BF16),
        in_specs=[any_spec] * 9,
        out_specs=any_spec,
        scratch_shapes=[
            pltpu.VMEM((DA, DA, HA), BF16),
            pltpu.VMEM((NM, D), BF16),
            pltpu.VMEM((S, D), BF16),
            pltpu.VMEM((D, 3 * D), BF16),
            pltpu.VMEM((D, D), BF16),
            pltpu.VMEM((4, HB * DB, D), BF16),
            pltpu.VMEM((9 * NPAIR, D // 2, 128), U32),
            pltpu.VMEM((HB * DB // 2, D), U32),
            pltpu.VMEM((S, D), F32),
            pltpu.VMEM((S, D), F32),
            pltpu.VMEM((S // 2, D), U32),
            pltpu.VMEM((3, D // 2, D), U32),
            pltpu.VMEM((16, 48, 80), F32),
            pltpu.VMEM((16, 40, S), U32),
            pltpu.VMEM((S // 2, D), U32),
            pltpu.VMEM((NM, D), F32),
            pltpu.VMEM((NPAIR, 8, 9 * 128), F32),
            pltpu.VMEM((NPAIR, 16, 9 * 128), F32),
            pltpu.VMEM((64 * UNROLL, D), F32),
            pltpu.SemaphoreType.DMA((7,)),
            pltpu.SemaphoreType.DMA((NXC,)),
            pltpu.SemaphoreType.DMA((NOC,)),
        ],
        compiler_params=pltpu.CompilerParams(vmem_limit_bytes=120 * 1024 * 1024),
    )(A_x.reshape(S, D), A_wqkv, jnp.transpose(A_w_phi, (1, 2, 0)), A_wo,
      B_mem0.reshape(NM, D), tr(B_Wq), tr(B_Wk), tr(B_Wv), B_Wo.reshape(HB * DB, D))
    return out.reshape(1, S, D)
```

```python
import functools

import jax
import jax.numpy as jnp
import jax.experimental.pallas as pl
import jax.experimental.pallas.tpu as pltpu

F32 = jnp.float32
BF16 = jnp.bfloat16
U32 = jnp.uint32

S = 2048
D = 640
HA = 32
DA = 20
HB = 32
DB = 192
NM = 8
SEG = 32
NPAIR = HB // 2
TB = 512
TC = 256
UNROLL = 2
RB = 64 * UNROLL
NXC = 8
NOC = 4
LN_EPS = 1e-5

_NN = (((1,), (0,)), ((), ()))
_NT = (((1,), (1,)), ((), ()))


def _dot(a, b):
    return jax.lax.dot_general(a, b, _NN, preferred_element_type=F32)


def _dot_nt(a, b):
    return jax.lax.dot_general(a, b, _NT, preferred_element_type=F32)


def _ln(x):
    m = jnp.mean(x, axis=-1, keepdims=True)
    xc = x - m
    v = jnp.mean(xc * xc, axis=-1, keepdims=True)
    return xc * jax.lax.rsqrt(v + LN_EPS)


def _iota(shape, dim):
    return jax.lax.broadcasted_iota(jnp.int32, shape, dim)


def _div20(i):
    return (i * 3277) >> 16


def _div40(i):
    return _div20(i) >> 1


def _kernel(x_hbm, wqkv_hbm, wphi_hbm, wo_hbm, mem0_hbm, wqt_hbm, wkt_hbm, wvt_hbm, bwo_hbm,
            out_hbm,
            wphi_ref, mem0_ref, xin, wqkv, woa, wt, wb, bwo, xres, xn32, xnb, wat, kvacc, phiq, obuf,
            memv, snext, sdef, opend, sems, xsems, osems):
    XC = S // NXC
    cp_phi = pltpu.make_async_copy(wphi_hbm, wphi_ref, sems.at[0])
    cp_wqkv = pltpu.make_async_copy(wqkv_hbm, wqkv, sems.at[1])

    def cp_x(c):
        rows = pl.ds(pl.multiple_of(c * XC, XC), XC)
        return pltpu.make_async_copy(x_hbm.at[rows], xin.at[rows], xsems.at[c])

    cp_wo = pltpu.make_async_copy(wo_hbm, woa, sems.at[2])
    cp_mem = pltpu.make_async_copy(mem0_hbm, mem0_ref, sems.at[3])
    cp_big = [
        pltpu.make_async_copy(wqt_hbm, wt.at[0], sems.at[4]),
        pltpu.make_async_copy(wkt_hbm, wt.at[1], sems.at[5]),
        pltpu.make_async_copy(wvt_hbm, wt.at[2], sems.at[6]),
    ]
    OC = HB * DB // NOC

    def cp_bwo(c):
        rows = pl.ds(pl.multiple_of(c * OC, OC), OC)
        return pltpu.make_async_copy(bwo_hbm.at[rows], wt.at[3, rows], osems.at[c])

    def start_first(c, carry):
        @pl.when(c == 0)
        def _():
            cp_phi.start()

        @pl.when(c == 1)
        def _():
            cp_wqkv.start()

        @pl.when(c >= 2)
        def _():
            cp_x(c - 2).start()

        return carry

    jax.lax.fori_loop(0, NXC + 2, start_first, 0)
    cp_phi.wait()

    wphi = wphi_ref[...].astype(F32)
    xw = jnp.concatenate([wphi[d] for d in range(DA)], axis=1)
    xw = jnp.concatenate([xw, jnp.zeros((32 - DA, D), F32)], axis=0).astype(BF16)
    r = _iota((D, D), 0)
    c = _iota((D, D), 1)
    perm = jnp.where((r & 31) * DA + (r >> 5) == c, 1.0, 0.0).astype(BF16)
    wf = _dot(xw, perm).astype(BF16)
    r = _iota((160, 32), 0)
    c = _iota((160, 32), 1)
    rsel = jnp.where(((r - _div40(r) * 40) >> 1) == c, 1.0, 0.0).astype(BF16)
    r = _iota((160, 128), 0)
    c = _iota((160, 128), 1)
    phit = []
    for t in range(5):
        keep = 2 * (_div40(r) + 3 * t) + (r & 1) == _div20(c + 128 * t)
        phit.append(jnp.where(keep, _dot(rsel, wf[:, 128 * t:128 * (t + 1)]), 0.0).astype(BF16))

    kvacc[...] = jnp.zeros_like(kvacc)
    cp_wqkv.wait()
    cp_big[0].start()
    for m, dst in ((1, 0), (0, 1)):
        p = [_dot_nt(phit[t], wqkv[:, m * D + 128 * t:m * D + 128 * (t + 1)]) for t in range(5)]
        rows = [p[0][0:120]]
        for t in range(1, 5):
            rows += [p[t - 1][120:160] + p[t][0:40], p[t][40:120]]
        rows.append(p[4][120:160])
        wat[dst] = pltpu.bitcast(jnp.concatenate(rows, axis=0).astype(BF16), U32)
    wat[2] = pltpu.bitcast(wqkv[:, 2 * D:3 * D].T, U32)

    def init_blk(i, carry):
        cp_x(i).wait()
        for u in range(XC // 64):
            off = pl.multiple_of(i * XC + u * 64, 64)
            x = xin[pl.ds(off, 64), :].astype(F32)
            xres[pl.ds(off, 64), :] = x
            xnb[pl.ds(pl.multiple_of(off // 2, 32), 32), :] = pltpu.bitcast(_ln(x).astype(BF16), U32)
        return carry

    jax.lax.fori_loop(0, NXC, init_blk, 0)
    cp_big[1].start()

    def transpose_tiles(src, dst, j0, n):
        for j in range(n):
            for t in range(3):
                off = (j0 + j) * 384 + t * 128
                if not isinstance(off, int):
                    off = pl.multiple_of(off, 128)
                wb[9 * (j0 + j) + 3 * dst + t] = pltpu.bitcast(wt[src, pl.ds(off, 128), :].T, U32)

    def layer_a(l):
        def sub_all(x, op):
            x = op(x, pltpu.roll(x, 2, 0))
            return op(x, pltpu.roll(x, 4, 0))

        def phi(p):
            ts = [p[8 * t:8 * (t + 1)] for t in range(5)]
            mx = sub_all(functools.reduce(jnp.maximum, ts), jnp.maximum)
            mn = sub_all(functools.reduce(jnp.minimum, ts), jnp.minimum)
            ep = [jnp.exp(t - mx) for t in ts]
            en = [jnp.exp(mn - t) for t in ts]
            rp = 1.0 / sub_all(functools.reduce(jnp.add, ep), jnp.add)
            rn = 1.0 / sub_all(functools.reduce(jnp.add, en), jnp.add)
            return jnp.concatenate([e * rp for e in ep] + [e * rn for e in en], axis=0).astype(BF16)

        def phase1(i, carry):
            @pl.when(jnp.logical_and(l == 0, i == 0))
            def _():
                cp_wo.start()
                cp_mem.start()

            @pl.when(jnp.logical_and(l == 0, i == 1))
            def _():
                cp_big[2].start()

            @pl.when(jnp.logical_and(l == 0, i == 2))
            def _():
                for c in range(NOC):
                    cp_bwo(c).start()
                cp_big[0].wait()

            @pl.when(jnp.logical_and(l == 0, i == 3))
            def _():
                cp_big[1].wait()

            transpose_tiles(jnp.where(i < 2, 3, i - 2), jnp.where(i < 2, 2, i - 2), 0, NPAIR)
            off = pl.multiple_of(i * TB, TB)
            xn = pltpu.bitcast(xnb[pl.ds(pl.multiple_of(i * (TB // 2), TB // 2), TB // 2), :], BF16)
            pk = _dot_nt(pltpu.bitcast(wat[0], BF16), xn)
            phik = [phi(pk[40 * j:40 * (j + 1)]) for j in range(16)]
            pq = _dot_nt(pltpu.bitcast(wat[1], BF16), xn)
            for j in range(16):
                phiq[j, :, pl.ds(off, TB)] = pltpu.bitcast(phi(pq[40 * j:40 * (j + 1)]), U32)
            hb = TB // 2
            vt = [_dot_nt(pltpu.bitcast(wat[2], BF16), xn[hb * u:hb * (u + 1)]) for u in range(2)]
            ones = jnp.ones((8, hb), F32)
            for u in range(2):
                for j in range(16):
                    lhs = jnp.concatenate([vt[u][40 * j:40 * (j + 1)], ones], axis=0).astype(BF16)
                    kvacc[j] = _dot_nt(lhs, phik[j][:, hb * u:hb * (u + 1)]) + kvacc[j]
            return carry

        jax.lax.fori_loop(0, S // TB, phase1, 0)

        rr = _iota((48, 80), 0)
        cc = _iota((48, 80), 1)
        keep = jnp.where(rr < 40, _div20(rr), (rr - 40) >> 2) == (cc & 1)
        kvm = [jnp.where(keep, kvacc[j], 0.0).astype(BF16) for j in range(16)]
        lo4 = _iota((8, TC), 0) < 4

        def num(b):
            parts = []
            for j in range(16):
                r = _dot(kvm[j], pltpu.bitcast(phiq[j, :, TC * b:TC * (b + 1)], BF16))
                rc = 1.0 / (r[40:48] + 1e-6)
                rc2 = pltpu.roll(rc, 4, 0)
                ra = jnp.where(lo4, rc, rc2)
                rb = jnp.where(lo4, rc2, rc)
                parts += [r[0:8] * ra, r[8:16] * ra, r[16:24] * rc, r[24:32] * rb, r[32:40] * rb]
            return jnp.concatenate(parts, axis=0).astype(BF16).T

        for b in range(S // TC):
            obuf[TC // 2 * b:TC // 2 * (b + 1), :] = pltpu.bitcast(num(b), U32)

        @pl.when(l == 0)
        def _():
            cp_wo.wait()
            cp_mem.wait()
            cp_big[2].wait()

        def out(i, carry):
            transpose_tiles(2, 2, i * (NPAIR // 4), NPAIR // 4)
            xn32[0:RB, :] = _ln(xres[0:RB, :])
            memv[...] = mem0_ref[...].astype(F32)
            opend[...] = jnp.zeros_like(opend)
            kvacc[...] = jnp.zeros_like(kvacc)
            rows = pl.ds(pl.multiple_of(i * TB, TB), TB)
            o = pltpu.bitcast(obuf[pl.ds(pl.multiple_of(i * (TB // 2), TB // 2), TB // 2), :], BF16)
            xres[rows, :] = _dot(o, woa[...]) + xres[rows, :]
            return carry

        jax.lax.fori_loop(0, S // TB, out, 0)

        @pl.when(l == 0)
        def _():
            def cpo(c, carry):
                cp_bwo(c).wait()
                for u in range(OC // 384):
                    off = pl.multiple_of(c * OC + u * 384, 384)
                    bwo[pl.ds(pl.multiple_of(off // 2, 192), 192), :] = pltpu.bitcast(
                        wt[3, pl.ds(off, 384), :], U32)
                return carry

            jax.lax.fori_loop(0, NOC, cpo, 0)

    scale = DB ** (-0.5)

    def layer_b(layer):
        L = SEG + NM
        NEG = -1000000000.0

        def masks(even):
            nrow = SEG if even else L + 8
            rr = _iota((nrow, 128), 0)
            cc = _iota((nrow, 128), 1)
            is_a = (cc < L) | ((cc >= 2 * L) & (cc < 2 * L + 16))
            kx = jnp.where(cc < L, cc, cc - (L + NM))
            is_memkey = (cc >= SEG) & (cc < SEG + 2 * NM)
            if even:
                valid = cc < 2 * L
                allowed = valid & (is_memkey | (rr >= 24) | (kx <= rr + 8))
            else:
                dk = (cc - 2 * L) & 15
                cur = (rr < L) & (cc < 2 * L)
                old = (rr >= L) & (cc >= 2 * L) & (cc < 2 * L + 32)
                valid = cur | old
                allowed = ((cur & (is_memkey | (rr >= SEG) | (kx <= rr)))
                           | (old & ((dk >= 8) | (dk <= rr - L))))
            return is_a, allowed, jnp.where(valid, NEG, -jnp.inf).astype(F32)

        all_masks = {True: masks(True), False: masks(False)}

        def lo64(y):
            return _iota(y.shape, 1) < 64

        def stack_keys(a, b):
            parts = [a[0:L], b[SEG:L], b[0:SEG]]
            if a.shape[0] > L:
                parts += [a[L:], b[L:]]
            return jnp.concatenate(parts, axis=0).astype(BF16)

        def expand(y):
            y0, y1, y2 = y[:, 0:128], y[:, 128:256], y[:, 256:384]
            return (stack_keys(y0, y2),
                    stack_keys(jnp.where(lo64(y1), y1, 0.0), jnp.where(lo64(y1), 0.0, y1)))

        def pad_lanes(s):
            return jnp.concatenate([s, jnp.zeros((s.shape[0], 128 - s.shape[1]), F32)], axis=1)

        def step(h, even, kmajor):
            is_a, allowed, fill = all_masks[even]
            nrow = SEG if even else L + 8
            nkey = 2 * L if even else 2 * L + 32

            def proj(j):
                w = jnp.concatenate(
                    [pltpu.bitcast(wb[9 * j + t], BF16) for t in range(9)], axis=1)
                if j == 0 and kmajor:
                    y = _dot(h[:, 0:128], w[0:128])
                    for t in range(1, 5):
                        y = _dot(h[:, 128 * t:128 * (t + 1)], w[128 * t:128 * (t + 1)]) + y
                else:
                    y = _dot(h, w)
                if even:
                    snext[j] = y[SEG:L]
                    sdef[j, 0:8, :] = y[0:8]
                    sdef[j, 8:16, 384:1152] = y[L:L + 8, 384:1152]
                    q = jnp.concatenate([y[8:SEG, 0:384], y[L:L + 8, 0:384]], axis=0)
                    kv = jnp.concatenate([y[0:SEG, 384:1152], y[L:L + 8, 384:1152]], axis=0)
                else:
                    q = jnp.concatenate(
                        [snext[j, :, 0:384], y[:, 0:384], sdef[j, 0:8, 0:384]], axis=0)
                    kv = jnp.concatenate(
                        [snext[j, :, 384:1152], y[:, 384:1152], sdef[j, :, 384:1152]], axis=0)
                q = q.astype(BF16)
                q = (jnp.concatenate([q[:, 0:128], q[:, 256:384]], axis=0), q[:, 128:256])
                return q, expand(kv[:, 0:384]), expand(kv[:, 384:768])

            def scores(q, k):
                s02 = pad_lanes(_dot_nt(q[0], k[0]))
                s = jnp.where(is_a, s02[0:nrow], s02[nrow:]) + pad_lanes(_dot_nt(q[1], k[1]))
                s = jnp.where(allowed, s * scale, fill)
                ma = jnp.max(jnp.where(is_a, s, -jnp.inf), axis=1, keepdims=True)
                mb = jnp.max(jnp.where(is_a, -jnp.inf, s), axis=1, keepdims=True)
                e = jnp.exp(s - jnp.where(is_a, ma, mb))
                ea = jnp.where(is_a, e, 0.0)
                eb = jnp.where(is_a, 0.0, e)
                pa = ea * (1.0 / jnp.sum(ea, axis=1, keepdims=True))
                pb = eb * (1.0 / jnp.sum(eb, axis=1, keepdims=True))
                return (jnp.concatenate([pa, pb], axis=0)[:, 0:nkey].astype(BF16),
                        (pa + pb)[:, 0:nkey].astype(BF16))

            def pv(p, v):
                o02 = _dot(p[0], v[0])
                return jnp.concatenate(
                    [o02[0:nrow], _dot(p[1], v[1]), o02[nrow:]], axis=1).astype(BF16)

            qkv = [None] * NPAIR
            ps = [None] * NPAIR
            os_ = [None] * NPAIR

            def wo_chunk(c0, c1):
                w = pltpu.bitcast(bwo[192 * c0:192 * c1, :], BF16)
                return _dot(jnp.concatenate(os_[c0:c1], axis=1), w)

            lag = NPAIR if even else 4
            cuts = (0, 4, 8, 11, 14, 16) if even else (11, 12, 13, 14, 15, 16)
            qkv[0] = proj(0)
            acc = None
            for j in range(NPAIR + 2):
                c = None
                if j + 1 < NPAIR:
                    qkv[j + 1] = proj(j + 1)
                    if j >= lag:
                        c = wo_chunk(j - lag, j - lag + 1)
                else:
                    c = wo_chunk(cuts[j + 1 - NPAIR], cuts[j + 2 - NPAIR])
                if c is not None:
                    acc = c if acc is None else c + acc
                if j < NPAIR:
                    ps[j] = scores(qkv[j][0], qkv[j][1])
                if j >= 2:
                    os_[j - 2] = pv(ps[j - 2], qkv[j - 2][2])
            acc = wo_chunk(cuts[3], cuts[4]) + acc
            return wo_chunk(cuts[4], cuts[5]) + acc

        def finish_rows(base):
            xnew = xres[pl.ds(base, RB), :] + opend[...]
            xres[pl.ds(base, RB), :] = xnew
            xnb[pl.ds(pl.multiple_of(base // 2, RB // 2), RB // 2), :] = pltpu.bitcast(
                _ln(xnew).astype(BF16), U32)
            xin[pl.ds(base, RB), :] = xnew.astype(BF16)

        def body(i, carry):
            base = pl.multiple_of(i * RB, RB)

            @pl.when(jnp.logical_and(layer == 1, i >= 2))
            def _():
                rows = pl.ds(pl.multiple_of((i - 2) * RB, RB), RB)
                pltpu.make_async_copy(xin.at[rows], out_hbm.at[rows], sems.at[0]).start()

            finish_rows(pl.multiple_of(jnp.maximum(i - 1, 0) * RB, RB))
            mem = memv[...]
            for u in range(UNROLL):
                r0 = 64 * u
                h0 = jnp.concatenate([xn32[pl.ds(base + r0, 40), :], mem], axis=0).astype(BF16)
                o0 = step(h0, True, u > 0)
                opend[r0 + 8:r0 + 32, :] = o0[0:24]
                h1 = jnp.concatenate(
                    [xn32[pl.ds(base + r0 + 40, 24), :], o0[24:32]], axis=0).astype(BF16)
                o1 = step(h1, False, True)
                mem = o1[32:40]
                opend[r0:r0 + 8, :] = o1[40:48]
                opend[r0 + 32:r0 + 64, :] = o1[0:32]
            memv[...] = mem
            nxt = pl.ds(pl.multiple_of(jnp.minimum(i + 1, S // RB - 1) * RB, RB), RB)
            xn32[nxt, :] = _ln(xres[nxt, :])
            return carry

        jax.lax.fori_loop(0, S // RB, body, 0)

        @pl.when(layer == 0)
        def _():
            finish_rows(S - RB)

    def layer(l, carry):
        layer_a(l)
        layer_b(l)
        return carry

    jax.lax.fori_loop(0, 2, layer, 0)

    rows = pl.ds(S - 2 * RB, RB)
    pltpu.make_async_copy(xin.at[rows], out_hbm.at[rows], sems.at[0]).start()
    rows = pl.ds(S - RB, RB)
    xin[rows, :] = (xres[rows, :] + opend[...]).astype(BF16)
    pltpu.make_async_copy(xin.at[rows], out_hbm.at[rows], sems.at[0]).start()
    pltpu.make_async_copy(xin, out_hbm, sems.at[0]).wait()


@jax.jit
def pallas_interleave_layers__linear_kernel_hedgehog__memory_aug_recurrent_mem_tr__prompt_kernel(
    A_x: jax.Array,
    A_wqkv: jax.Array,
    A_w_phi: jax.Array,
    A_wo: jax.Array,
    B_x: jax.Array,
    B_mem0: jax.Array,
    B_Wq: jax.Array,
    B_Wk: jax.Array,
    B_Wv: jax.Array,
    B_Wo: jax.Array,
    B_seg_len: jax.Array,
):
    assert A_x.shape == (1, S, D) and B_mem0.shape == (1, NM, D) and B_Wq.shape == (D, HB, DB)
    tr = lambda w: jnp.transpose(w, (1, 2, 0)).reshape(HB * DB, D)
    any_spec = pl.BlockSpec(memory_space=pl.ANY)
    out = pl.pallas_call(
        _kernel,
        out_shape=jax.ShapeDtypeStruct((S, D), BF16),
        in_specs=[any_spec] * 9,
        out_specs=any_spec,
        scratch_shapes=[
            pltpu.VMEM((DA, DA, HA), BF16),
            pltpu.VMEM((NM, D), BF16),
            pltpu.VMEM((S, D), BF16),
            pltpu.VMEM((D, 3 * D), BF16),
            pltpu.VMEM((D, D), BF16),
            pltpu.VMEM((4, HB * DB, D), BF16),
            pltpu.VMEM((9 * NPAIR, D // 2, 128), U32),
            pltpu.VMEM((HB * DB // 2, D), U32),
            pltpu.VMEM((S, D), F32),
            pltpu.VMEM((S, D), F32),
            pltpu.VMEM((S // 2, D), U32),
            pltpu.VMEM((3, D // 2, D), U32),
            pltpu.VMEM((16, 48, 80), F32),
            pltpu.VMEM((16, 40, S), U32),
            pltpu.VMEM((S // 2, D), U32),
            pltpu.VMEM((NM, D), F32),
            pltpu.VMEM((NPAIR, 8, 9 * 128), F32),
            pltpu.VMEM((NPAIR, 16, 9 * 128), F32),
            pltpu.VMEM((64 * UNROLL, D), F32),
            pltpu.SemaphoreType.DMA((7,)),
            pltpu.SemaphoreType.DMA((NXC,)),
            pltpu.SemaphoreType.DMA((NOC,)),
        ],
        compiler_params=pltpu.CompilerParams(vmem_limit_bytes=120 * 1024 * 1024),
    )(A_x.reshape(S, D), A_wqkv, jnp.transpose(A_w_phi, (1, 2, 0)), A_wo,
      B_mem0.reshape(NM, D), tr(B_Wq), tr(B_Wk), tr(B_Wv), B_Wo.reshape(HB * DB, D))
    return out.reshape(1, S, D)
```

```python
import functools

import jax
import jax.numpy as jnp
import jax.experimental.pallas as pl
import jax.experimental.pallas.tpu as pltpu

F32 = jnp.float32
BF16 = jnp.bfloat16
U32 = jnp.uint32

S = 2048
D = 640
HA = 32
DA = 20
HB = 32
DB = 192
NM = 8
SEG = 32
NPAIR = HB // 2
TB = 512
TC = 512
UNROLL = 2
RB = 64 * UNROLL
NXC = 8
NOC = 8
LN_EPS = 1e-5

_NN = (((1,), (0,)), ((), ()))
_NT = (((1,), (1,)), ((), ()))


def _dot(a, b):
    return jax.lax.dot_general(a, b, _NN, preferred_element_type=F32)


def _dot_nt(a, b):
    return jax.lax.dot_general(a, b, _NT, preferred_element_type=F32)


def _ln(x):
    m = jnp.mean(x, axis=-1, keepdims=True)
    xc = x - m
    v = jnp.mean(xc * xc, axis=-1, keepdims=True)
    return xc * jax.lax.rsqrt(v + LN_EPS)


def _iota(shape, dim):
    return jax.lax.broadcasted_iota(jnp.int32, shape, dim)


def _div20(i):
    return (i * 3277) >> 16


def _div40(i):
    return _div20(i) >> 1


def _kernel(x_hbm, wqkv_hbm, wphi_hbm, wo_hbm, mem0_hbm, wqt_hbm, wkt_hbm, wvt_hbm, bwo_hbm,
            out_hbm,
            wphi_ref, mem0_ref, xin, wqkv, woa, wt, wb, bwo, xres, xn32, xnb, wat, kvacc, phiq, obuf,
            memv, snext, sdef, opend, sems, xsems, osems):
    XC = S // NXC
    cp_phi = pltpu.make_async_copy(wphi_hbm, wphi_ref, sems.at[0])
    cp_wqkv = pltpu.make_async_copy(wqkv_hbm, wqkv, sems.at[1])

    def cp_x(c):
        rows = pl.ds(pl.multiple_of(c * XC, XC), XC)
        return pltpu.make_async_copy(x_hbm.at[rows], xin.at[rows], xsems.at[c])

    cp_wo = pltpu.make_async_copy(wo_hbm, woa, sems.at[2])
    cp_mem = pltpu.make_async_copy(mem0_hbm, mem0_ref, sems.at[3])
    cp_big = [
        pltpu.make_async_copy(wqt_hbm, wt.at[0], sems.at[4]),
        pltpu.make_async_copy(wkt_hbm, wt.at[1], sems.at[5]),
        pltpu.make_async_copy(wvt_hbm, wt.at[2], sems.at[6]),
    ]
    OC = HB * DB // NOC

    def cp_bwo(c):
        rows = pl.ds(pl.multiple_of(c * OC, OC), OC)
        return pltpu.make_async_copy(bwo_hbm.at[rows], wt.at[3, rows], osems.at[c])

    def start_first(c, carry):
        @pl.when(c == 0)
        def _():
            cp_phi.start()

        @pl.when(c == 1)
        def _():
            cp_wqkv.start()

        @pl.when(c >= 2)
        def _():
            cp_x(c - 2).start()

        return carry

    jax.lax.fori_loop(0, NXC + 2, start_first, 0)
    cp_phi.wait()

    wphi = wphi_ref[...].astype(F32)
    xw = jnp.concatenate([wphi[d] for d in range(DA)], axis=1)
    xw = jnp.concatenate([xw, jnp.zeros((32 - DA, D), F32)], axis=0).astype(BF16)
    r = _iota((D, D), 0)
    c = _iota((D, D), 1)
    perm = jnp.where((r & 31) * DA + (r >> 5) == c, 1.0, 0.0).astype(BF16)
    wf = _dot(xw, perm).astype(BF16)
    r = _iota((160, 32), 0)
    c = _iota((160, 32), 1)
    rsel = jnp.where(((r - _div40(r) * 40) >> 1) == c, 1.0, 0.0).astype(BF16)
    r = _iota((160, 128), 0)
    c = _iota((160, 128), 1)
    phit = []
    for t in range(5):
        keep = 2 * (_div40(r) + 3 * t) + (r & 1) == _div20(c + 128 * t)
        phit.append(jnp.where(keep, _dot(rsel, wf[:, 128 * t:128 * (t + 1)]), 0.0).astype(BF16))

    kvacc[...] = jnp.zeros_like(kvacc)
    cp_wqkv.wait()
    cp_big[0].start()
    for m, dst in ((1, 0), (0, 1)):
        p = [_dot_nt(phit[t], wqkv[:, m * D + 128 * t:m * D + 128 * (t + 1)]) for t in range(5)]
        rows = [p[0][0:120]]
        for t in range(1, 5):
            rows += [p[t - 1][120:160] + p[t][0:40], p[t][40:120]]
        rows.append(p[4][120:160])
        wat[dst] = pltpu.bitcast(jnp.concatenate(rows, axis=0).astype(BF16), U32)
    wat[2] = pltpu.bitcast(wqkv[:, 2 * D:3 * D].T, U32)

    def init_blk(i, carry):
        cp_x(i).wait()
        for u in range(XC // 64):
            off = pl.multiple_of(i * XC + u * 64, 64)
            x = xin[pl.ds(off, 64), :].astype(F32)
            xres[pl.ds(off, 64), :] = x
            xnb[pl.ds(pl.multiple_of(off // 2, 32), 32), :] = pltpu.bitcast(_ln(x).astype(BF16), U32)
        return carry

    jax.lax.fori_loop(0, NXC, init_blk, 0)
    cp_big[1].start()

    def transpose_tiles(src, dst, j0, n):
        for j in range(n):
            for t in range(3):
                off = (j0 + j) * 384 + t * 128
                if not isinstance(off, int):
                    off = pl.multiple_of(off, 128)
                wb[9 * (j0 + j) + 3 * dst + t] = pltpu.bitcast(wt[src, pl.ds(off, 128), :].T, U32)

    def layer_a(l):
        def sub_all(x, op):
            x = op(x, pltpu.roll(x, 2, 0))
            return op(x, pltpu.roll(x, 4, 0))

        def phi(p):
            ts = [p[8 * t:8 * (t + 1)] for t in range(5)]
            mx = sub_all(functools.reduce(jnp.maximum, ts), jnp.maximum)
            mn = sub_all(functools.reduce(jnp.minimum, ts), jnp.minimum)
            ep = [jnp.exp(t - mx) for t in ts]
            en = [jnp.exp(mn - t) for t in ts]
            rp = 1.0 / sub_all(functools.reduce(jnp.add, ep), jnp.add)
            rn = 1.0 / sub_all(functools.reduce(jnp.add, en), jnp.add)
            return jnp.concatenate([e * rp for e in ep] + [e * rn for e in en], axis=0).astype(BF16)

        def phase1(i, carry):
            @pl.when(jnp.logical_and(l == 0, i == 0))
            def _():
                cp_wo.start()
                cp_mem.start()

            @pl.when(jnp.logical_and(l == 0, i == 1))
            def _():
                cp_big[2].start()

            @pl.when(jnp.logical_and(l == 0, i == 2))
            def _():
                for c in range(NOC):
                    cp_bwo(c).start()
                cp_big[0].wait()

            @pl.when(jnp.logical_and(l == 0, i == 3))
            def _():
                cp_big[1].wait()

            transpose_tiles(jnp.where(i < 2, 3, i - 2), jnp.where(i < 2, 2, i - 2), 0, NPAIR)
            off = pl.multiple_of(i * TB, TB)
            xn = pltpu.bitcast(xnb[pl.ds(pl.multiple_of(i * (TB // 2), TB // 2), TB // 2), :], BF16)
            xs = [xn[128 * u:128 * (u + 1)] for u in range(TB // 128)]
            for u, x in enumerate(xs):
                pq = _dot_nt(pltpu.bitcast(wat[1], BF16), x)
                for j in range(16):
                    phiq[j, :, pl.ds(off + 128 * u, 128)] = pltpu.bitcast(
                        phi(pq[40 * j:40 * (j + 1)]), U32)
            phik = []
            for x in xs:
                pk = _dot_nt(pltpu.bitcast(wat[0], BF16), x)
                phik.append([phi(pk[40 * j:40 * (j + 1)]) for j in range(16)])
            vt = [_dot_nt(pltpu.bitcast(wat[2], BF16), x) for x in xs]
            ones = jnp.ones((8, 128), F32)
            for u in range(len(xs)):
                for j in range(16):
                    lhs = jnp.concatenate([vt[u][40 * j:40 * (j + 1)], ones], axis=0).astype(BF16)
                    kvacc[j] = _dot_nt(lhs, phik[u][j]) + kvacc[j]
            return carry

        jax.lax.fori_loop(0, S // TB, phase1, 0)

        rr = _iota((48, 80), 0)
        cc = _iota((48, 80), 1)
        keep = jnp.where(rr < 40, _div20(rr), (rr - 40) >> 2) == (cc & 1)
        kvm = [jnp.where(keep, kvacc[j], 0.0).astype(BF16) for j in range(16)]
        lo4 = _iota((8, TC), 0) < 4

        def num(b):
            parts = []
            for j in range(16):
                r = _dot(kvm[j], pltpu.bitcast(phiq[j, :, TC * b:TC * (b + 1)], BF16))
                rc = 1.0 / (r[40:48] + 1e-6)
                rc2 = pltpu.roll(rc, 4, 0)
                ra = jnp.where(lo4, rc, rc2)
                rb = jnp.where(lo4, rc2, rc)
                parts += [r[0:8] * ra, r[8:16] * ra, r[16:24] * rc, r[24:32] * rb, r[32:40] * rb]
            return jnp.concatenate(parts, axis=0).astype(BF16).T

        for b in range(S // TC):
            obuf[TC // 2 * b:TC // 2 * (b + 1), :] = pltpu.bitcast(num(b), U32)

        @pl.when(l == 0)
        def _():
            cp_wo.wait()
            cp_mem.wait()
            cp_big[2].wait()

        def out(i, carry):
            transpose_tiles(2, 2, i * (NPAIR // 4), NPAIR // 4)
            xn32[0:RB, :] = _ln(xres[0:RB, :])
            memv[...] = mem0_ref[...].astype(F32)
            opend[...] = jnp.zeros_like(opend)
            kvacc[...] = jnp.zeros_like(kvacc)
            rows = pl.ds(pl.multiple_of(i * TB, TB), TB)
            o = pltpu.bitcast(obuf[pl.ds(pl.multiple_of(i * (TB // 2), TB // 2), TB // 2), :], BF16)
            xres[rows, :] = _dot(o, woa[...]) + xres[rows, :]
            return carry

        jax.lax.fori_loop(0, S // TB, out, 0)

        @pl.when(l == 0)
        def _():
            def cpo(c, carry):
                cp_bwo(c).wait()
                for u in range(OC // 384):
                    off = pl.multiple_of(c * OC + u * 384, 384)
                    bwo[pl.ds(pl.multiple_of(off // 2, 192), 192), :] = pltpu.bitcast(
                        wt[3, pl.ds(off, 384), :], U32)
                return carry

            jax.lax.fori_loop(0, NOC, cpo, 0)

    scale = DB ** (-0.5)

    def layer_b(layer):
        L = SEG + NM
        NEG = -1000000000.0

        def masks(even):
            nrow = SEG if even else L + 8
            rr = _iota((nrow, 128), 0)
            cc = _iota((nrow, 128), 1)
            is_a = (cc < L) | ((cc >= 2 * L) & (cc < 2 * L + 16))
            kx = jnp.where(cc < L, cc, cc - (L + NM))
            is_memkey = (cc >= SEG) & (cc < SEG + 2 * NM)
            if even:
                valid = cc < 2 * L
                allowed = valid & (is_memkey | (rr >= 24) | (kx <= rr + 8))
            else:
                dk = (cc - 2 * L) & 15
                cur = (rr < L) & (cc < 2 * L)
                old = (rr >= L) & (cc >= 2 * L) & (cc < 2 * L + 32)
                valid = cur | old
                allowed = ((cur & (is_memkey | (rr >= SEG) | (kx <= rr)))
                           | (old & ((dk >= 8) | (dk <= rr - L))))
            return is_a, allowed, jnp.where(valid, NEG, -jnp.inf).astype(F32)

        all_masks = {True: masks(True), False: masks(False)}

        def lo64(y):
            return _iota(y.shape, 1) < 64

        def stack_keys(a, b):
            parts = [a[0:L], b[SEG:L], b[0:SEG]]
            if a.shape[0] > L:
                parts += [a[L:], b[L:]]
            return jnp.concatenate(parts, axis=0).astype(BF16)

        def expand(y):
            y0, y1, y2 = y[:, 0:128], y[:, 128:256], y[:, 256:384]
            return (stack_keys(y0, y2),
                    stack_keys(jnp.where(lo64(y1), y1, 0.0), jnp.where(lo64(y1), 0.0, y1)))

        def pad_lanes(s):
            return jnp.concatenate([s, jnp.zeros((s.shape[0], 128 - s.shape[1]), F32)], axis=1)

        def step(h, even, kmajor):
            is_a, allowed, fill = all_masks[even]
            nrow = SEG if even else L + 8
            nkey = 2 * L if even else 2 * L + 32

            def proj(j):
                w = jnp.concatenate(
                    [pltpu.bitcast(wb[9 * j + t], BF16) for t in range(9)], axis=1)
                if j == 0 and kmajor:
                    y = _dot(h[:, 0:128], w[0:128])
                    for t in range(1, 5):
                        y = _dot(h[:, 128 * t:128 * (t + 1)], w[128 * t:128 * (t + 1)]) + y
                else:
                    y = _dot(h, w)
                if even:
                    snext[j] = y[SEG:L]
                    sdef[j, 0:8, :] = y[0:8]
                    sdef[j, 8:16, 384:1152] = y[L:L + 8, 384:1152]
                    q = jnp.concatenate([y[8:SEG, 0:384], y[L:L + 8, 0:384]], axis=0)
                    kv = jnp.concatenate([y[0:SEG, 384:1152], y[L:L + 8, 384:1152]], axis=0)
                else:
                    q = jnp.concatenate(
                        [snext[j, :, 0:384], y[:, 0:384], sdef[j, 0:8, 0:384]], axis=0)
                    kv = jnp.concatenate(
                        [snext[j, :, 384:1152], y[:, 384:1152], sdef[j, :, 384:1152]], axis=0)
                q = q.astype(BF16)
                q = (jnp.concatenate([q[:, 0:128], q[:, 256:384]], axis=0), q[:, 128:256])
                return q, expand(kv[:, 0:384]), expand(kv[:, 384:768])

            def scores(q, k):
                s02 = pad_lanes(_dot_nt(q[0], k[0]))
                s = jnp.where(is_a, s02[0:nrow], s02[nrow:]) + pad_lanes(_dot_nt(q[1], k[1]))
                s = jnp.where(allowed, s * scale, fill)
                ma = jnp.max(jnp.where(is_a, s, -jnp.inf), axis=1, keepdims=True)
                mb = jnp.max(jnp.where(is_a, -jnp.inf, s), axis=1, keepdims=True)
                e = jnp.exp(s - jnp.where(is_a, ma, mb))
                ea = jnp.where(is_a, e, 0.0)
                eb = jnp.where(is_a, 0.0, e)
                pa = ea * (1.0 / jnp.sum(ea, axis=1, keepdims=True))
                pb = eb * (1.0 / jnp.sum(eb, axis=1, keepdims=True))
                return (jnp.concatenate([pa, pb], axis=0)[:, 0:nkey].astype(BF16),
                        (pa + pb)[:, 0:nkey].astype(BF16))

            def pv(p, v):
                o02 = _dot(p[0], v[0])
                return jnp.concatenate(
                    [o02[0:nrow], _dot(p[1], v[1]), o02[nrow:]], axis=1).astype(BF16)

            qkv = [None] * NPAIR
            ps = [None] * NPAIR
            os_ = [None] * NPAIR

            def wo_chunk(c0, c1):
                w = pltpu.bitcast(bwo[192 * c0:192 * c1, :], BF16)
                return _dot(jnp.concatenate(os_[c0:c1], axis=1), w)

            lag = NPAIR if even else 4
            cuts = (0, 4, 8, 11, 14, 16) if even else (11, 12, 13, 14, 15, 16)
            qkv[0] = proj(0)
            acc = None
            for j in range(NPAIR + 2):
                c = None
                if j + 1 < NPAIR:
                    qkv[j + 1] = proj(j + 1)
                    if j >= lag:
                        c = wo_chunk(j - lag, j - lag + 1)
                else:
                    c = wo_chunk(cuts[j + 1 - NPAIR], cuts[j + 2 - NPAIR])
                if c is not None:
                    acc = c if acc is None else c + acc
                if j < NPAIR:
                    ps[j] = scores(qkv[j][0], qkv[j][1])
                if j >= 2:
                    os_[j - 2] = pv(ps[j - 2], qkv[j - 2][2])
            acc = wo_chunk(cuts[3], cuts[4]) + acc
            return wo_chunk(cuts[4], cuts[5]) + acc

        def finish_rows(base):
            xnew = xres[pl.ds(base, RB), :] + opend[...]
            xres[pl.ds(base, RB), :] = xnew
            xnb[pl.ds(pl.multiple_of(base // 2, RB // 2), RB // 2), :] = pltpu.bitcast(
                _ln(xnew).astype(BF16), U32)
            xin[pl.ds(base, RB), :] = xnew.astype(BF16)

        def body(i, carry):
            base = pl.multiple_of(i * RB, RB)

            @pl.when(jnp.logical_and(layer == 1, i >= 2))
            def _():
                rows = pl.ds(pl.multiple_of((i - 2) * RB, RB), RB)
                pltpu.make_async_copy(xin.at[rows], out_hbm.at[rows], sems.at[0]).start()

            finish_rows(pl.multiple_of(jnp.maximum(i - 1, 0) * RB, RB))
            mem = memv[...]
            for u in range(UNROLL):
                r0 = 64 * u
                h0 = jnp.concatenate([xn32[pl.ds(base + r0, 40), :], mem], axis=0).astype(BF16)
                o0 = step(h0, True, u > 0)
                opend[r0 + 8:r0 + 32, :] = o0[0:24]
                h1 = jnp.concatenate(
                    [xn32[pl.ds(base + r0 + 40, 24), :], o0[24:32]], axis=0).astype(BF16)
                o1 = step(h1, False, True)
                mem = o1[32:40]
                opend[r0:r0 + 8, :] = o1[40:48]
                opend[r0 + 32:r0 + 64, :] = o1[0:32]
            memv[...] = mem
            nxt = pl.ds(pl.multiple_of(jnp.minimum(i + 1, S // RB - 1) * RB, RB), RB)
            xn32[nxt, :] = _ln(xres[nxt, :])
            return carry

        jax.lax.fori_loop(0, S // RB, body, 0)

        @pl.when(layer == 0)
        def _():
            finish_rows(S - RB)

    def layer(l, carry):
        layer_a(l)
        layer_b(l)
        return carry

    jax.lax.fori_loop(0, 2, layer, 0)

    rows = pl.ds(S - 2 * RB, RB)
    pltpu.make_async_copy(xin.at[rows], out_hbm.at[rows], sems.at[0]).start()
    rows = pl.ds(S - RB, RB)
    xin[rows, :] = (xres[rows, :] + opend[...]).astype(BF16)
    pltpu.make_async_copy(xin.at[rows], out_hbm.at[rows], sems.at[0]).start()
    pltpu.make_async_copy(xin, out_hbm, sems.at[0]).wait()


@jax.jit
def pallas_interleave_layers__linear_kernel_hedgehog__memory_aug_recurrent_mem_tr__prompt_kernel(
    A_x: jax.Array,
    A_wqkv: jax.Array,
    A_w_phi: jax.Array,
    A_wo: jax.Array,
    B_x: jax.Array,
    B_mem0: jax.Array,
    B_Wq: jax.Array,
    B_Wk: jax.Array,
    B_Wv: jax.Array,
    B_Wo: jax.Array,
    B_seg_len: jax.Array,
):
    assert A_x.shape == (1, S, D) and B_mem0.shape == (1, NM, D) and B_Wq.shape == (D, HB, DB)
    tr = lambda w: jnp.transpose(w, (1, 2, 0)).reshape(HB * DB, D)
    any_spec = pl.BlockSpec(memory_space=pl.ANY)
    out = pl.pallas_call(
        _kernel,
        out_shape=jax.ShapeDtypeStruct((S, D), BF16),
        in_specs=[any_spec] * 9,
        out_specs=any_spec,
        scratch_shapes=[
            pltpu.VMEM((DA, DA, HA), BF16),
            pltpu.VMEM((NM, D), BF16),
            pltpu.VMEM((S, D), BF16),
            pltpu.VMEM((D, 3 * D), BF16),
            pltpu.VMEM((D, D), BF16),
            pltpu.VMEM((4, HB * DB, D), BF16),
            pltpu.VMEM((9 * NPAIR, D // 2, 128), U32),
            pltpu.VMEM((HB * DB // 2, D), U32),
            pltpu.VMEM((S, D), F32),
            pltpu.VMEM((S, D), F32),
            pltpu.VMEM((S // 2, D), U32),
            pltpu.VMEM((3, D // 2, D), U32),
            pltpu.VMEM((16, 48, 80), F32),
            pltpu.VMEM((16, 40, S), U32),
            pltpu.VMEM((S // 2, D), U32),
            pltpu.VMEM((NM, D), F32),
            pltpu.VMEM((NPAIR, 8, 9 * 128), F32),
            pltpu.VMEM((NPAIR, 16, 9 * 128), F32),
            pltpu.VMEM((64 * UNROLL, D), F32),
            pltpu.SemaphoreType.DMA((7,)),
            pltpu.SemaphoreType.DMA((NXC,)),
            pltpu.SemaphoreType.DMA((NOC,)),
        ],
        compiler_params=pltpu.CompilerParams(vmem_limit_bytes=120 * 1024 * 1024),
    )(A_x.reshape(S, D), A_wqkv, jnp.transpose(A_w_phi, (1, 2, 0)), A_wo,
      B_mem0.reshape(NM, D), tr(B_Wq), tr(B_Wk), tr(B_Wv), B_Wo.reshape(HB * DB, D))
    return out.reshape(1, S, D)
```

```python
import functools

import jax
import jax.numpy as jnp
import jax.experimental.pallas as pl
import jax.experimental.pallas.tpu as pltpu

F32 = jnp.float32
BF16 = jnp.bfloat16
U32 = jnp.uint32

S = 2048
D = 640
HA = 32
DA = 20
HB = 32
DB = 192
NM = 8
SEG = 32
NPAIR = HB // 2
TB = 512
TC = 512
UNROLL = 2
RB = 64 * UNROLL
NXC = 8
NOC = 8
LN_EPS = 1e-5

_NN = (((1,), (0,)), ((), ()))
_NT = (((1,), (1,)), ((), ()))


def _dot(a, b):
    return jax.lax.dot_general(a, b, _NN, preferred_element_type=F32)


def _dot_nt(a, b):
    return jax.lax.dot_general(a, b, _NT, preferred_element_type=F32)


def _ln(x):
    m = jnp.mean(x, axis=-1, keepdims=True)
    xc = x - m
    v = jnp.mean(xc * xc, axis=-1, keepdims=True)
    return xc * jax.lax.rsqrt(v + LN_EPS)


def _iota(shape, dim):
    return jax.lax.broadcasted_iota(jnp.int32, shape, dim)


def _div20(i):
    return (i * 3277) >> 16


def _div40(i):
    return _div20(i) >> 1


def _kernel(x_hbm, wqkv_hbm, wphi_hbm, wo_hbm, mem0_hbm, wqt_hbm, wkt_hbm, wvt_hbm, bwo_hbm,
            out_hbm,
            wphi_ref, mem0_ref, xin, wqkv, woa, wt, wb, bwo, xres, xn32, xnb, wat, kvacc, phiq, obuf,
            memv, snext, sdef, opend, sems, xsems, osems):
    XC = S // NXC
    cp_phi = pltpu.make_async_copy(wphi_hbm, wphi_ref, sems.at[0])
    cp_wqkv = pltpu.make_async_copy(wqkv_hbm, wqkv, sems.at[1])

    def cp_x(c):
        rows = pl.ds(pl.multiple_of(c * XC, XC), XC)
        return pltpu.make_async_copy(x_hbm.at[rows], xin.at[rows], xsems.at[c])

    cp_wo = pltpu.make_async_copy(wo_hbm, woa, sems.at[2])
    cp_mem = pltpu.make_async_copy(mem0_hbm, mem0_ref, sems.at[3])
    cp_big = [
        pltpu.make_async_copy(wqt_hbm, wt.at[0], sems.at[4]),
        pltpu.make_async_copy(wkt_hbm, wt.at[1], sems.at[5]),
        pltpu.make_async_copy(wvt_hbm, wt.at[2], sems.at[6]),
    ]
    OC = HB * DB // NOC

    def cp_bwo(c):
        rows = pl.ds(pl.multiple_of(c * OC, OC), OC)
        return pltpu.make_async_copy(bwo_hbm.at[rows], wt.at[3, rows], osems.at[c])

    def start_first(c, carry):
        @pl.when(c == 0)
        def _():
            cp_phi.start()

        @pl.when(c == 1)
        def _():
            cp_wqkv.start()

        @pl.when(c >= 2)
        def _():
            cp_x(c - 2).start()

        return carry

    jax.lax.fori_loop(0, NXC + 2, start_first, 0)
    cp_phi.wait()

    wphi = wphi_ref[...].astype(F32)
    xw = jnp.concatenate([wphi[d] for d in range(DA)], axis=1)
    xw = jnp.concatenate([xw, jnp.zeros((32 - DA, D), F32)], axis=0).astype(BF16)
    r = _iota((D, D), 0)
    c = _iota((D, D), 1)
    perm = jnp.where((r & 31) * DA + (r >> 5) == c, 1.0, 0.0).astype(BF16)
    wf = _dot(xw, perm).astype(BF16)
    r = _iota((160, 32), 0)
    c = _iota((160, 32), 1)
    rsel = jnp.where(((r - _div40(r) * 40) >> 1) == c, 1.0, 0.0).astype(BF16)
    r = _iota((160, 128), 0)
    c = _iota((160, 128), 1)
    phit = []
    for t in range(5):
        keep = 2 * (_div40(r) + 3 * t) + (r & 1) == _div20(c + 128 * t)
        phit.append(jnp.where(keep, _dot(rsel, wf[:, 128 * t:128 * (t + 1)]), 0.0).astype(BF16))

    kvacc[...] = jnp.zeros_like(kvacc)

    def clear_slot(c, carry):
        wt[3, pl.ds(pl.multiple_of(c * 384, 384), 384), :] = jnp.zeros((384, D), BF16)
        return carry

    jax.lax.fori_loop(0, NPAIR, clear_slot, 0)
    cp_wqkv.wait()
    cp_big[0].start()
    for m, dst in ((1, 0), (0, 1)):
        p = [_dot_nt(phit[t], wqkv[:, m * D + 128 * t:m * D + 128 * (t + 1)]) for t in range(5)]
        rows = [p[0][0:120]]
        for t in range(1, 5):
            rows += [p[t - 1][120:160] + p[t][0:40], p[t][40:120]]
        rows.append(p[4][120:160])
        wat[dst] = pltpu.bitcast(jnp.concatenate(rows, axis=0).astype(BF16), U32)
    wat[2] = pltpu.bitcast(wqkv[:, 2 * D:3 * D].T, U32)

    def init_blk(i, carry):
        cp_x(i).wait()
        for u in range(XC // 64):
            off = pl.multiple_of(i * XC + u * 64, 64)
            x = xin[pl.ds(off, 64), :].astype(F32)
            xres[pl.ds(off, 64), :] = x
            xnb[pl.ds(pl.multiple_of(off // 2, 32), 32), :] = pltpu.bitcast(_ln(x).astype(BF16), U32)
        return carry

    jax.lax.fori_loop(0, NXC, init_blk, 0)
    cp_big[1].start()

    def transpose_tiles(src, dst, j0, n):
        for j in range(n):
            for t in range(3):
                off = (j0 + j) * 384 + t * 128
                if not isinstance(off, int):
                    off = pl.multiple_of(off, 128)
                wb[9 * (j0 + j) + 3 * dst + t] = pltpu.bitcast(wt[src, pl.ds(off, 128), :].T, U32)

    def layer_a(l):
        def sub_all(x, op):
            x = op(x, pltpu.roll(x, 2, 0))
            return op(x, pltpu.roll(x, 4, 0))

        def phi(p):
            ts = [p[8 * t:8 * (t + 1)] for t in range(5)]
            mx = sub_all(functools.reduce(jnp.maximum, ts), jnp.maximum)
            mn = sub_all(functools.reduce(jnp.minimum, ts), jnp.minimum)
            ep = [jnp.exp(t - mx) for t in ts]
            en = [jnp.exp(mn - t) for t in ts]
            rp = 1.0 / sub_all(functools.reduce(jnp.add, ep), jnp.add)
            rn = 1.0 / sub_all(functools.reduce(jnp.add, en), jnp.add)
            return jnp.concatenate([e * rp for e in ep] + [e * rn for e in en], axis=0).astype(BF16)

        def phase1(i, carry):
            @pl.when(jnp.logical_and(l == 0, i == 0))
            def _():
                cp_wo.start()
                cp_mem.start()

            @pl.when(jnp.logical_and(l == 0, i == 1))
            def _():
                cp_big[2].start()

            @pl.when(jnp.logical_and(l == 0, i == 2))
            def _():
                for c in range(NOC):
                    cp_bwo(c).start()
                cp_big[0].wait()

            @pl.when(jnp.logical_and(l == 0, i == 3))
            def _():
                cp_big[1].wait()

            transpose_tiles(jnp.where(i < 2, 3, i - 2), jnp.where(i < 2, 2, i - 2), 0, NPAIR)
            off = pl.multiple_of(i * TB, TB)
            xn = pltpu.bitcast(xnb[pl.ds(pl.multiple_of(i * (TB // 2), TB // 2), TB // 2), :], BF16)
            xs = [xn[128 * u:128 * (u + 1)] for u in range(TB // 128)]
            for u, x in enumerate(xs):
                pq = _dot_nt(pltpu.bitcast(wat[1], BF16), x)
                for j in range(16):
                    phiq[j, :, pl.ds(off + 128 * u, 128)] = pltpu.bitcast(
                        phi(pq[40 * j:40 * (j + 1)]), U32)
            phik = []
            for x in xs:
                pk = _dot_nt(pltpu.bitcast(wat[0], BF16), x)
                phik.append([phi(pk[40 * j:40 * (j + 1)]) for j in range(16)])
            vt = [_dot_nt(pltpu.bitcast(wat[2], BF16), x) for x in xs]
            ones = jnp.ones((8, 128), F32)
            for u in range(len(xs)):
                for j in range(16):
                    lhs = jnp.concatenate([vt[u][40 * j:40 * (j + 1)], ones], axis=0).astype(BF16)
                    kvacc[j] = _dot_nt(lhs, phik[u][j]) + kvacc[j]
            return carry

        jax.lax.fori_loop(0, S // TB, phase1, 0)

        rr = _iota((48, 80), 0)
        cc = _iota((48, 80), 1)
        keep = jnp.where(rr < 40, _div20(rr), (rr - 40) >> 2) == (cc & 1)
        kvm = [jnp.where(keep, kvacc[j], 0.0).astype(BF16) for j in range(16)]
        lo4 = _iota((8, TC), 0) < 4

        def num(b):
            parts = []
            for j in range(16):
                r = _dot(kvm[j], pltpu.bitcast(phiq[j, :, TC * b:TC * (b + 1)], BF16))
                rc = 1.0 / (r[40:48] + 1e-6)
                rc2 = pltpu.roll(rc, 4, 0)
                ra = jnp.where(lo4, rc, rc2)
                rb = jnp.where(lo4, rc2, rc)
                parts += [r[0:8] * ra, r[8:16] * ra, r[16:24] * rc, r[24:32] * rb, r[32:40] * rb]
            return jnp.concatenate(parts, axis=0).astype(BF16).T

        for b in range(S // TC):
            obuf[TC // 2 * b:TC // 2 * (b + 1), :] = pltpu.bitcast(num(b), U32)

        @pl.when(l == 0)
        def _():
            cp_wo.wait()
            cp_mem.wait()
            cp_big[2].wait()

        def out(i, carry):
            transpose_tiles(2, 2, i * (NPAIR // 4), NPAIR // 4)
            xn32[0:RB, :] = _ln(xres[0:RB, :])
            memv[...] = mem0_ref[...].astype(F32)
            opend[...] = jnp.zeros_like(opend)
            kvacc[...] = jnp.zeros_like(kvacc)
            rows = pl.ds(pl.multiple_of(i * TB, TB), TB)
            o = pltpu.bitcast(obuf[pl.ds(pl.multiple_of(i * (TB // 2), TB // 2), TB // 2), :], BF16)
            xres[rows, :] = _dot(o, woa[...]) + xres[rows, :]
            return carry

        jax.lax.fori_loop(0, S // TB, out, 0)

        @pl.when(l == 0)
        def _():
            def cpo(c, carry):
                cp_bwo(c).wait()
                for u in range(OC // 384):
                    off = pl.multiple_of(c * OC + u * 384, 384)
                    bwo[pl.ds(pl.multiple_of(off // 2, 192), 192), :] = pltpu.bitcast(
                        wt[3, pl.ds(off, 384), :], U32)
                return carry

            jax.lax.fori_loop(0, NOC, cpo, 0)

    scale = DB ** (-0.5)

    def layer_b(layer):
        L = SEG + NM
        NEG = -1000000000.0

        def masks(even):
            nrow = SEG if even else L + 8
            rr = _iota((nrow, 128), 0)
            cc = _iota((nrow, 128), 1)
            is_a = (cc < L) | ((cc >= 2 * L) & (cc < 2 * L + 16))
            kx = jnp.where(cc < L, cc, cc - (L + NM))
            is_memkey = (cc >= SEG) & (cc < SEG + 2 * NM)
            if even:
                valid = cc < 2 * L
                allowed = valid & (is_memkey | (rr >= 24) | (kx <= rr + 8))
            else:
                dk = (cc - 2 * L) & 15
                cur = (rr < L) & (cc < 2 * L)
                old = (rr >= L) & (cc >= 2 * L) & (cc < 2 * L + 32)
                valid = cur | old
                allowed = ((cur & (is_memkey | (rr >= SEG) | (kx <= rr)))
                           | (old & ((dk >= 8) | (dk <= rr - L))))
            return is_a, allowed, jnp.where(valid, NEG, -jnp.inf).astype(F32)

        all_masks = {True: masks(True), False: masks(False)}

        def lo64(y):
            return _iota(y.shape, 1) < 64

        def stack_keys(a, b):
            parts = [a[0:L], b[SEG:L], b[0:SEG]]
            if a.shape[0] > L:
                parts += [a[L:], b[L:]]
            return jnp.concatenate(parts, axis=0).astype(BF16)

        def expand(y):
            y0, y1, y2 = y[:, 0:128], y[:, 128:256], y[:, 256:384]
            return (stack_keys(y0, y2),
                    stack_keys(jnp.where(lo64(y1), y1, 0.0), jnp.where(lo64(y1), 0.0, y1)))

        def pad_lanes(s):
            return jnp.concatenate([s, jnp.zeros((s.shape[0], 128 - s.shape[1]), F32)], axis=1)

        def step(hq, hkv, even, kmajor, side=None, never=None):
            is_a, allowed, fill = all_masks[even]
            nrow = SEG if even else L + 8
            nkey = 2 * L if even else 2 * L + 32

            def tiles(j, ts):
                return jnp.concatenate([pltpu.bitcast(wb[9 * j + t], BF16) for t in ts], axis=1)

            def proj(j):
                if j == 0 and kmajor:
                    wq, wkv = tiles(j, range(3)), tiles(j, range(3, 9))
                    q = _dot(hq[:, 0:128], wq[0:128])
                    y = _dot(hkv[:, 0:128], wkv[0:128])
                    for t in range(1, 5):
                        ks = slice(128 * t, 128 * (t + 1))
                        q = _dot(hq[:, ks], wq[ks]) + q
                        y = _dot(hkv[:, ks], wkv[ks]) + y
                else:
                    q = _dot(hq, tiles(j, range(3)))
                    y = _dot(hkv, tiles(j, range(3, 9)))
                if even:
                    snext[j] = y[SEG:L]
                    sdef[j, 0:8, :] = y[0:8]
                    sdef[j, 8:16, :] = y[L:L + 8]
                    kv = jnp.concatenate([y[0:SEG], y[L:L + 8]], axis=0)
                else:
                    kv = jnp.concatenate([snext[j], y, sdef[j]], axis=0)
                q = q.astype(BF16)
                q = (jnp.concatenate([q[:, 0:128], q[:, 256:384]], axis=0), q[:, 128:256])
                return q, expand(kv[:, 0:384]), expand(kv[:, 384:768])

            def scores(q, k, tok=None):
                s02 = pad_lanes(_dot_nt(q[0], k[0]))
                s = jnp.where(is_a, s02[0:nrow], s02[nrow:]) + pad_lanes(_dot_nt(q[1], k[1]))
                s = jnp.where(allowed, s * scale, fill)
                ma = jnp.max(jnp.where(is_a, s, -jnp.inf), axis=1, keepdims=True)
                mb = jnp.max(jnp.where(is_a, -jnp.inf, s), axis=1, keepdims=True)
                e = jnp.exp(s - jnp.where(is_a, ma, mb))
                ea = jnp.where(is_a, e, 0.0)
                eb = jnp.where(is_a, 0.0, e)
                pa = ea * (1.0 / jnp.sum(ea, axis=1, keepdims=True))
                pb = eb * (1.0 / jnp.sum(eb, axis=1, keepdims=True))
                if tok is not None:
                    pb = jnp.concatenate([jnp.where(never, tok, pb[0:16]), pb[16:]], axis=0)
                return (jnp.concatenate([pa, pb], axis=0)[:, 0:nkey].astype(BF16),
                        (pa + pb)[:, 0:nkey].astype(BF16))

            def pv(p, v):
                o02 = _dot(p[0], v[0])
                return jnp.concatenate(
                    [o02[0:nrow], _dot(p[1], v[1]), o02[nrow:]], axis=1).astype(BF16)

            qkv = [None] * NPAIR
            ps = [None] * NPAIR
            os_ = [None] * NPAIR

            def wo_chunk(c0, c1):
                w = pltpu.bitcast(bwo[192 * c0:192 * c1, :], BF16)
                return _dot(jnp.concatenate(os_[c0:c1], axis=1), w)

            cuts = (0, 4, 8, 11, 14, 16) if even else (11, 12, 13, 14, 15, 16)
            lag = NPAIR - 1 - cuts[0]
            qkv[0] = proj(0)
            acc = None
            for j in range(NPAIR + 2):
                c = None
                if j + 1 < NPAIR:
                    qkv[j + 1] = proj(j + 1)
                    if j >= lag:
                        c = wo_chunk(j - lag, j - lag + 1)
                else:
                    c = wo_chunk(cuts[j + 1 - NPAIR], cuts[j + 2 - NPAIR])
                if c is not None:
                    acc = c if acc is None else c + acc
                if j < NPAIR:
                    ps[j] = scores(qkv[j][0], qkv[j][1], side(j) if side else None)
                if j >= 2:
                    os_[j - 2] = pv(ps[j - 2], qkv[j - 2][2])
            acc = wo_chunk(cuts[3], cuts[4]) + acc
            return wo_chunk(cuts[4], cuts[5]) + acc

        def finish_rows(base, r0, n):
            rows = pl.ds(base + r0, n)
            xnew = xres[rows, :] + opend[r0:r0 + n, :]
            xres[rows, :] = xnew
            xin[rows, :] = xnew.astype(BF16)
            y = _ln(xnew)
            xnb[pl.ds(pl.multiple_of(base // 2, RB // 2) + r0 // 2, n // 2), :] = pltpu.bitcast(
                y.astype(BF16), U32)
            return y

        def body(i, carry):
            base = pl.multiple_of(i * RB, RB)

            @pl.when(jnp.logical_and(layer == 1, i >= 2))
            def _():
                rows = pl.ds(pl.multiple_of((i - 2) * RB, RB), RB)
                pltpu.make_async_copy(xin.at[rows], out_hbm.at[rows], sems.at[0]).start()

            prev = pl.multiple_of(jnp.maximum(i - 1, 0) * RB, RB)
            nxt = pl.multiple_of(jnp.minimum(i + 1, S // RB - 1) * RB, RB)

            def token(y):
                return functools.reduce(
                    jnp.maximum, [y[:, 128 * t:128 * (t + 1)] for t in range(5)])

            def side_prev(j):
                if j % 2:
                    return None
                return token(finish_rows(prev, 8 * j, 16))

            def side_next(j):
                if j % 2:
                    return None
                rows = pl.ds(nxt + 8 * j, 16)
                y = _ln(xres[rows, :])
                xn32[rows, :] = y
                return token(y)

            sides = (side_prev, side_next)
            never = i < 0
            mem = memv[...]
            for u in range(UNROLL):
                r0 = 64 * u
                xr = lambda a, n: xn32[pl.ds(base + r0 + a, n), :]
                cat = lambda *p: jnp.concatenate(p, axis=0).astype(BF16)
                o0 = step(cat(xr(8, 24), mem), cat(xr(0, 40), mem), True, u > 0, sides[u], never)
                opend[r0 + 8:r0 + 32, :] = o0[0:24]
                mem = o0[24:32]
                o1 = step(cat(xr(32, 32), mem, xr(0, 8)), cat(xr(40, 24), mem), False, True)
                mem = o1[32:40]
                opend[r0:r0 + 8, :] = o1[40:48]
                opend[r0 + 32:r0 + 64, :] = o1[0:32]
            memv[...] = mem
            return carry

        jax.lax.fori_loop(0, S // RB, body, 0)

        @pl.when(layer == 0)
        def _():
            finish_rows(S - RB, 0, RB)

    def layer(l, carry):
        layer_a(l)
        layer_b(l)
        return carry

    jax.lax.fori_loop(0, 2, layer, 0)

    rows = pl.ds(S - 2 * RB, RB)
    pltpu.make_async_copy(xin.at[rows], out_hbm.at[rows], sems.at[0]).start()
    rows = pl.ds(S - RB, RB)
    xin[rows, :] = (xres[rows, :] + opend[...]).astype(BF16)
    pltpu.make_async_copy(xin.at[rows], out_hbm.at[rows], sems.at[0]).start()
    pltpu.make_async_copy(xin, out_hbm, sems.at[0]).wait()


@jax.jit
def pallas_interleave_layers__linear_kernel_hedgehog__memory_aug_recurrent_mem_tr__prompt_kernel(
    A_x: jax.Array,
    A_wqkv: jax.Array,
    A_w_phi: jax.Array,
    A_wo: jax.Array,
    B_x: jax.Array,
    B_mem0: jax.Array,
    B_Wq: jax.Array,
    B_Wk: jax.Array,
    B_Wv: jax.Array,
    B_Wo: jax.Array,
    B_seg_len: jax.Array,
):
    assert A_x.shape == (1, S, D) and B_mem0.shape == (1, NM, D) and B_Wq.shape == (D, HB, DB)
    tr = lambda w: jnp.transpose(w, (1, 2, 0)).reshape(HB * DB, D)
    any_spec = pl.BlockSpec(memory_space=pl.ANY)
    out = pl.pallas_call(
        _kernel,
        out_shape=jax.ShapeDtypeStruct((S, D), BF16),
        in_specs=[any_spec] * 9,
        out_specs=any_spec,
        scratch_shapes=[
            pltpu.VMEM((DA, DA, HA), BF16),
            pltpu.VMEM((NM, D), BF16),
            pltpu.VMEM((S, D), BF16),
            pltpu.VMEM((D, 3 * D), BF16),
            pltpu.VMEM((D, D), BF16),
            pltpu.VMEM((4, HB * DB, D), BF16),
            pltpu.VMEM((9 * NPAIR, D // 2, 128), U32),
            pltpu.VMEM((HB * DB // 2, D), U32),
            pltpu.VMEM((S, D), F32),
            pltpu.VMEM((S, D), F32),
            pltpu.VMEM((S // 2, D), U32),
            pltpu.VMEM((3, D // 2, D), U32),
            pltpu.VMEM((16, 48, 80), F32),
            pltpu.VMEM((16, 40, S), U32),
            pltpu.VMEM((S // 2, D), U32),
            pltpu.VMEM((NM, D), F32),
            pltpu.VMEM((NPAIR, 8, 6 * 128), F32),
            pltpu.VMEM((NPAIR, 16, 6 * 128), F32),
            pltpu.VMEM((64 * UNROLL, D), F32),
            pltpu.SemaphoreType.DMA((7,)),
            pltpu.SemaphoreType.DMA((NXC,)),
            pltpu.SemaphoreType.DMA((NOC,)),
        ],
        compiler_params=pltpu.CompilerParams(vmem_limit_bytes=120 * 1024 * 1024),
    )(A_x.reshape(S, D), A_wqkv, jnp.transpose(A_w_phi, (1, 2, 0)), A_wo,
      B_mem0.reshape(NM, D), tr(B_Wq), tr(B_Wk), tr(B_Wv), B_Wo.reshape(HB * DB, D))
    return out.reshape(1, S, D)
```

```python
import functools

import jax
import jax.numpy as jnp
import jax.experimental.pallas as pl
import jax.experimental.pallas.tpu as pltpu

F32 = jnp.float32
BF16 = jnp.bfloat16
U32 = jnp.uint32

S = 2048
D = 640
HA = 32
DA = 20
HB = 32
DB = 192
NM = 8
SEG = 32
NPAIR = HB // 2
NF = HA * (DA - 1)
TB = 512
TC = 512
UNROLL = 2
RB = 64 * UNROLL
NXC = 8
NOC = 8
LN_EPS = 1e-5

_NN = (((1,), (0,)), ((), ()))
_NT = (((1,), (1,)), ((), ()))


def _dot(a, b):
    return jax.lax.dot_general(a, b, _NN, preferred_element_type=F32)


def _dot_nt(a, b):
    return jax.lax.dot_general(a, b, _NT, preferred_element_type=F32)


def _ln(x):
    m = jnp.mean(x, axis=-1, keepdims=True)
    xc = x - m
    v = jnp.mean(xc * xc, axis=-1, keepdims=True)
    return xc * jax.lax.rsqrt(v + LN_EPS)


def _iota(shape, dim):
    return jax.lax.broadcasted_iota(jnp.int32, shape, dim)


def _div20(i):
    return (i * 3277) >> 16


def _div40(i):
    return _div20(i) >> 1


def _kernel(x_hbm, wqkv_hbm, wphi_hbm, wo_hbm, mem0_hbm, wqt_hbm, wkt_hbm, wvt_hbm, bwo_hbm,
            out_hbm,
            wphi_ref, mem0_ref, xin, wqkv, woa, wt, wb, bwo, xres, xn32, xnb, wat, kvacc, phiq, obuf,
            memv, snext, sdef, opend, sems, xsems, osems):
    XC = S // NXC
    cp_phi = pltpu.make_async_copy(wphi_hbm, wphi_ref, sems.at[0])
    cp_wqkv = pltpu.make_async_copy(wqkv_hbm, wqkv, sems.at[1])

    def cp_x(c):
        rows = pl.ds(pl.multiple_of(c * XC, XC), XC)
        return pltpu.make_async_copy(x_hbm.at[rows], xin.at[rows], xsems.at[c])

    cp_wo = pltpu.make_async_copy(wo_hbm, woa, sems.at[2])
    cp_mem = pltpu.make_async_copy(mem0_hbm, mem0_ref, sems.at[3])
    cp_big = [
        pltpu.make_async_copy(wqt_hbm, wt.at[0], sems.at[4]),
        pltpu.make_async_copy(wkt_hbm, wt.at[1], sems.at[5]),
        pltpu.make_async_copy(wvt_hbm, wt.at[2], sems.at[6]),
    ]
    OC = HB * DB // NOC

    def cp_bwo(c):
        rows = pl.ds(pl.multiple_of(c * OC, OC), OC)
        return pltpu.make_async_copy(bwo_hbm.at[rows], wt.at[3, rows], osems.at[c])

    def start_first(c, carry):
        @pl.when(c == 0)
        def _():
            cp_phi.start()

        @pl.when(c == 1)
        def _():
            cp_wqkv.start()

        @pl.when(c >= 2)
        def _():
            cp_x(c - 2).start()

        return carry

    jax.lax.fori_loop(0, NXC + 2, start_first, 0)
    cp_phi.wait()

    wphi = wphi_ref[...].astype(F32)
    xw = jnp.concatenate([wphi[d] for d in range(DA)], axis=1)
    xw = jnp.concatenate([xw, jnp.zeros((32 - DA, D), F32)], axis=0).astype(BF16)
    r = _iota((D, D), 0)
    c = _iota((D, D), 1)
    perm = jnp.where((r & 31) * DA + (r >> 5) == c, 1.0, 0.0).astype(BF16)
    wf = _dot(xw, perm).astype(BF16)
    r = _iota((160, 32), 0)
    c = _iota((160, 32), 1)
    rsel = jnp.where(((r - _div40(r) * 40) >> 1) == c, 1.0, 0.0).astype(BF16)
    r = _iota((160, 128), 0)
    c = _iota((160, 128), 1)
    phit = []
    for t in range(5):
        keep = 2 * (_div40(r) + 3 * t) + (r & 1) == _div20(c + 128 * t)
        phit.append(jnp.where(keep, _dot(rsel, wf[:, 128 * t:128 * (t + 1)]), 0.0).astype(BF16))

    kvacc[...] = jnp.zeros_like(kvacc)

    def clear_slot(c, carry):
        wt[3, pl.ds(pl.multiple_of(c * 384, 384), 384), :] = jnp.zeros((384, D), BF16)
        return carry

    jax.lax.fori_loop(0, NPAIR, clear_slot, 0)
    cp_wqkv.wait()
    cp_big[0].start()
    for m, dst in ((1, 0), (0, 1)):
        p = [_dot_nt(phit[t], wqkv[:, m * D + 128 * t:m * D + 128 * (t + 1)]) for t in range(5)]
        rows = [p[0][0:120]]
        for t in range(1, 5):
            rows += [p[t - 1][120:160] + p[t][0:40], p[t][40:120]]
        rows.append(p[4][120:160])
        w = jnp.concatenate(rows, axis=0)
        sub = _iota((8, D), 0)
        groups = []
        for j in range(16):
            ref = jnp.where(sub < 2, w[40 * j:40 * j + 8], 0.0)
            ref = ref + pltpu.roll(ref, 2, 0)
            ref = ref + pltpu.roll(ref, 4, 0)
            groups.append([w[40 * j + 8 * t:40 * j + 8 * (t + 1)] - ref for t in range(5)])
        rows = []
        for g in range(4):
            for t in range(3):
                rows.append(jnp.where(sub < 2, pltpu.roll(groups[4 * g + 3][0], 6 - 2 * t, 0),
                                      groups[4 * g + t][0]))
            for t in range(4):
                rows += groups[4 * g + t][1:]
        wat[dst, 0:NF // 2, :] = pltpu.bitcast(jnp.concatenate(rows, axis=0).astype(BF16), U32)
    wat[2] = pltpu.bitcast(wqkv[:, 2 * D:3 * D].T, U32)

    def init_blk(i, carry):
        cp_x(i).wait()
        for u in range(XC // 64):
            off = pl.multiple_of(i * XC + u * 64, 64)
            x = xin[pl.ds(off, 64), :].astype(F32)
            xres[pl.ds(off, 64), :] = x
            xnb[pl.ds(pl.multiple_of(off // 2, 32), 32), :] = pltpu.bitcast(_ln(x).astype(BF16), U32)
        return carry

    jax.lax.fori_loop(0, NXC, init_blk, 0)
    cp_big[1].start()

    def transpose_tiles(src, dst, j0, n):
        for j in range(n):
            for t in range(3):
                off = (j0 + j) * 384 + t * 128
                if not isinstance(off, int):
                    off = pl.multiple_of(off, 128)
                wb[9 * (j0 + j) + 3 * dst + t] = pltpu.bitcast(wt[src, pl.ds(off, 128), :].T, U32)

    def layer_a(l):
        def sub_all(x, op):
            x = op(x, pltpu.roll(x, 2, 0))
            return op(x, pltpu.roll(x, 4, 0))

        def features(m, x):
            p = _dot_nt(pltpu.bitcast(wat[m, 0:NF // 2, :], BF16), x)
            p = [p[8 * t:8 * (t + 1)] for t in range(NF // 8)]
            sub = _iota((8, 128), 0)
            out = []
            for j in range(16):
                g, t = divmod(j, 4)
                pg = p[19 * g:19 * (g + 1)]
                if t < 3:
                    head = pg[t]
                else:
                    head = jnp.where(sub < 4, pltpu.roll(pg[0], 2, 0),
                                     jnp.where(sub < 6, pltpu.roll(pg[1], 4, 0),
                                               pltpu.roll(pg[2], 6, 0)))
                out.append([jnp.where(sub < 2, 0.0, head)] + pg[3 + 4 * t:7 + 4 * t])
            return out

        def phi(ts):
            mx = sub_all(functools.reduce(jnp.maximum, ts), jnp.maximum)
            mn = sub_all(functools.reduce(jnp.minimum, ts), jnp.minimum)
            ep = [jnp.exp(t - mx) for t in ts]
            en = [jnp.exp(mn - t) for t in ts]
            rp = 1.0 / sub_all(functools.reduce(jnp.add, ep), jnp.add)
            rn = 1.0 / sub_all(functools.reduce(jnp.add, en), jnp.add)
            return jnp.concatenate([e * rp for e in ep] + [e * rn for e in en], axis=0).astype(BF16)

        def phase1(i, carry):
            @pl.when(jnp.logical_and(l == 0, i == 0))
            def _():
                cp_wo.start()
                cp_mem.start()

            @pl.when(jnp.logical_and(l == 0, i == 1))
            def _():
                cp_big[2].start()

            @pl.when(jnp.logical_and(l == 0, i == 2))
            def _():
                for c in range(NOC):
                    cp_bwo(c).start()
                cp_big[0].wait()

            @pl.when(jnp.logical_and(l == 0, i == 3))
            def _():
                cp_big[1].wait()

            transpose_tiles(jnp.where(i < 2, 3, i - 2), jnp.where(i < 2, 2, i - 2), 0, NPAIR)
            off = pl.multiple_of(i * TB, TB)
            xn = pltpu.bitcast(xnb[pl.ds(pl.multiple_of(i * (TB // 2), TB // 2), TB // 2), :], BF16)
            xs = [xn[128 * u:128 * (u + 1)] for u in range(TB // 128)]
            for u, x in enumerate(xs):
                for j, ts in enumerate(features(1, x)):
                    phiq[j, :, pl.ds(off + 128 * u, 128)] = pltpu.bitcast(phi(ts), U32)
            phik = [[phi(ts) for ts in features(0, x)] for x in xs]
            vt = [_dot_nt(pltpu.bitcast(wat[2], BF16), x) for x in xs]
            ones = jnp.ones((8, 128), F32)
            for u in range(len(xs)):
                for j in range(16):
                    lhs = jnp.concatenate([vt[u][40 * j:40 * (j + 1)], ones], axis=0).astype(BF16)
                    kvacc[j] = _dot_nt(lhs, phik[u][j]) + kvacc[j]
            return carry

        jax.lax.fori_loop(0, S // TB, phase1, 0)

        rr = _iota((48, 80), 0)
        cc = _iota((48, 80), 1)
        keep = jnp.where(rr < 40, _div20(rr), (rr - 40) >> 2) == (cc & 1)
        kvm = [jnp.where(keep, kvacc[j], 0.0).astype(BF16) for j in range(16)]
        lo4 = _iota((8, TC), 0) < 4

        def num(b):
            parts = []
            for j in range(16):
                r = _dot(kvm[j], pltpu.bitcast(phiq[j, :, TC * b:TC * (b + 1)], BF16))
                rc = 1.0 / (r[40:48] + 1e-6)
                rc2 = pltpu.roll(rc, 4, 0)
                ra = jnp.where(lo4, rc, rc2)
                rb = jnp.where(lo4, rc2, rc)
                parts += [r[0:8] * ra, r[8:16] * ra, r[16:24] * rc, r[24:32] * rb, r[32:40] * rb]
            return jnp.concatenate(parts, axis=0).astype(BF16).T

        for b in range(S // TC):
            obuf[TC // 2 * b:TC // 2 * (b + 1), :] = pltpu.bitcast(num(b), U32)

        @pl.when(l == 0)
        def _():
            cp_wo.wait()
            cp_mem.wait()
            cp_big[2].wait()

        def out(i, carry):
            transpose_tiles(2, 2, i * (NPAIR // 4), NPAIR // 4)
            xn32[0:RB, :] = _ln(xres[0:RB, :])
            memv[...] = mem0_ref[...].astype(F32)
            opend[...] = jnp.zeros_like(opend)
            kvacc[...] = jnp.zeros_like(kvacc)
            rows = pl.ds(pl.multiple_of(i * TB, TB), TB)
            o = pltpu.bitcast(obuf[pl.ds(pl.multiple_of(i * (TB // 2), TB // 2), TB // 2), :], BF16)
            xres[rows, :] = _dot(o, woa[...]) + xres[rows, :]
            return carry

        jax.lax.fori_loop(0, S // TB, out, 0)

        @pl.when(l == 0)
        def _():
            def cpo(c, carry):
                cp_bwo(c).wait()
                for u in range(OC // 384):
                    off = pl.multiple_of(c * OC + u * 384, 384)
                    bwo[pl.ds(pl.multiple_of(off // 2, 192), 192), :] = pltpu.bitcast(
                        wt[3, pl.ds(off, 384), :], U32)
                return carry

            jax.lax.fori_loop(0, NOC, cpo, 0)

    scale = DB ** (-0.5)

    def layer_b(layer):
        L = SEG + NM
        NEG = -1000000000.0

        def masks(even):
            nrow = SEG if even else L + 8
            rr = _iota((nrow, 128), 0)
            cc = _iota((nrow, 128), 1)
            is_a = (cc < L) | ((cc >= 2 * L) & (cc < 2 * L + 16))
            kx = jnp.where(cc < L, cc, cc - (L + NM))
            is_memkey = (cc >= SEG) & (cc < SEG + 2 * NM)
            if even:
                valid = cc < 2 * L
                allowed = valid & (is_memkey | (rr >= 24) | (kx <= rr + 8))
            else:
                dk = (cc - 2 * L) & 15
                cur = (rr < L) & (cc < 2 * L)
                old = (rr >= L) & (cc >= 2 * L) & (cc < 2 * L + 32)
                valid = cur | old
                allowed = ((cur & (is_memkey | (rr >= SEG) | (kx <= rr)))
                           | (old & ((dk >= 8) | (dk <= rr - L))))
            return is_a, allowed, jnp.where(valid, NEG, -jnp.inf).astype(F32)

        all_masks = {True: masks(True), False: masks(False)}

        def lo64(y):
            return _iota(y.shape, 1) < 64

        def stack_keys(a, b):
            parts = [a[0:L], b[SEG:L], b[0:SEG]]
            if a.shape[0] > L:
                parts += [a[L:], b[L:]]
            return jnp.concatenate(parts, axis=0).astype(BF16)

        def expand(y):
            y0, y1, y2 = y[:, 0:128], y[:, 128:256], y[:, 256:384]
            return (stack_keys(y0, y2),
                    stack_keys(jnp.where(lo64(y1), y1, 0.0), jnp.where(lo64(y1), 0.0, y1)))

        def pad_lanes(s):
            return jnp.concatenate([s, jnp.zeros((s.shape[0], 128 - s.shape[1]), F32)], axis=1)

        def step(hq, hkv, even, kmajor, side=None, never=None):
            is_a, allowed, fill = all_masks[even]
            nrow = SEG if even else L + 8
            nkey = 2 * L if even else 2 * L + 32

            def tiles(j, ts):
                return jnp.concatenate([pltpu.bitcast(wb[9 * j + t], BF16) for t in ts], axis=1)

            def proj(j):
                if j == 0 and kmajor:
                    wq, wkv = tiles(j, range(3)), tiles(j, range(3, 9))
                    q = _dot(hq[:, 0:128], wq[0:128])
                    y = _dot(hkv[:, 0:128], wkv[0:128])
                    for t in range(1, 5):
                        ks = slice(128 * t, 128 * (t + 1))
                        q = _dot(hq[:, ks], wq[ks]) + q
                        y = _dot(hkv[:, ks], wkv[ks]) + y
                else:
                    q = _dot(hq, tiles(j, range(3)))
                    y = _dot(hkv, tiles(j, range(3, 9)))
                if even:
                    snext[j] = y[SEG:L]
                    sdef[j, 0:8, :] = y[0:8]
                    sdef[j, 8:16, :] = y[L:L + 8]
                    kv = jnp.concatenate([y[0:SEG], y[L:L + 8]], axis=0)
                else:
                    kv = jnp.concatenate([snext[j], y, sdef[j]], axis=0)
                q = q.astype(BF16)
                q = (jnp.concatenate([q[:, 0:128], q[:, 256:384]], axis=0), q[:, 128:256])
                return q, expand(kv[:, 0:384]), expand(kv[:, 384:768])

            def scores(q, k, tok=None):
                s02 = pad_lanes(_dot_nt(q[0], k[0]))
                s = jnp.where(is_a, s02[0:nrow], s02[nrow:]) + pad_lanes(_dot_nt(q[1], k[1]))
                s = jnp.where(allowed, s * scale, fill)
                ma = jnp.max(jnp.where(is_a, s, -jnp.inf), axis=1, keepdims=True)
                mb = jnp.max(jnp.where(is_a, -jnp.inf, s), axis=1, keepdims=True)
                e = jnp.exp(s - jnp.where(is_a, ma, mb))
                ea = jnp.where(is_a, e, 0.0)
                eb = jnp.where(is_a, 0.0, e)
                pa = ea * (1.0 / jnp.sum(ea, axis=1, keepdims=True))
                pb = eb * (1.0 / jnp.sum(eb, axis=1, keepdims=True))
                if tok is not None:
                    pb = jnp.concatenate([jnp.where(never, tok, pb[0:16]), pb[16:]], axis=0)
                return (jnp.concatenate([pa, pb], axis=0)[:, 0:nkey].astype(BF16),
                        (pa + pb)[:, 0:nkey].astype(BF16))

            def pv(p, v):
                o02 = _dot(p[0], v[0])
                return jnp.concatenate(
                    [o02[0:nrow], _dot(p[1], v[1]), o02[nrow:]], axis=1).astype(BF16)

            qkv = [None] * NPAIR
            ps = [None] * NPAIR
            os_ = [None] * NPAIR

            def wo_chunk(c0, c1):
                w = pltpu.bitcast(bwo[192 * c0:192 * c1, :], BF16)
                return _dot(jnp.concatenate(os_[c0:c1], axis=1), w)

            cuts = (0, 4, 8, 11, 14, 16) if even else (11, 12, 13, 14, 15, 16)
            lag = NPAIR - 1 - cuts[0]
            qkv[0] = proj(0)
            acc = None
            for j in range(NPAIR + 2):
                c = None
                if j + 1 < NPAIR:
                    qkv[j + 1] = proj(j + 1)
                    if j >= lag:
                        c = wo_chunk(j - lag, j - lag + 1)
                else:
                    c = wo_chunk(cuts[j + 1 - NPAIR], cuts[j + 2 - NPAIR])
                if c is not None:
                    acc = c if acc is None else c + acc
                if j < NPAIR:
                    ps[j] = scores(qkv[j][0], qkv[j][1], side(j) if side else None)
                if j >= 2:
                    os_[j - 2] = pv(ps[j - 2], qkv[j - 2][2])
            acc = wo_chunk(cuts[3], cuts[4]) + acc
            return wo_chunk(cuts[4], cuts[5]) + acc

        def finish_rows(base, r0, n):
            rows = pl.ds(base + r0, n)
            xnew = xres[rows, :] + opend[r0:r0 + n, :]
            xres[rows, :] = xnew
            xin[rows, :] = xnew.astype(BF16)
            y = _ln(xnew)
            xnb[pl.ds(pl.multiple_of(base // 2, RB // 2) + r0 // 2, n // 2), :] = pltpu.bitcast(
                y.astype(BF16), U32)
            return y

        def body(i, carry):
            base = pl.multiple_of(i * RB, RB)

            @pl.when(jnp.logical_and(layer == 1, i >= 2))
            def _():
                rows = pl.ds(pl.multiple_of((i - 2) * RB, RB), RB)
                pltpu.make_async_copy(xin.at[rows], out_hbm.at[rows], sems.at[0]).start()

            prev = pl.multiple_of(jnp.maximum(i - 1, 0) * RB, RB)
            nxt = pl.multiple_of(jnp.minimum(i + 1, S // RB - 1) * RB, RB)

            def token(y):
                return functools.reduce(
                    jnp.maximum, [y[:, 128 * t:128 * (t + 1)] for t in range(5)])

            def side_prev(j):
                if j % 2:
                    return None
                return token(finish_rows(prev, 8 * j, 16))

            def side_next(j):
                if j % 2:
                    return None
                rows = pl.ds(nxt + 8 * j, 16)
                y = _ln(xres[rows, :])
                xn32[rows, :] = y
                return token(y)

            sides = (side_prev, side_next)
            never = i < 0
            mem = memv[...]
            for u in range(UNROLL):
                r0 = 64 * u
                xr = lambda a, n: xn32[pl.ds(base + r0 + a, n), :]
                cat = lambda *p: jnp.concatenate(p, axis=0).astype(BF16)
                o0 = step(cat(xr(8, 24), mem), cat(xr(0, 40), mem), True, u > 0, sides[u], never)
                opend[r0 + 8:r0 + 32, :] = o0[0:24]
                mem = o0[24:32]
                o1 = step(cat(xr(32, 32), mem, xr(0, 8)), cat(xr(40, 24), mem), False, True)
                mem = o1[32:40]
                opend[r0:r0 + 8, :] = o1[40:48]
                opend[r0 + 32:r0 + 64, :] = o1[0:32]
            memv[...] = mem
            return carry

        jax.lax.fori_loop(0, S // RB, body, 0)

        @pl.when(layer == 0)
        def _():
            finish_rows(S - RB, 0, RB)

    def layer(l, carry):
        layer_a(l)
        layer_b(l)
        return carry

    jax.lax.fori_loop(0, 2, layer, 0)

    rows = pl.ds(S - 2 * RB, RB)
    pltpu.make_async_copy(xin.at[rows], out_hbm.at[rows], sems.at[0]).start()
    rows = pl.ds(S - RB, RB)
    xin[rows, :] = (xres[rows, :] + opend[...]).astype(BF16)
    pltpu.make_async_copy(xin.at[rows], out_hbm.at[rows], sems.at[0]).start()
    pltpu.make_async_copy(xin, out_hbm, sems.at[0]).wait()


@jax.jit
def pallas_interleave_layers__linear_kernel_hedgehog__memory_aug_recurrent_mem_tr__prompt_kernel(
    A_x: jax.Array,
    A_wqkv: jax.Array,
    A_w_phi: jax.Array,
    A_wo: jax.Array,
    B_x: jax.Array,
    B_mem0: jax.Array,
    B_Wq: jax.Array,
    B_Wk: jax.Array,
    B_Wv: jax.Array,
    B_Wo: jax.Array,
    B_seg_len: jax.Array,
):
    assert A_x.shape == (1, S, D) and B_mem0.shape == (1, NM, D) and B_Wq.shape == (D, HB, DB)
    tr = lambda w: jnp.transpose(w, (1, 2, 0)).reshape(HB * DB, D)
    any_spec = pl.BlockSpec(memory_space=pl.ANY)
    out = pl.pallas_call(
        _kernel,
        out_shape=jax.ShapeDtypeStruct((S, D), BF16),
        in_specs=[any_spec] * 9,
        out_specs=any_spec,
        scratch_shapes=[
            pltpu.VMEM((DA, DA, HA), BF16),
            pltpu.VMEM((NM, D), BF16),
            pltpu.VMEM((S, D), BF16),
            pltpu.VMEM((D, 3 * D), BF16),
            pltpu.VMEM((D, D), BF16),
            pltpu.VMEM((4, HB * DB, D), BF16),
            pltpu.VMEM((9 * NPAIR, D // 2, 128), U32),
            pltpu.VMEM((HB * DB // 2, D), U32),
            pltpu.VMEM((S, D), F32),
            pltpu.VMEM((S, D), F32),
            pltpu.VMEM((S // 2, D), U32),
            pltpu.VMEM((3, D // 2, D), U32),
            pltpu.VMEM((16, 48, 80), F32),
            pltpu.VMEM((16, 40, S), U32),
            pltpu.VMEM((S // 2, D), U32),
            pltpu.VMEM((NM, D), F32),
            pltpu.VMEM((NPAIR, 8, 6 * 128), F32),
            pltpu.VMEM((NPAIR, 16, 6 * 128), F32),
            pltpu.VMEM((64 * UNROLL, D), F32),
            pltpu.SemaphoreType.DMA((7,)),
            pltpu.SemaphoreType.DMA((NXC,)),
            pltpu.SemaphoreType.DMA((NOC,)),
        ],
        compiler_params=pltpu.CompilerParams(vmem_limit_bytes=120 * 1024 * 1024),
    )(A_x.reshape(S, D), A_wqkv, jnp.transpose(A_w_phi, (1, 2, 0)), A_wo,
      B_mem0.reshape(NM, D), tr(B_Wq), tr(B_Wk), tr(B_Wv), B_Wo.reshape(HB * DB, D))
    return out.reshape(1, S, D)
```

```python
import functools

import jax
import jax.numpy as jnp
import jax.experimental.pallas as pl
import jax.experimental.pallas.tpu as pltpu

F32 = jnp.float32
BF16 = jnp.bfloat16
U32 = jnp.uint32

S = 2048
D = 640
HA = 32
DA = 20
HB = 32
DB = 192
NM = 8
SEG = 32
NPAIR = HB // 2
NF = HA * (DA - 1)
TB = 512
TC = 512
UNROLL = 2
RB = 64 * UNROLL
NXC = 8
NOC = 8
LN_EPS = 1e-5

_NN = (((1,), (0,)), ((), ()))
_NT = (((1,), (1,)), ((), ()))


def _dot(a, b):
    return jax.lax.dot_general(a, b, _NN, preferred_element_type=F32)


def _dot_nt(a, b):
    return jax.lax.dot_general(a, b, _NT, preferred_element_type=F32)


def _ln(x):
    m = jnp.mean(x, axis=-1, keepdims=True)
    xc = x - m
    v = jnp.mean(xc * xc, axis=-1, keepdims=True)
    return xc * jax.lax.rsqrt(v + LN_EPS)


def _iota(shape, dim):
    return jax.lax.broadcasted_iota(jnp.int32, shape, dim)


def _div20(i):
    return (i * 3277) >> 16


def _div40(i):
    return _div20(i) >> 1


def _kernel(x_hbm, wqkv_hbm, wphi_hbm, wo_hbm, mem0_hbm, wqt_hbm, wkt_hbm, wvt_hbm, bwo_hbm,
            out_hbm,
            wphi_ref, mem0_ref, xin, wqkv, woa, wt, wb, bwo, xres, xn32, xnb, wat, kvacc, phiq, obuf,
            memv, snext, sdef, opend, sems, xsems, osems):
    XC = S // NXC
    cp_phi = pltpu.make_async_copy(wphi_hbm, wphi_ref, sems.at[0])
    cp_wqkv = pltpu.make_async_copy(wqkv_hbm, wqkv, sems.at[1])

    def cp_x(c):
        rows = pl.ds(pl.multiple_of(c * XC, XC), XC)
        return pltpu.make_async_copy(x_hbm.at[rows], xin.at[rows], xsems.at[c])

    cp_wo = pltpu.make_async_copy(wo_hbm, woa, sems.at[2])
    cp_mem = pltpu.make_async_copy(mem0_hbm, mem0_ref, sems.at[3])
    cp_big = [
        pltpu.make_async_copy(wqt_hbm, wt.at[0], sems.at[4]),
        pltpu.make_async_copy(wkt_hbm, wt.at[1], sems.at[5]),
        pltpu.make_async_copy(wvt_hbm, wt.at[2], sems.at[6]),
    ]
    OC = HB * DB // NOC

    def cp_bwo(c):
        rows = pl.ds(pl.multiple_of(c * OC, OC), OC)
        return pltpu.make_async_copy(bwo_hbm.at[rows], wt.at[3, rows], osems.at[c])

    def start_first(c, carry):
        @pl.when(c == 0)
        def _():
            cp_phi.start()

        @pl.when(c == 1)
        def _():
            cp_wqkv.start()

        @pl.when(c >= 2)
        def _():
            cp_x(c - 2).start()

        return carry

    jax.lax.fori_loop(0, NXC + 2, start_first, 0)
    cp_phi.wait()

    wphi = wphi_ref[...].astype(F32)
    xw = jnp.concatenate([wphi[d] for d in range(DA)], axis=1)
    xw = jnp.concatenate([xw, jnp.zeros((32 - DA, D), F32)], axis=0).astype(BF16)
    r = _iota((D, D), 0)
    c = _iota((D, D), 1)
    perm = jnp.where((r & 31) * DA + (r >> 5) == c, 1.0, 0.0).astype(BF16)
    wf = _dot(xw, perm).astype(BF16)
    r = _iota((160, 32), 0)
    c = _iota((160, 32), 1)
    rsel = jnp.where(((r - _div40(r) * 40) >> 1) == c, 1.0, 0.0).astype(BF16)
    r = _iota((160, 128), 0)
    c = _iota((160, 128), 1)
    phit = []
    for t in range(5):
        keep = 2 * (_div40(r) + 3 * t) + (r & 1) == _div20(c + 128 * t)
        phit.append(jnp.where(keep, _dot(rsel, wf[:, 128 * t:128 * (t + 1)]), 0.0).astype(BF16))

    kvacc[...] = jnp.zeros_like(kvacc)

    def clear_slot(c, carry):
        wt[3, pl.ds(pl.multiple_of(c * 384, 384), 384), :] = jnp.zeros((384, D), BF16)
        return carry

    jax.lax.fori_loop(0, NPAIR // 2, clear_slot, 0)
    cp_wqkv.wait()
    cp_big[0].start()
    for m, dst in ((1, 0), (0, 1)):
        p = [_dot_nt(phit[t], wqkv[:, m * D + 128 * t:m * D + 128 * (t + 1)]) for t in range(5)]
        rows = [p[0][0:120]]
        for t in range(1, 5):
            rows += [p[t - 1][120:160] + p[t][0:40], p[t][40:120]]
        rows.append(p[4][120:160])
        w = jnp.concatenate(rows, axis=0)
        sub = _iota((8, D), 0)
        groups = []
        for j in range(16):
            ref = jnp.where(sub < 2, w[40 * j:40 * j + 8], 0.0)
            ref = ref + pltpu.roll(ref, 2, 0)
            ref = ref + pltpu.roll(ref, 4, 0)
            groups.append([w[40 * j + 8 * t:40 * j + 8 * (t + 1)] - ref for t in range(5)])
        rows = []
        for g in range(4):
            for t in range(3):
                rows.append(jnp.where(sub < 2, pltpu.roll(groups[4 * g + 3][0], 6 - 2 * t, 0),
                                      groups[4 * g + t][0]))
            for t in range(4):
                rows += groups[4 * g + t][1:]
        wat[dst, 0:NF // 2, :] = pltpu.bitcast(jnp.concatenate(rows, axis=0).astype(BF16), U32)
    wat[2] = pltpu.bitcast(wqkv[:, 2 * D:3 * D].T, U32)

    def init_blk(i, carry):
        cp_x(i).wait()
        for u in range(XC // 64):
            off = pl.multiple_of(i * XC + u * 64, 64)
            x = xin[pl.ds(off, 64), :].astype(F32)
            xres[pl.ds(off, 64), :] = x
            xnb[pl.ds(pl.multiple_of(off // 2, 32), 32), :] = pltpu.bitcast(_ln(x).astype(BF16), U32)
        return carry

    jax.lax.fori_loop(0, NXC, init_blk, 0)
    cp_big[1].start()

    def transpose_tiles(src, dst, j0, n):
        for j in range(n):
            for t in range(3):
                off = (j0 + j) * 384 + t * 128
                if not isinstance(off, int):
                    off = pl.multiple_of(off, 128)
                wb[9 * (j0 + j) + 3 * dst + t] = pltpu.bitcast(wt[src, pl.ds(off, 128), :].T, U32)

    def layer_a(l):
        def sub_all(x, op):
            x = op(x, pltpu.roll(x, 2, 0))
            return op(x, pltpu.roll(x, 4, 0))

        def features(m, x):
            p = _dot_nt(pltpu.bitcast(wat[m, 0:NF // 2, :], BF16), x)
            p = [p[8 * t:8 * (t + 1)] for t in range(NF // 8)]
            sub = _iota((8, 128), 0)
            out = []
            for j in range(16):
                g, t = divmod(j, 4)
                pg = p[19 * g:19 * (g + 1)]
                if t < 3:
                    head = pg[t]
                else:
                    head = jnp.where(sub < 4, pltpu.roll(pg[0], 2, 0),
                                     jnp.where(sub < 6, pltpu.roll(pg[1], 4, 0),
                                               pltpu.roll(pg[2], 6, 0)))
                out.append([jnp.where(sub < 2, 0.0, head)] + pg[3 + 4 * t:7 + 4 * t])
            return out

        def phi(ts):
            mx = sub_all(functools.reduce(jnp.maximum, ts), jnp.maximum)
            mn = sub_all(functools.reduce(jnp.minimum, ts), jnp.minimum)
            ep = [jnp.exp(t - mx) for t in ts]
            en = [jnp.exp(mn - t) for t in ts]
            rp = 1.0 / sub_all(functools.reduce(jnp.add, ep), jnp.add)
            rn = 1.0 / sub_all(functools.reduce(jnp.add, en), jnp.add)
            return jnp.concatenate([e * rp for e in ep] + [e * rn for e in en], axis=0).astype(BF16)

        def phase1(i, carry):
            @pl.when(jnp.logical_and(l == 0, i == 0))
            def _():
                cp_wo.start()
                cp_mem.start()

            @pl.when(jnp.logical_and(l == 0, i == 1))
            def _():
                cp_big[2].start()

            @pl.when(jnp.logical_and(l == 0, i == 2))
            def _():
                for c in range(NOC):
                    cp_bwo(c).start()
                cp_big[0].wait()

            transpose_tiles(jnp.where(i < 2, 3, 0), 0, jnp.where(i == 3, NPAIR // 2, 0), NPAIR // 2)
            off = pl.multiple_of(i * TB, TB)
            xn = pltpu.bitcast(xnb[pl.ds(pl.multiple_of(i * (TB // 2), TB // 2), TB // 2), :], BF16)
            xs = [xn[128 * u:128 * (u + 1)] for u in range(TB // 128)]
            for u, x in enumerate(xs):
                for j, ts in enumerate(features(1, x)):
                    phiq[j, :, pl.ds(off + 128 * u, 128)] = pltpu.bitcast(phi(ts), U32)
            phik = [[phi(ts) for ts in features(0, x)] for x in xs]
            vt = [_dot_nt(pltpu.bitcast(wat[2], BF16), x) for x in xs]
            ones = jnp.ones((8, 128), F32)
            for u in range(len(xs)):
                for j in range(16):
                    lhs = jnp.concatenate([vt[u][40 * j:40 * (j + 1)], ones], axis=0).astype(BF16)
                    kvacc[j] = _dot_nt(lhs, phik[u][j]) + kvacc[j]
            return carry

        jax.lax.fori_loop(0, S // TB, phase1, 0)

        rr = _iota((48, 80), 0)
        cc = _iota((48, 80), 1)
        keep = jnp.where(rr < 40, _div20(rr), (rr - 40) >> 2) == (cc & 1)
        kvm = [jnp.where(keep, kvacc[j], 0.0).astype(BF16) for j in range(16)]
        lo4 = _iota((8, TC), 0) < 4

        def num(b):
            parts = []
            for j in range(16):
                r = _dot(kvm[j], pltpu.bitcast(phiq[j, :, TC * b:TC * (b + 1)], BF16))
                rc = 1.0 / (r[40:48] + 1e-6)
                rc2 = pltpu.roll(rc, 4, 0)
                ra = jnp.where(lo4, rc, rc2)
                rb = jnp.where(lo4, rc2, rc)
                parts += [r[0:8] * ra, r[8:16] * ra, r[16:24] * rc, r[24:32] * rb, r[32:40] * rb]
            return jnp.concatenate(parts, axis=0).astype(BF16).T

        for b in range(S // TC):
            obuf[TC // 2 * b:TC // 2 * (b + 1), :] = pltpu.bitcast(num(b), U32)

        @pl.when(l == 0)
        def _():
            cp_wo.wait()
            cp_mem.wait()
            cp_big[1].wait()

        def out(i, carry):
            @pl.when(jnp.logical_and(l == 0, i == 2))
            def _():
                cp_big[2].wait()

            m = 1 + (i >> 1)
            transpose_tiles(m, m, (i & 1) * (NPAIR // 2), NPAIR // 2)
            xn32[0:RB, :] = _ln(xres[0:RB, :])
            memv[...] = mem0_ref[...].astype(F32)
            opend[...] = jnp.zeros_like(opend)
            kvacc[...] = jnp.zeros_like(kvacc)
            rows = pl.ds(pl.multiple_of(i * TB, TB), TB)
            o = pltpu.bitcast(obuf[pl.ds(pl.multiple_of(i * (TB // 2), TB // 2), TB // 2), :], BF16)
            xres[rows, :] = _dot(o, woa[...]) + xres[rows, :]
            return carry

        jax.lax.fori_loop(0, S // TB, out, 0)

        @pl.when(l == 0)
        def _():
            def cpo(c, carry):
                cp_bwo(c).wait()
                for u in range(OC // 384):
                    off = pl.multiple_of(c * OC + u * 384, 384)
                    bwo[pl.ds(pl.multiple_of(off // 2, 192), 192), :] = pltpu.bitcast(
                        wt[3, pl.ds(off, 384), :], U32)
                return carry

            jax.lax.fori_loop(0, NOC, cpo, 0)

    scale = DB ** (-0.5)

    def layer_b(layer):
        L = SEG + NM
        NEG = -1000000000.0

        def masks(even):
            nrow = SEG if even else L + 8
            rr = _iota((nrow, 128), 0)
            cc = _iota((nrow, 128), 1)
            is_a = (cc < L) | ((cc >= 2 * L) & (cc < 2 * L + 16))
            kx = jnp.where(cc < L, cc, cc - (L + NM))
            is_memkey = (cc >= SEG) & (cc < SEG + 2 * NM)
            if even:
                valid = cc < 2 * L
                allowed = valid & (is_memkey | (rr >= 24) | (kx <= rr + 8))
            else:
                dk = (cc - 2 * L) & 15
                cur = (rr < L) & (cc < 2 * L)
                old = (rr >= L) & (cc >= 2 * L) & (cc < 2 * L + 32)
                valid = cur | old
                allowed = ((cur & (is_memkey | (rr >= SEG) | (kx <= rr)))
                           | (old & ((dk >= 8) | (dk <= rr - L))))
            return is_a, allowed, jnp.where(valid, NEG, -jnp.inf).astype(F32)

        all_masks = {True: masks(True), False: masks(False)}

        def lo64(y):
            return _iota(y.shape, 1) < 64

        def stack_keys(a, b):
            parts = [a[0:L], b[SEG:L], b[0:SEG]]
            if a.shape[0] > L:
                parts += [a[L:], b[L:]]
            return jnp.concatenate(parts, axis=0).astype(BF16)

        def expand(y):
            y0, y1, y2 = y[:, 0:128], y[:, 128:256], y[:, 256:384]
            return (stack_keys(y0, y2),
                    stack_keys(jnp.where(lo64(y1), y1, 0.0), jnp.where(lo64(y1), 0.0, y1)))

        def pad_lanes(s):
            return jnp.concatenate([s, jnp.zeros((s.shape[0], 128 - s.shape[1]), F32)], axis=1)

        def step(hq, hkv, even, kmajor, side=None, never=None):
            is_a, allowed, fill = all_masks[even]
            nrow = SEG if even else L + 8
            nkey = 2 * L if even else 2 * L + 32

            def tiles(j, ts):
                return jnp.concatenate([pltpu.bitcast(wb[9 * j + t], BF16) for t in ts], axis=1)

            def proj(j):
                if j == 0 and kmajor:
                    wq, wkv = tiles(j, range(3)), tiles(j, range(3, 9))
                    q = _dot(hq[:, 0:128], wq[0:128])
                    y = _dot(hkv[:, 0:128], wkv[0:128])
                    for t in range(1, 5):
                        ks = slice(128 * t, 128 * (t + 1))
                        q = _dot(hq[:, ks], wq[ks]) + q
                        y = _dot(hkv[:, ks], wkv[ks]) + y
                else:
                    q = _dot(hq, tiles(j, range(3)))
                    y = _dot(hkv, tiles(j, range(3, 9)))
                if even:
                    snext[j] = y[SEG:L]
                    sdef[j, 0:8, :] = y[0:8]
                    sdef[j, 8:16, :] = y[L:L + 8]
                    kv = jnp.concatenate([y[0:SEG], y[L:L + 8]], axis=0)
                else:
                    kv = jnp.concatenate([snext[j], y, sdef[j]], axis=0)
                q = q.astype(BF16)
                q = (jnp.concatenate([q[:, 0:128], q[:, 256:384]], axis=0), q[:, 128:256])
                return q, expand(kv[:, 0:384]), expand(kv[:, 384:768])

            def scores(q, k, tok=None):
                s02 = pad_lanes(_dot_nt(q[0], k[0]))
                s = jnp.where(is_a, s02[0:nrow], s02[nrow:]) + pad_lanes(_dot_nt(q[1], k[1]))
                s = jnp.where(allowed, s * scale, fill)
                ma = jnp.max(jnp.where(is_a, s, -jnp.inf), axis=1, keepdims=True)
                mb = jnp.max(jnp.where(is_a, -jnp.inf, s), axis=1, keepdims=True)
                e = jnp.exp(s - jnp.where(is_a, ma, mb))
                ea = jnp.where(is_a, e, 0.0)
                eb = jnp.where(is_a, 0.0, e)
                pa = ea * (1.0 / jnp.sum(ea, axis=1, keepdims=True))
                pb = eb * (1.0 / jnp.sum(eb, axis=1, keepdims=True))
                if tok is not None:
                    pb = jnp.concatenate([jnp.where(never, tok, pb[0:16]), pb[16:]], axis=0)
                return (jnp.concatenate([pa, pb], axis=0)[:, 0:nkey].astype(BF16),
                        (pa + pb)[:, 0:nkey].astype(BF16))

            def pv(p, v):
                o02 = _dot(p[0], v[0])
                return jnp.concatenate(
                    [o02[0:nrow], _dot(p[1], v[1]), o02[nrow:]], axis=1).astype(BF16)

            qkv = [None] * NPAIR
            ps = [None] * NPAIR
            os_ = [None] * NPAIR

            def wo_chunk(c0, c1):
                w = pltpu.bitcast(bwo[192 * c0:192 * c1, :], BF16)
                return _dot(jnp.concatenate(os_[c0:c1], axis=1), w)

            cuts = (0, 4, 8, 11, 14, 16) if even else (11, 12, 13, 14, 15, 16)
            lag = NPAIR - 1 - cuts[0]
            qkv[0] = proj(0)
            acc = None
            for j in range(NPAIR + 2):
                c = None
                if j + 1 < NPAIR:
                    qkv[j + 1] = proj(j + 1)
                    if j >= lag:
                        c = wo_chunk(j - lag, j - lag + 1)
                else:
                    c = wo_chunk(cuts[j + 1 - NPAIR], cuts[j + 2 - NPAIR])
                if c is not None:
                    acc = c if acc is None else c + acc
                if j < NPAIR:
                    ps[j] = scores(qkv[j][0], qkv[j][1], side(j) if side else None)
                if j >= 2:
                    os_[j - 2] = pv(ps[j - 2], qkv[j - 2][2])
            acc = wo_chunk(cuts[3], cuts[4]) + acc
            return wo_chunk(cuts[4], cuts[5]) + acc

        def finish_rows(base, r0, n):
            rows = pl.ds(base + r0, n)
            xnew = xres[rows, :] + opend[r0:r0 + n, :]
            xres[rows, :] = xnew
            xin[rows, :] = xnew.astype(BF16)
            y = _ln(xnew)
            xnb[pl.ds(pl.multiple_of(base // 2, RB // 2) + r0 // 2, n // 2), :] = pltpu.bitcast(
                y.astype(BF16), U32)
            return y

        def body(i, carry):
            base = pl.multiple_of(i * RB, RB)

            @pl.when(jnp.logical_and(layer == 1, i >= 2))
            def _():
                rows = pl.ds(pl.multiple_of((i - 2) * RB, RB), RB)
                pltpu.make_async_copy(xin.at[rows], out_hbm.at[rows], sems.at[0]).start()

            prev = pl.multiple_of(jnp.maximum(i - 1, 0) * RB, RB)
            nxt = pl.multiple_of(jnp.minimum(i + 1, S // RB - 1) * RB, RB)

            def token(y):
                return functools.reduce(
                    jnp.maximum, [y[:, 128 * t:128 * (t + 1)] for t in range(5)])

            def side_prev(j):
                if j % 2:
                    return None
                return token(finish_rows(prev, 8 * j, 16))

            def side_next(j):
                if j % 2:
                    return None
                rows = pl.ds(nxt + 8 * j, 16)
                y = _ln(xres[rows, :])
                xn32[rows, :] = y
                return token(y)

            sides = (side_prev, side_next)
            never = i < 0
            mem = memv[...]
            for u in range(UNROLL):
                r0 = 64 * u
                xr = lambda a, n: xn32[pl.ds(base + r0 + a, n), :]
                cat = lambda *p: jnp.concatenate(p, axis=0).astype(BF16)
                o0 = step(cat(xr(8, 24), mem), cat(xr(0, 40), mem), True, u > 0, sides[u], never)
                opend[r0 + 8:r0 + 32, :] = o0[0:24]
                mem = o0[24:32]
                o1 = step(cat(xr(32, 32), mem, xr(0, 8)), cat(xr(40, 24), mem), False, True)
                mem = o1[32:40]
                opend[r0:r0 + 8, :] = o1[40:48]
                opend[r0 + 32:r0 + 64, :] = o1[0:32]
            memv[...] = mem
            return carry

        jax.lax.fori_loop(0, S // RB, body, 0)

        @pl.when(layer == 0)
        def _():
            finish_rows(S - RB, 0, RB)

    def layer(l, carry):
        layer_a(l)
        layer_b(l)
        return carry

    jax.lax.fori_loop(0, 2, layer, 0)

    rows = pl.ds(S - 2 * RB, RB)
    pltpu.make_async_copy(xin.at[rows], out_hbm.at[rows], sems.at[0]).start()
    rows = pl.ds(S - RB, RB)
    xin[rows, :] = (xres[rows, :] + opend[...]).astype(BF16)
    pltpu.make_async_copy(xin.at[rows], out_hbm.at[rows], sems.at[0]).start()
    pltpu.make_async_copy(xin, out_hbm, sems.at[0]).wait()


@jax.jit
def pallas_interleave_layers__linear_kernel_hedgehog__memory_aug_recurrent_mem_tr__prompt_kernel(
    A_x: jax.Array,
    A_wqkv: jax.Array,
    A_w_phi: jax.Array,
    A_wo: jax.Array,
    B_x: jax.Array,
    B_mem0: jax.Array,
    B_Wq: jax.Array,
    B_Wk: jax.Array,
    B_Wv: jax.Array,
    B_Wo: jax.Array,
    B_seg_len: jax.Array,
):
    assert A_x.shape == (1, S, D) and B_mem0.shape == (1, NM, D) and B_Wq.shape == (D, HB, DB)
    tr = lambda w: jnp.transpose(w, (1, 2, 0)).reshape(HB * DB, D)
    any_spec = pl.BlockSpec(memory_space=pl.ANY)
    out = pl.pallas_call(
        _kernel,
        out_shape=jax.ShapeDtypeStruct((S, D), BF16),
        in_specs=[any_spec] * 9,
        out_specs=any_spec,
        scratch_shapes=[
            pltpu.VMEM((DA, DA, HA), BF16),
            pltpu.VMEM((NM, D), BF16),
            pltpu.VMEM((S, D), BF16),
            pltpu.VMEM((D, 3 * D), BF16),
            pltpu.VMEM((D, D), BF16),
            pltpu.VMEM((4, HB * DB, D), BF16),
            pltpu.VMEM((9 * NPAIR, D // 2, 128), U32),
            pltpu.VMEM((HB * DB // 2, D), U32),
            pltpu.VMEM((S, D), F32),
            pltpu.VMEM((S, D), F32),
            pltpu.VMEM((S // 2, D), U32),
            pltpu.VMEM((3, D // 2, D), U32),
            pltpu.VMEM((16, 48, 80), F32),
            pltpu.VMEM((16, 40, S), U32),
            pltpu.VMEM((S // 2, D), U32),
            pltpu.VMEM((NM, D), F32),
            pltpu.VMEM((NPAIR, 8, 6 * 128), F32),
            pltpu.VMEM((NPAIR, 16, 6 * 128), F32),
            pltpu.VMEM((64 * UNROLL, D), F32),
            pltpu.SemaphoreType.DMA((7,)),
            pltpu.SemaphoreType.DMA((NXC,)),
            pltpu.SemaphoreType.DMA((NOC,)),
        ],
        compiler_params=pltpu.CompilerParams(vmem_limit_bytes=120 * 1024 * 1024),
    )(A_x.reshape(S, D), A_wqkv, jnp.transpose(A_w_phi, (1, 2, 0)), A_wo,
      B_mem0.reshape(NM, D), tr(B_Wq), tr(B_Wk), tr(B_Wv), B_Wo.reshape(HB * DB, D))
    return out.reshape(1, S, D)
```

```python
import functools

import jax
import jax.numpy as jnp
import jax.experimental.pallas as pl
import jax.experimental.pallas.tpu as pltpu

F32 = jnp.float32
BF16 = jnp.bfloat16
U32 = jnp.uint32

S = 2048
D = 640
HA = 32
DA = 20
HB = 32
DB = 192
NM = 8
SEG = 32
NPAIR = HB // 2
NF = HA * (DA - 1)
TB = 512
TC = 512
UNROLL = 2
RB = 64 * UNROLL
NPRE = 3
JPRE = 8
NXC = S // TB
NOC = 8
LN_EPS = 1e-5

_NN = (((1,), (0,)), ((), ()))
_NT = (((1,), (1,)), ((), ()))


def _dot(a, b):
    return jax.lax.dot_general(a, b, _NN, preferred_element_type=F32)


def _dot_nt(a, b):
    return jax.lax.dot_general(a, b, _NT, preferred_element_type=F32)


def _ln(x):
    m = jnp.mean(x, axis=-1, keepdims=True)
    xc = x - m
    v = jnp.mean(xc * xc, axis=-1, keepdims=True)
    return xc * jax.lax.rsqrt(v + LN_EPS)


def _iota(shape, dim):
    return jax.lax.broadcasted_iota(jnp.int32, shape, dim)


def _div20(i):
    return (i * 3277) >> 16


def _div40(i):
    return _div20(i) >> 1


def _kernel(x_hbm, wqkv_hbm, wphi_hbm, wo_hbm, mem0_hbm, wqt_hbm, wkt_hbm, wvt_hbm, bwo_hbm,
            out_hbm,
            wphi_ref, mem0_ref, xin, wqkv, woa, wt, wb, bwo, xres, xn32, xnb, wat, kvacc, phiq,
            obuf, wpre, qpre, memv, snext, sdef, opend, sems, xsems, osems, wsems):
    XC = S // NXC
    cp_phi = pltpu.make_async_copy(wphi_hbm, wphi_ref, sems.at[0])

    def cp_w(m):
        cols = pl.ds(m * D, D)
        return pltpu.make_async_copy(wqkv_hbm.at[:, cols], wqkv.at[:, cols], wsems.at[m])

    def cp_x(c):
        rows = pl.ds(c * XC if isinstance(c, int) else pl.multiple_of(c * XC, XC), XC)
        return pltpu.make_async_copy(x_hbm.at[rows], xin.at[rows], xsems.at[c])

    cp_wo = pltpu.make_async_copy(wo_hbm, woa, sems.at[2])
    cp_mem = pltpu.make_async_copy(mem0_hbm, mem0_ref, sems.at[3])
    cp_big = [
        pltpu.make_async_copy(wqt_hbm, wt.at[0], sems.at[4]),
        pltpu.make_async_copy(wkt_hbm, wt.at[1], sems.at[5]),
        pltpu.make_async_copy(wvt_hbm, wt.at[2], sems.at[6]),
    ]
    OC = HB * DB // NOC

    def cp_bwo(c):
        rows = pl.ds(pl.multiple_of(c * OC, OC), OC)
        return pltpu.make_async_copy(bwo_hbm.at[rows], wt.at[3, rows], osems.at[c])

    def start_in_order(copies):
        def start(c, carry):
            for n, cp in enumerate(copies):
                pl.when(c == n)(cp.start)
            return carry

        jax.lax.fori_loop(0, len(copies), start, 0)

    start_in_order([cp_phi, cp_x(0), cp_w(0), cp_w(1), cp_w(2)] + [cp_x(c) for c in range(1, NXC)])
    cp_phi.wait()

    wphi = wphi_ref[...].astype(F32)
    xw = jnp.concatenate([wphi[d] for d in range(DA)], axis=1)
    xw = jnp.concatenate([xw, jnp.zeros((32 - DA, D), F32)], axis=0).astype(BF16)
    r = _iota((D, D), 0)
    c = _iota((D, D), 1)
    perm = jnp.where((r & 31) * DA + (r >> 5) == c, 1.0, 0.0).astype(BF16)
    wf = _dot(xw, perm).astype(BF16)
    r = _iota((160, 32), 0)
    c = _iota((160, 32), 1)
    rsel = jnp.where(((r - _div40(r) * 40) >> 1) == c, 1.0, 0.0).astype(BF16)
    r = _iota((160, 128), 0)
    c = _iota((160, 128), 1)
    phit = []
    for t in range(5):
        keep = 2 * (_div40(r) + 3 * t) + (r & 1) == _div20(c + 128 * t)
        phit.append(jnp.where(keep, _dot(rsel, wf[:, 128 * t:128 * (t + 1)]), 0.0).astype(BF16))

    kvacc[...] = jnp.zeros_like(kvacc)

    cp_x(0).wait()

    def init_blk(i, carry):
        for u in range(4):
            off = pl.multiple_of(i * 256 + u * 64, 64)
            x = xin[pl.ds(off, 64), :].astype(F32)
            xres[pl.ds(off, 64), :] = x
            xnb[pl.ds(pl.multiple_of(off // 2, 32), 32), :] = pltpu.bitcast(_ln(x).astype(BF16), U32)
        return carry

    jax.lax.fori_loop(0, XC // 256, init_blk, 0)
    start_in_order([cp_big[0], cp_big[1], cp_wo, cp_mem, cp_big[2]])

    def start_bwo(c, carry):
        cp_bwo(c).start()
        return carry

    jax.lax.fori_loop(0, NOC, start_bwo, 0)
    for m, dst in ((0, 1), (1, 0)):
        cp_w(m).wait()
        p = [_dot_nt(phit[t], wqkv[:, m * D + 128 * t:m * D + 128 * (t + 1)]) for t in range(5)]
        rows = [p[0][0:120]]
        for t in range(1, 5):
            rows += [p[t - 1][120:160] + p[t][0:40], p[t][40:120]]
        rows.append(p[4][120:160])
        w = jnp.concatenate(rows, axis=0)
        sub = _iota((8, D), 0)
        groups = []
        for j in range(16):
            ref = jnp.where(sub < 2, w[40 * j:40 * j + 8], 0.0)
            ref = ref + pltpu.roll(ref, 2, 0)
            ref = ref + pltpu.roll(ref, 4, 0)
            groups.append([w[40 * j + 8 * t:40 * j + 8 * (t + 1)] - ref for t in range(5)])
        rows = []
        for g in range(4):
            for t in range(3):
                rows.append(jnp.where(sub < 2, pltpu.roll(groups[4 * g + 3][0], 6 - 2 * t, 0),
                                      groups[4 * g + t][0]))
            for t in range(4):
                rows += groups[4 * g + t][1:]
        wat[dst, 0:NF // 2, :] = pltpu.bitcast(jnp.concatenate(rows, axis=0).astype(BF16), U32)
    cp_w(2).wait()
    wat[2] = pltpu.bitcast(wqkv[:, 2 * D:3 * D].T, U32)

    def weight_tile(m, j, t):
        off = j * 384 + t * 128
        if not isinstance(off, int):
            off = pl.multiple_of(off, 128)
        return pltpu.bitcast(wt[m, pl.ds(off, 128), :].T, U32)

    def layer_a(l):
        def sub_all(x, op):
            x = op(x, pltpu.roll(x, 2, 0))
            return op(x, pltpu.roll(x, 4, 0))

        def features(m, x):
            p = _dot_nt(pltpu.bitcast(wat[m, 0:NF // 2, :], BF16), x)
            p = [p[8 * t:8 * (t + 1)] for t in range(NF // 8)]
            sub = _iota((8, 128), 0)
            out = []
            for j in range(16):
                g, t = divmod(j, 4)
                pg = p[19 * g:19 * (g + 1)]
                if t < 3:
                    head = pg[t]
                else:
                    head = jnp.where(sub < 4, pltpu.roll(pg[0], 2, 0),
                                     jnp.where(sub < 6, pltpu.roll(pg[1], 4, 0),
                                               pltpu.roll(pg[2], 6, 0)))
                out.append([jnp.where(sub < 2, 0.0, head)] + pg[3 + 4 * t:7 + 4 * t])
            return out

        def phi(ts):
            mx = sub_all(functools.reduce(jnp.maximum, ts), jnp.maximum)
            mn = sub_all(functools.reduce(jnp.minimum, ts), jnp.minimum)
            ep = [jnp.exp(t - mx) for t in ts]
            en = [jnp.exp(mn - t) for t in ts]
            rp = 1.0 / sub_all(functools.reduce(jnp.add, ep), jnp.add)
            rn = 1.0 / sub_all(functools.reduce(jnp.add, en), jnp.add)
            return jnp.concatenate([e * rp for e in ep] + [e * rn for e in en], axis=0).astype(BF16)

        def phase1(i, carry):
            @pl.when(jnp.logical_and(l == 0, i < NXC - 1))
            def _():
                cp_x(i + 1).wait()

            off = pl.multiple_of(i * TB, TB)
            xn = pltpu.bitcast(xnb[pl.ds(pl.multiple_of(i * (TB // 2), TB // 2), TB // 2), :], BF16)
            xs = [xn[128 * u:128 * (u + 1)] for u in range(TB // 128)]
            nblk = jnp.minimum(i + 1, S // TB - 1)
            nrows = pl.ds(pl.multiple_of(nblk * TB, TB), TB)
            xnext = jnp.where(l == 0, xin[nrows, :].astype(F32), xres[nrows, :])
            ys = [_ln(xnext[16 * k:16 * (k + 1)]).astype(BF16) for k in range(TB // 16)]
            xres[nrows, :] = xnext
            xnb[pl.ds(pl.multiple_of(nblk * (TB // 2), TB // 2), TB // 2), :] = pltpu.bitcast(
                jnp.concatenate(ys, axis=0), U32)

            for u, x in enumerate(xs):
                for j, ts in enumerate(features(1, x)):
                    phiq[j, :, pl.ds(off + 128 * u, 128)] = pltpu.bitcast(phi(ts), U32)
            phik = [[phi(ts) for ts in features(0, x)] for x in xs]
            vt = [_dot_nt(pltpu.bitcast(wat[2], BF16), x) for x in xs]
            ones = jnp.ones((8, 128), F32)
            for u in range(len(xs)):
                for j in range(16):
                    lhs = jnp.concatenate([vt[u][40 * j:40 * (j + 1)], ones], axis=0).astype(BF16)
                    kvacc[j] = _dot_nt(lhs, phik[u][j]) + kvacc[j]
            return carry

        jax.lax.fori_loop(0, S // TB, phase1, 0)

        @pl.when(l == 0)
        def _():
            cp_big[0].wait()
            cp_big[1].wait()
            cp_wo.wait()
            cp_mem.wait()

        rr = _iota((48, 80), 0)
        cc = _iota((48, 80), 1)
        keep = jnp.where(rr < 40, _div20(rr), (rr - 40) >> 2) == (cc & 1)
        kvm = [jnp.where(keep, kvacc[j], 0.0).astype(BF16) for j in range(16)]
        lo4 = _iota((8, TC), 0) < 4
        opend[...] = jnp.zeros_like(opend)
        kvacc[...] = jnp.zeros_like(kvacc)
        for j in range(NPRE):
            for t in range(3):
                wpre[3 * j + t] = weight_tile(0, JPRE + j, t)

        def num(b):
            parts = []
            for j in range(16):
                r = _dot(kvm[j], pltpu.bitcast(phiq[j, :, TC * b:TC * (b + 1)], BF16))
                rc = 1.0 / (r[40:48] + 1e-6)
                rc2 = pltpu.roll(rc, 4, 0)
                ra = jnp.where(lo4, rc, rc2)
                rb = jnp.where(lo4, rc2, rc)
                parts += [r[0:8] * ra, r[8:16] * ra, r[16:24] * rc, r[24:32] * rb, r[32:40] * rb]
            return jnp.concatenate(parts, axis=0).astype(BF16).T

        for b in range(S // TC):
            obuf[TC // 2 * b:TC // 2 * (b + 1), :] = pltpu.bitcast(num(b), U32)

        def out(i, carry):
            @pl.when(jnp.logical_and(l == 0, i == 2))
            def _():
                cp_big[2].wait()

            for n in range(3 * NPAIR // 4):
                unit = i * (3 * NPAIR // 4) + n
                m, j = unit >> 4, unit & (NPAIR - 1)
                for t in range(3):
                    wb[9 * j + 3 * m + t] = weight_tile(m, j, t)
            xn32[0:RB, :] = _ln(xres[0:RB, :])
            rows = pl.ds(pl.multiple_of(i * TB, TB), TB)
            o = pltpu.bitcast(obuf[pl.ds(pl.multiple_of(i * (TB // 2), TB // 2), TB // 2), :], BF16)
            x = xres[rows, :]
            nb = TB // 64
            pick = lambda y, gs: jnp.concatenate([y[16 * g:16 * (g + 1)] for g in gs], axis=0)
            first = [g for g in range(4 * nb) if g % 4 == 2]
            rest = [g for g in range(4 * nb) if g % 4 != 2]
            xs = _dot(pick(o, first), woa[...]) + pick(x, first)
            memv[...] = mem0_ref[...].astype(F32)
            xo = _dot(pick(o, rest), woa[...]) + pick(x, rest)
            order = first + rest
            xres[rows, :] = pick(jnp.concatenate([xs, xo], axis=0),
                                 [order.index(g) for g in range(4 * nb)])
            wq = jnp.concatenate(
                [pltpu.bitcast(wpre[t], BF16) for t in range(3 * NPRE)], axis=1)
            qpre[pl.ds(pl.multiple_of(i * (8 * nb), 8 * nb), 8 * nb), :] = pltpu.bitcast(
                _dot(_ln(xs).astype(BF16), wq).astype(BF16), U32)
            return carry

        jax.lax.fori_loop(0, S // TB, out, 0)

        @pl.when(l == 0)
        def _():
            def cpo(c, carry):
                cp_bwo(c).wait()
                for u in range(OC // 384):
                    off = pl.multiple_of(c * OC + u * 384, 384)
                    bwo[pl.ds(pl.multiple_of(off // 2, 192), 192), :] = pltpu.bitcast(
                        wt[3, pl.ds(off, 384), :], U32)
                return carry

            jax.lax.fori_loop(0, NOC, cpo, 0)

    scale = DB ** (-0.5)

    def layer_b(layer):
        L = SEG + NM
        NEG = -1000000000.0

        def masks(even):
            nrow = SEG if even else L + 8
            rr = _iota((nrow, 128), 0)
            cc = _iota((nrow, 128), 1)
            is_a = (cc < L) | ((cc >= 2 * L) & (cc < 2 * L + 16))
            kx = jnp.where(cc < L, cc, cc - (L + NM))
            is_memkey = (cc >= SEG) & (cc < SEG + 2 * NM)
            if even:
                valid = cc < 2 * L
                allowed = valid & (is_memkey | (rr >= 24) | (kx <= rr + 8))
            else:
                dk = (cc - 2 * L) & 15
                cur = (rr < L) & (cc < 2 * L)
                old = (rr >= L) & (cc >= 2 * L) & (cc < 2 * L + 32)
                valid = cur | old
                allowed = ((cur & (is_memkey | (rr >= SEG) | (kx <= rr)))
                           | (old & ((dk >= 8) | (dk <= rr - L))))
            return is_a, allowed, jnp.where(valid, NEG, -jnp.inf).astype(F32)

        all_masks = {True: masks(True), False: masks(False)}

        def lo64(y):
            return _iota(y.shape, 1) < 64

        def stack_keys(a, b):
            parts = [a[0:L], b[SEG:L], b[0:SEG]]
            if a.shape[0] > L:
                parts += [a[L:], b[L:]]
            return jnp.concatenate(parts, axis=0).astype(BF16)

        def expand(y):
            y0, y1, y2 = y[:, 0:128], y[:, 128:256], y[:, 256:384]
            return (stack_keys(y0, y2),
                    stack_keys(jnp.where(lo64(y1), y1, 0.0), jnp.where(lo64(y1), 0.0, y1)))

        def pad_lanes(s):
            return jnp.concatenate([s, jnp.zeros((s.shape[0], 128 - s.shape[1]), F32)], axis=1)

        def step(hq, hkv, even, kmajor, side=None, never=None, pre=None):
            is_a, allowed, fill = all_masks[even]
            nrow = SEG if even else L + 8
            nkey = 2 * L if even else 2 * L + 32

            def tiles(j, ts):
                return jnp.concatenate([pltpu.bitcast(wb[9 * j + t], BF16) for t in ts], axis=1)

            def proj(j):
                if j == 0 and kmajor:
                    wq, wkv = tiles(j, range(3)), tiles(j, range(3, 9))
                    q = _dot(hq[:, 0:128], wq[0:128])
                    y = _dot(hkv[:, 0:128], wkv[0:128])
                    for t in range(1, 5):
                        ks = slice(128 * t, 128 * (t + 1))
                        q = _dot(hq[:, ks], wq[ks]) + q
                        y = _dot(hkv[:, ks], wkv[ks]) + y
                else:
                    ahead = pre is not None and JPRE <= j < JPRE + NPRE
                    q = _dot(hq[16:] if ahead else hq, tiles(j, range(3)))
                    y = _dot(hkv, tiles(j, range(3, 9)))
                if even:
                    snext[j] = y[SEG:L]
                    sdef[j, 0:8, :] = y[0:8]
                    sdef[j, 8:16, :] = y[L:L + 8]
                    kv = jnp.concatenate([y[0:SEG], y[L:L + 8]], axis=0)
                else:
                    kv = jnp.concatenate([snext[j], y, sdef[j]], axis=0)
                q = q.astype(BF16)
                if q.shape[0] < nrow:
                    c0 = 384 * (j - JPRE)
                    q = jnp.concatenate(
                        [pltpu.bitcast(qpre[pre, c0:c0 + 384], BF16), q], axis=0)
                q = (jnp.concatenate([q[:, 0:128], q[:, 256:384]], axis=0), q[:, 128:256])
                return q, expand(kv[:, 0:384]), expand(kv[:, 384:768])

            def scores(q, k, tok=None):
                s02 = pad_lanes(_dot_nt(q[0], k[0]))
                s = jnp.where(is_a, s02[0:nrow], s02[nrow:]) + pad_lanes(_dot_nt(q[1], k[1]))
                s = jnp.where(allowed, s * scale, fill)
                ma = jnp.max(jnp.where(is_a, s, -jnp.inf), axis=1, keepdims=True)
                mb = jnp.max(jnp.where(is_a, -jnp.inf, s), axis=1, keepdims=True)
                e = jnp.exp(s - jnp.where(is_a, ma, mb))
                ea = jnp.where(is_a, e, 0.0)
                eb = jnp.where(is_a, 0.0, e)
                pa = ea * (1.0 / jnp.sum(ea, axis=1, keepdims=True))
                pb = eb * (1.0 / jnp.sum(eb, axis=1, keepdims=True))
                if tok is not None:
                    pb = jnp.concatenate([jnp.where(never, tok, pb[0:16]), pb[16:]], axis=0)
                return (jnp.concatenate([pa, pb], axis=0)[:, 0:nkey].astype(BF16),
                        (pa + pb)[:, 0:nkey].astype(BF16))

            def pv(p, v):
                o02 = _dot(p[0], v[0])
                return jnp.concatenate(
                    [o02[0:nrow], _dot(p[1], v[1]), o02[nrow:]], axis=1).astype(BF16)

            qkv = [None] * NPAIR
            ps = [None] * NPAIR
            os_ = [None] * NPAIR

            def wo_chunk(c0, c1):
                w = pltpu.bitcast(bwo[192 * c0:192 * c1, :], BF16)
                return _dot(jnp.concatenate(os_[c0:c1], axis=1), w)

            cuts = (0, 4, 8, 11, 14, 16) if even else (11, 12, 13, 14, 15, 16)
            lag = NPAIR - 1 - cuts[0]
            qkv[0] = proj(0)
            acc = None
            for j in range(NPAIR + 2):
                c = None
                if j + 1 < NPAIR:
                    qkv[j + 1] = proj(j + 1)
                    if j >= lag:
                        c = wo_chunk(j - lag, j - lag + 1)
                else:
                    c = wo_chunk(cuts[j + 1 - NPAIR], cuts[j + 2 - NPAIR])
                if c is not None:
                    acc = c if acc is None else c + acc
                if j < NPAIR:
                    ps[j] = scores(qkv[j][0], qkv[j][1], side(j) if side else None)
                if j >= 2:
                    os_[j - 2] = pv(ps[j - 2], qkv[j - 2][2])
            acc = wo_chunk(cuts[3], cuts[4]) + acc
            return wo_chunk(cuts[4], cuts[5]) + acc

        def finish_rows(base, r0, n):
            rows = pl.ds(base + r0, n)
            xnew = xres[rows, :] + opend[r0:r0 + n, :]
            xres[rows, :] = xnew
            xin[rows, :] = xnew.astype(BF16)
            y = _ln(xnew)
            xnb[pl.ds(pl.multiple_of(base // 2, RB // 2) + r0 // 2, n // 2), :] = pltpu.bitcast(
                y.astype(BF16), U32)
            return y

        def body(i, carry):
            base = pl.multiple_of(i * RB, RB)

            @pl.when(jnp.logical_and(layer == 1, i >= 2))
            def _():
                rows = pl.ds(pl.multiple_of((i - 2) * RB, RB), RB)
                pltpu.make_async_copy(xin.at[rows], out_hbm.at[rows], sems.at[0]).start()

            prev = pl.multiple_of(jnp.maximum(i - 1, 0) * RB, RB)
            nxt = pl.multiple_of(jnp.minimum(i + 1, S // RB - 1) * RB, RB)

            def token(y):
                return functools.reduce(
                    jnp.maximum, [y[:, 128 * t:128 * (t + 1)] for t in range(5)])

            def side_prev(j):
                if j % 2:
                    return None
                return token(finish_rows(prev, 8 * j, 16))

            def side_next(j):
                if j % 2:
                    return None
                rows = pl.ds(nxt + 8 * j, 16)
                y = _ln(xres[rows, :])
                xn32[rows, :] = y
                return token(y)

            sides = (side_prev, side_next)
            never = i < 0
            mem = memv[...]
            for u in range(UNROLL):
                r0 = 64 * u
                xr = lambda a, n: xn32[pl.ds(base + r0 + a, n), :]
                cat = lambda *p: jnp.concatenate(p, axis=0).astype(BF16)
                o0 = step(cat(xr(8, 24), mem), cat(xr(0, 40), mem), True, u > 0, sides[u], never)
                opend[r0 + 8:r0 + 32, :] = o0[0:24]
                mem = o0[24:32]
                o1 = step(cat(xr(32, 32), mem, xr(0, 8)), cat(xr(40, 24), mem), False, True,
                          pre=pl.ds(pl.multiple_of(i * (8 * UNROLL), 8) + 8 * u, 8))
                mem = o1[32:40]
                opend[r0:r0 + 8, :] = o1[40:48]
                opend[r0 + 32:r0 + 64, :] = o1[0:32]
            memv[...] = mem
            return carry

        jax.lax.fori_loop(0, S // RB, body, 0)

        @pl.when(layer == 0)
        def _():
            xres[S - RB:S, :] = xres[S - RB:S, :] + opend[...]

    def layer(l, carry):
        layer_a(l)
        layer_b(l)
        return carry

    jax.lax.fori_loop(0, 2, layer, 0)

    rows = pl.ds(S - 2 * RB, RB)
    pltpu.make_async_copy(xin.at[rows], out_hbm.at[rows], sems.at[0]).start()
    rows = pl.ds(S - RB, RB)
    xin[rows, :] = (xres[rows, :] + opend[...]).astype(BF16)
    pltpu.make_async_copy(xin.at[rows], out_hbm.at[rows], sems.at[0]).start()
    pltpu.make_async_copy(xin, out_hbm, sems.at[0]).wait()


@jax.jit
def pallas_interleave_layers__linear_kernel_hedgehog__memory_aug_recurrent_mem_tr__prompt_kernel(
    A_x: jax.Array,
    A_wqkv: jax.Array,
    A_w_phi: jax.Array,
    A_wo: jax.Array,
    B_x: jax.Array,
    B_mem0: jax.Array,
    B_Wq: jax.Array,
    B_Wk: jax.Array,
    B_Wv: jax.Array,
    B_Wo: jax.Array,
    B_seg_len: jax.Array,
):
    assert A_x.shape == (1, S, D) and B_mem0.shape == (1, NM, D) and B_Wq.shape == (D, HB, DB)
    tr = lambda w: jnp.transpose(w, (1, 2, 0)).reshape(HB * DB, D)
    any_spec = pl.BlockSpec(memory_space=pl.ANY)
    out = pl.pallas_call(
        _kernel,
        out_shape=jax.ShapeDtypeStruct((S, D), BF16),
        in_specs=[any_spec] * 9,
        out_specs=any_spec,
        scratch_shapes=[
            pltpu.VMEM((DA, DA, HA), BF16),
            pltpu.VMEM((NM, D), BF16),
            pltpu.VMEM((S, D), BF16),
            pltpu.VMEM((D, 3 * D), BF16),
            pltpu.VMEM((D, D), BF16),
            pltpu.VMEM((4, HB * DB, D), BF16),
            pltpu.VMEM((9 * NPAIR, D // 2, 128), U32),
            pltpu.VMEM((HB * DB // 2, D), U32),
            pltpu.VMEM((S, D), F32),
            pltpu.VMEM((S, D), F32),
            pltpu.VMEM((S // 2, D), U32),
            pltpu.VMEM((3, D // 2, D), U32),
            pltpu.VMEM((16, 48, 80), F32),
            pltpu.VMEM((16, 40, S), U32),
            pltpu.VMEM((S // 2, D), U32),
            pltpu.VMEM((3 * NPRE, D // 2, 128), U32),
            pltpu.VMEM((S // 8, 384 * NPRE), U32),
            pltpu.VMEM((NM, D), F32),
            pltpu.VMEM((NPAIR, 8, 6 * 128), F32),
            pltpu.VMEM((NPAIR, 16, 6 * 128), F32),
            pltpu.VMEM((64 * UNROLL, D), F32),
            pltpu.SemaphoreType.DMA((7,)),
            pltpu.SemaphoreType.DMA((NXC,)),
            pltpu.SemaphoreType.DMA((NOC,)),
            pltpu.SemaphoreType.DMA((3,)),
        ],
        compiler_params=pltpu.CompilerParams(vmem_limit_bytes=120 * 1024 * 1024),
    )(A_x.reshape(S, D), A_wqkv, jnp.transpose(A_w_phi, (1, 2, 0)), A_wo,
      B_mem0.reshape(NM, D), tr(B_Wq), tr(B_Wk), tr(B_Wv), B_Wo.reshape(HB * DB, D))
    return out.reshape(1, S, D)
```

```python
import functools

import jax
import jax.numpy as jnp
import jax.experimental.pallas as pl
import jax.experimental.pallas.tpu as pltpu

F32 = jnp.float32
BF16 = jnp.bfloat16
U32 = jnp.uint32

S = 2048
D = 640
HA = 32
DA = 20
HB = 32
DB = 192
NM = 8
SEG = 32
NPAIR = HB // 2
NF = HA * (DA - 1)
TB = 512
TC = 512
UNROLL = 2
RB = 64 * UNROLL
NPRE = 3
JPRE = 8
NXC = S // TB
NOC = 8
LN_EPS = 1e-5

_NN = (((1,), (0,)), ((), ()))
_NT = (((1,), (1,)), ((), ()))


def _dot(a, b):
    return jax.lax.dot_general(a, b, _NN, preferred_element_type=F32)


def _dot_nt(a, b):
    return jax.lax.dot_general(a, b, _NT, preferred_element_type=F32)


def _ln(x):
    m = jnp.mean(x, axis=-1, keepdims=True)
    xc = x - m
    v = jnp.mean(xc * xc, axis=-1, keepdims=True)
    return xc * jax.lax.rsqrt(v + LN_EPS)


def _iota(shape, dim):
    return jax.lax.broadcasted_iota(jnp.int32, shape, dim)


def _div20(i):
    return (i * 3277) >> 16


def _div40(i):
    return _div20(i) >> 1


def _kernel(x_hbm, wqkv_hbm, wphi_hbm, wo_hbm, mem0_hbm, wqt_hbm, wkt_hbm, wvt_hbm, bwo_hbm,
            out_hbm,
            wphi_ref, mem0_ref, xin, wqkv, woa, wt, wb, bwo, xres, xn32, xnb, wat, kvacc, phiq,
            obuf, wpre, qpre, memv, snext, sdef, opend, sems, xsems, osems, wsems):
    XC = S // NXC
    cp_phi = pltpu.make_async_copy(wphi_hbm, wphi_ref, sems.at[0])

    def cp_w(m):
        cols = pl.ds(m * D, D)
        return pltpu.make_async_copy(wqkv_hbm.at[:, cols], wqkv.at[:, cols], wsems.at[m])

    def cp_x(c):
        rows = pl.ds(c * XC if isinstance(c, int) else pl.multiple_of(c * XC, XC), XC)
        return pltpu.make_async_copy(x_hbm.at[rows], xin.at[rows], xsems.at[c])

    cp_wo = pltpu.make_async_copy(wo_hbm, woa, sems.at[2])
    cp_mem = pltpu.make_async_copy(mem0_hbm, mem0_ref, sems.at[3])
    cp_big = [
        pltpu.make_async_copy(wqt_hbm, wt.at[0], sems.at[4]),
        pltpu.make_async_copy(wkt_hbm, wt.at[1], sems.at[5]),
        pltpu.make_async_copy(wvt_hbm, wt.at[2], sems.at[6]),
    ]
    OC = HB * DB // NOC

    def cp_bwo(c):
        rows = pl.ds(pl.multiple_of(c * OC, OC), OC)
        return pltpu.make_async_copy(bwo_hbm.at[rows], wt.at[3, rows], osems.at[c])

    def start_in_order(copies):
        def start(c, carry):
            for n, cp in enumerate(copies):
                pl.when(c == n)(cp.start)
            return carry

        jax.lax.fori_loop(0, len(copies), start, 0)

    start_in_order([cp_phi, cp_x(0), cp_w(0), cp_w(1), cp_w(2)] + [cp_x(c) for c in range(1, NXC)])
    cp_phi.wait()

    wphi = wphi_ref[...].astype(F32)
    xw = jnp.concatenate([wphi[d] for d in range(DA)], axis=1)
    xw = jnp.concatenate([xw, jnp.zeros((32 - DA, D), F32)], axis=0).astype(BF16)
    r = _iota((D, D), 0)
    c = _iota((D, D), 1)
    perm = jnp.where((r & 31) * DA + (r >> 5) == c, 1.0, 0.0).astype(BF16)
    wf = _dot(xw, perm).astype(BF16)
    r = _iota((160, 32), 0)
    c = _iota((160, 32), 1)
    rsel = jnp.where(((r - _div40(r) * 40) >> 1) == c, 1.0, 0.0).astype(BF16)
    r = _iota((160, 128), 0)
    c = _iota((160, 128), 1)
    phit = []
    for t in range(5):
        keep = 2 * (_div40(r) + 3 * t) + (r & 1) == _div20(c + 128 * t)
        phit.append(jnp.where(keep, _dot(rsel, wf[:, 128 * t:128 * (t + 1)]), 0.0).astype(BF16))

    kvacc[...] = jnp.zeros_like(kvacc)

    cp_x(0).wait()

    def init_blk(i, carry):
        for u in range(4):
            off = pl.multiple_of(i * 256 + u * 64, 64)
            x = xin[pl.ds(off, 64), :].astype(F32)
            xres[pl.ds(off, 64), :] = x
            xnb[pl.ds(pl.multiple_of(off // 2, 32), 32), :] = pltpu.bitcast(_ln(x).astype(BF16), U32)
        return carry

    jax.lax.fori_loop(0, XC // 256, init_blk, 0)
    start_in_order([cp_big[0], cp_big[1], cp_wo, cp_mem, cp_big[2]])

    def start_bwo(c, carry):
        cp_bwo(c).start()
        return carry

    jax.lax.fori_loop(0, NOC, start_bwo, 0)
    for m, dst in ((0, 1), (1, 0)):
        cp_w(m).wait()
        p = [_dot_nt(phit[t], wqkv[:, m * D + 128 * t:m * D + 128 * (t + 1)]) for t in range(5)]
        rows = [p[0][0:120]]
        for t in range(1, 5):
            rows += [p[t - 1][120:160] + p[t][0:40], p[t][40:120]]
        rows.append(p[4][120:160])
        w = jnp.concatenate(rows, axis=0)
        sub = _iota((8, D), 0)
        groups = []
        for j in range(16):
            ref = jnp.where(sub < 2, w[40 * j:40 * j + 8], 0.0)
            ref = ref + pltpu.roll(ref, 2, 0)
            ref = ref + pltpu.roll(ref, 4, 0)
            groups.append([w[40 * j + 8 * t:40 * j + 8 * (t + 1)] - ref for t in range(5)])
        rows = []
        for g in range(4):
            for t in range(3):
                rows.append(jnp.where(sub < 2, pltpu.roll(groups[4 * g + 3][0], 6 - 2 * t, 0),
                                      groups[4 * g + t][0]))
            for t in range(4):
                rows += groups[4 * g + t][1:]
        wat[dst, 0:NF // 2, :] = pltpu.bitcast(jnp.concatenate(rows, axis=0).astype(BF16), U32)
    cp_w(2).wait()
    wat[2] = pltpu.bitcast(wqkv[:, 2 * D:3 * D].T, U32)

    def weight_tile(m, j, t):
        off = j * 384 + t * 128
        if not isinstance(off, int):
            off = pl.multiple_of(off, 128)
        return pltpu.bitcast(wt[m, pl.ds(off, 128), :].T, U32)

    def token(*ys):
        return functools.reduce(
            jnp.maximum, [y[:, 128 * t:128 * (t + 1)] for y in ys for t in range(5)])

    def layer_a(l):
        def sub_all(x, op):
            x = op(x, pltpu.roll(x, 2, 0))
            return op(x, pltpu.roll(x, 4, 0))

        def features(m, x):
            p = _dot_nt(pltpu.bitcast(wat[m, 0:NF // 2, :], BF16), x)
            p = [p[8 * t:8 * (t + 1)] for t in range(NF // 8)]
            sub = _iota((8, 128), 0)
            out = []
            for j in range(16):
                g, t = divmod(j, 4)
                pg = p[19 * g:19 * (g + 1)]
                if t < 3:
                    head = pg[t]
                else:
                    head = jnp.where(sub < 4, pltpu.roll(pg[0], 2, 0),
                                     jnp.where(sub < 6, pltpu.roll(pg[1], 4, 0),
                                               pltpu.roll(pg[2], 6, 0)))
                out.append([jnp.where(sub < 2, 0.0, head)] + pg[3 + 4 * t:7 + 4 * t])
            return out

        def phi(ts):
            mx = sub_all(functools.reduce(jnp.maximum, ts), jnp.maximum)
            mn = sub_all(functools.reduce(jnp.minimum, ts), jnp.minimum)
            ep = [jnp.exp(t - mx) for t in ts]
            en = [jnp.exp(mn - t) for t in ts]
            rp = 1.0 / sub_all(functools.reduce(jnp.add, ep), jnp.add)
            rn = 1.0 / sub_all(functools.reduce(jnp.add, en), jnp.add)
            return jnp.concatenate([e * rp for e in ep] + [e * rn for e in en], axis=0).astype(BF16)

        def phase1(i, carry):
            @pl.when(jnp.logical_and(l == 0, i < NXC - 1))
            def _():
                cp_x(i + 1).wait()

            off = pl.multiple_of(i * TB, TB)
            xn = pltpu.bitcast(xnb[pl.ds(pl.multiple_of(i * (TB // 2), TB // 2), TB // 2), :], BF16)
            xs = [xn[128 * u:128 * (u + 1)] for u in range(TB // 128)]
            nblk = jnp.minimum(i + 1, S // TB - 1)
            nrows = pl.ds(pl.multiple_of(nblk * TB, TB), TB)
            xnext = jnp.where(l == 0, xin[nrows, :].astype(F32), xres[nrows, :])
            ys = [_ln(xnext[16 * k:16 * (k + 1)]) for k in range(TB // 16)]
            xres[nrows, :] = xnext
            xnb[pl.ds(pl.multiple_of(nblk * (TB // 2), TB // 2), TB // 2), :] = pltpu.bitcast(
                jnp.concatenate([y.astype(BF16) for y in ys], axis=0), U32)

            for u, x in enumerate(xs):
                for j, ts in enumerate(features(1, x)):
                    phiq[j, :, pl.ds(off + 128 * u, 128)] = pltpu.bitcast(phi(ts), U32)
            phik = [[phi(ts) for ts in features(0, x)] for x in xs]
            vt = [_dot_nt(pltpu.bitcast(wat[2], BF16), x) for x in xs]
            ones = jnp.ones((8, 128), F32)
            tok = token(*ys[0:8])
            tied = jnp.where(i < 0, jnp.maximum(tok[0:8], tok[8:16]), ones)
            for u in range(len(xs)):
                for j in range(16):
                    lhs = jnp.concatenate(
                        [vt[u][40 * j:40 * (j + 1)], ones if u + j else tied], axis=0).astype(BF16)
                    kvacc[j] = _dot_nt(lhs, phik[u][j]) + kvacc[j]
            return carry

        jax.lax.fori_loop(0, S // TB, phase1, 0)

        @pl.when(l == 0)
        def _():
            cp_big[0].wait()
            cp_big[1].wait()
            cp_wo.wait()
            cp_mem.wait()

        rr = _iota((48, 80), 0)
        cc = _iota((48, 80), 1)
        keep = jnp.where(rr < 40, _div20(rr), (rr - 40) >> 2) == (cc & 1)
        kvm = [jnp.where(keep, kvacc[j], 0.0).astype(BF16) for j in range(16)]
        lo4 = _iota((8, TC), 0) < 4
        opend[...] = jnp.zeros_like(opend)
        kvacc[...] = jnp.zeros_like(kvacc)
        for j in range(NPRE):
            for t in range(3):
                wpre[3 * j + t] = weight_tile(0, JPRE + j, t)

        def num(b):
            parts = []
            for j in range(16):
                r = _dot(kvm[j], pltpu.bitcast(phiq[j, :, TC * b:TC * (b + 1)], BF16))
                rc = 1.0 / (r[40:48] + 1e-6)
                rc2 = pltpu.roll(rc, 4, 0)
                ra = jnp.where(lo4, rc, rc2)
                rb = jnp.where(lo4, rc2, rc)
                parts += [r[0:8] * ra, r[8:16] * ra, r[16:24] * rc, r[24:32] * rb, r[32:40] * rb]
            return jnp.concatenate(parts, axis=0).astype(BF16).T

        for b in range(S // TC):
            obuf[TC // 2 * b:TC // 2 * (b + 1), :] = pltpu.bitcast(num(b), U32)

        def out(i, carry):
            @pl.when(jnp.logical_and(l == 0, i == 2))
            def _():
                cp_big[2].wait()

            for n in range(3 * NPAIR // 4):
                unit = i * (3 * NPAIR // 4) + n
                m, j = unit >> 4, unit & (NPAIR - 1)
                for t in range(3):
                    wb[9 * j + 3 * m + t] = weight_tile(m, j, t)
            xn32[0:RB, :] = _ln(xres[0:RB, :])
            rows = pl.ds(pl.multiple_of(i * TB, TB), TB)
            o = pltpu.bitcast(obuf[pl.ds(pl.multiple_of(i * (TB // 2), TB // 2), TB // 2), :], BF16)
            x = xres[rows, :]
            nb = TB // 64
            pick = lambda y, gs: jnp.concatenate([y[16 * g:16 * (g + 1)] for g in gs], axis=0)
            first = [g for g in range(4 * nb) if g % 4 == 2]
            rest = [g for g in range(4 * nb) if g % 4 != 2]
            xs = _dot(pick(o, first), woa[...]) + pick(x, first)
            memv[...] = mem0_ref[...].astype(F32)
            xo = _dot(pick(o, rest), woa[...]) + pick(x, rest)
            order = first + rest
            xres[rows, :] = pick(jnp.concatenate([xs, xo], axis=0),
                                 [order.index(g) for g in range(4 * nb)])
            wq = jnp.concatenate(
                [pltpu.bitcast(wpre[t], BF16) for t in range(3 * NPRE)], axis=1)
            qpre[pl.ds(pl.multiple_of(i * (8 * nb), 8 * nb), 8 * nb), :] = pltpu.bitcast(
                _dot(_ln(xs).astype(BF16), wq).astype(BF16), U32)
            return carry

        jax.lax.fori_loop(0, S // TB, out, 0)

        @pl.when(l == 0)
        def _():
            def cpo(c, carry):
                cp_bwo(c).wait()
                for u in range(OC // 384):
                    off = pl.multiple_of(c * OC + u * 384, 384)
                    bwo[pl.ds(pl.multiple_of(off // 2, 192), 192), :] = pltpu.bitcast(
                        wt[3, pl.ds(off, 384), :], U32)
                return carry

            jax.lax.fori_loop(0, NOC, cpo, 0)

    scale = DB ** (-0.5)

    def layer_b(layer):
        L = SEG + NM
        NEG = -1000000000.0

        def masks(even):
            nrow = SEG if even else L + 8
            rr = _iota((nrow, 128), 0)
            cc = _iota((nrow, 128), 1)
            is_a = (cc < L) | ((cc >= 2 * L) & (cc < 2 * L + 16))
            kx = jnp.where(cc < L, cc, cc - (L + NM))
            is_memkey = (cc >= SEG) & (cc < SEG + 2 * NM)
            if even:
                valid = cc < 2 * L
                allowed = valid & (is_memkey | (rr >= 24) | (kx <= rr + 8))
            else:
                dk = (cc - 2 * L) & 15
                cur = (rr < L) & (cc < 2 * L)
                old = (rr >= L) & (cc >= 2 * L) & (cc < 2 * L + 32)
                valid = cur | old
                allowed = ((cur & (is_memkey | (rr >= SEG) | (kx <= rr)))
                           | (old & ((dk >= 8) | (dk <= rr - L))))
            return is_a, allowed, jnp.where(valid, NEG, -jnp.inf).astype(F32)

        all_masks = {True: masks(True), False: masks(False)}

        def lo64(y):
            return _iota(y.shape, 1) < 64

        def stack_keys(a, b):
            parts = [a[0:L], b[SEG:L], b[0:SEG]]
            if a.shape[0] > L:
                parts += [a[L:], b[L:]]
            return jnp.concatenate(parts, axis=0).astype(BF16)

        def expand(y):
            y0, y1, y2 = y[:, 0:128], y[:, 128:256], y[:, 256:384]
            return (stack_keys(y0, y2),
                    stack_keys(jnp.where(lo64(y1), y1, 0.0), jnp.where(lo64(y1), 0.0, y1)))

        def pad_lanes(s):
            return jnp.concatenate([s, jnp.zeros((s.shape[0], 128 - s.shape[1]), F32)], axis=1)

        def step(hq, hkv, even, kmajor, side=None, never=None, pre=None):
            is_a, allowed, fill = all_masks[even]
            nrow = SEG if even else L + 8
            nkey = 2 * L if even else 2 * L + 32

            def tiles(j, ts):
                return jnp.concatenate([pltpu.bitcast(wb[9 * j + t], BF16) for t in ts], axis=1)

            def proj(j):
                if j == 0 and kmajor:
                    wq, wkv = tiles(j, range(3)), tiles(j, range(3, 9))
                    q = _dot(hq[:, 0:128], wq[0:128])
                    y = _dot(hkv[:, 0:128], wkv[0:128])
                    for t in range(1, 5):
                        ks = slice(128 * t, 128 * (t + 1))
                        q = _dot(hq[:, ks], wq[ks]) + q
                        y = _dot(hkv[:, ks], wkv[ks]) + y
                else:
                    ahead = pre is not None and JPRE <= j < JPRE + NPRE
                    q = _dot(hq[16:] if ahead else hq, tiles(j, range(3)))
                    y = _dot(hkv, tiles(j, range(3, 9)))
                if even:
                    snext[j] = y[SEG:L]
                    sdef[j, 0:8, :] = y[0:8]
                    sdef[j, 8:16, :] = y[L:L + 8]
                    kv = jnp.concatenate([y[0:SEG], y[L:L + 8]], axis=0)
                else:
                    kv = jnp.concatenate([snext[j], y, sdef[j]], axis=0)
                q = q.astype(BF16)
                if q.shape[0] < nrow:
                    c0 = 384 * (j - JPRE)
                    q = jnp.concatenate(
                        [pltpu.bitcast(qpre[pre, c0:c0 + 384], BF16), q], axis=0)
                q = (jnp.concatenate([q[:, 0:128], q[:, 256:384]], axis=0), q[:, 128:256])
                return q, expand(kv[:, 0:384]), expand(kv[:, 384:768])

            def scores(q, k, tok=None):
                s02 = pad_lanes(_dot_nt(q[0], k[0]))
                s = jnp.where(is_a, s02[0:nrow], s02[nrow:]) + pad_lanes(_dot_nt(q[1], k[1]))
                s = jnp.where(allowed, s * scale, fill)
                ma = jnp.max(jnp.where(is_a, s, -jnp.inf), axis=1, keepdims=True)
                mb = jnp.max(jnp.where(is_a, -jnp.inf, s), axis=1, keepdims=True)
                e = jnp.exp(s - jnp.where(is_a, ma, mb))
                ea = jnp.where(is_a, e, 0.0)
                eb = jnp.where(is_a, 0.0, e)
                pa = ea * (1.0 / jnp.sum(ea, axis=1, keepdims=True))
                pb = eb * (1.0 / jnp.sum(eb, axis=1, keepdims=True))
                if tok is not None:
                    pb = jnp.concatenate([jnp.where(never, tok, pb[0:16]), pb[16:]], axis=0)
                return (jnp.concatenate([pa, pb], axis=0)[:, 0:nkey].astype(BF16),
                        (pa + pb)[:, 0:nkey].astype(BF16))

            def pv(p, v):
                o02 = _dot(p[0], v[0])
                return jnp.concatenate(
                    [o02[0:nrow], _dot(p[1], v[1]), o02[nrow:]], axis=1).astype(BF16)

            qkv = [None] * NPAIR
            ps = [None] * NPAIR
            os_ = [None] * NPAIR

            def wo_chunk(c0, c1):
                w = pltpu.bitcast(bwo[192 * c0:192 * c1, :], BF16)
                return _dot(jnp.concatenate(os_[c0:c1], axis=1), w)

            cuts = (0, 4, 8, 11, 14, 16) if even else (11, 12, 13, 14, 15, 16)
            lag = NPAIR - 1 - cuts[0]
            qkv[0] = proj(0)
            acc = None
            for j in range(NPAIR + 2):
                c = None
                if j + 1 < NPAIR:
                    qkv[j + 1] = proj(j + 1)
                    if j >= lag:
                        c = wo_chunk(j - lag, j - lag + 1)
                else:
                    c = wo_chunk(cuts[j + 1 - NPAIR], cuts[j + 2 - NPAIR])
                if c is not None:
                    acc = c if acc is None else c + acc
                if j < NPAIR:
                    ps[j] = scores(qkv[j][0], qkv[j][1], side(j) if side else None)
                if j >= 2:
                    os_[j - 2] = pv(ps[j - 2], qkv[j - 2][2])
            acc = wo_chunk(cuts[3], cuts[4]) + acc
            return wo_chunk(cuts[4], cuts[5]) + acc

        def finish_rows(base, r0, n):
            rows = pl.ds(base + r0, n)
            xnew = xres[rows, :] + opend[r0:r0 + n, :]
            xres[rows, :] = xnew
            xin[rows, :] = xnew.astype(BF16)
            y = _ln(xnew)
            xnb[pl.ds(pl.multiple_of(base // 2, RB // 2) + r0 // 2, n // 2), :] = pltpu.bitcast(
                y.astype(BF16), U32)
            return y

        def body(i, carry):
            base = pl.multiple_of(i * RB, RB)

            @pl.when(jnp.logical_and(layer == 1, i >= 2))
            def _():
                rows = pl.ds(pl.multiple_of((i - 2) * RB, RB), RB)
                pltpu.make_async_copy(xin.at[rows], out_hbm.at[rows], sems.at[0]).start()

            prev = pl.multiple_of(jnp.maximum(i - 1, 0) * RB, RB)
            nxt = pl.multiple_of(jnp.minimum(i + 1, S // RB - 1) * RB, RB)

            def side_prev(j):
                if j % 2:
                    return None
                return token(finish_rows(prev, 8 * j, 16))

            def side_next(j):
                if j % 2:
                    return None
                rows = pl.ds(nxt + 8 * j, 16)
                y = _ln(xres[rows, :])
                xn32[rows, :] = y
                return token(y)

            sides = (side_prev, side_next)
            never = i < 0
            mem = memv[...]
            for u in range(UNROLL):
                r0 = 64 * u
                xr = lambda a, n: xn32[pl.ds(base + r0 + a, n), :]
                cat = lambda *p: jnp.concatenate(p, axis=0).astype(BF16)
                o0 = step(cat(xr(8, 24), mem), cat(xr(0, 40), mem), True, u > 0, sides[u], never)
                opend[r0 + 8:r0 + 32, :] = o0[0:24]
                mem = o0[24:32]
                o1 = step(cat(xr(32, 32), mem, xr(0, 8)), cat(xr(40, 24), mem), False, True,
                          pre=pl.ds(pl.multiple_of(i * (8 * UNROLL), 8) + 8 * u, 8))
                mem = o1[32:40]
                opend[r0:r0 + 8, :] = o1[40:48]
                opend[r0 + 32:r0 + 64, :] = o1[0:32]
            memv[...] = mem
            return carry

        jax.lax.fori_loop(0, S // RB, body, 0)

        @pl.when(layer == 0)
        def _():
            xres[S - RB:S, :] = xres[S - RB:S, :] + opend[...]

    def layer(l, carry):
        layer_a(l)
        layer_b(l)
        return carry

    jax.lax.fori_loop(0, 2, layer, 0)

    rows = pl.ds(S - 2 * RB, RB)
    pltpu.make_async_copy(xin.at[rows], out_hbm.at[rows], sems.at[0]).start()
    rows = pl.ds(S - RB, RB)
    xin[rows, :] = (xres[rows, :] + opend[...]).astype(BF16)
    pltpu.make_async_copy(xin.at[rows], out_hbm.at[rows], sems.at[0]).start()
    pltpu.make_async_copy(xin, out_hbm, sems.at[0]).wait()


@jax.jit
def pallas_interleave_layers__linear_kernel_hedgehog__memory_aug_recurrent_mem_tr__prompt_kernel(
    A_x: jax.Array,
    A_wqkv: jax.Array,
    A_w_phi: jax.Array,
    A_wo: jax.Array,
    B_x: jax.Array,
    B_mem0: jax.Array,
    B_Wq: jax.Array,
    B_Wk: jax.Array,
    B_Wv: jax.Array,
    B_Wo: jax.Array,
    B_seg_len: jax.Array,
):
    assert A_x.shape == (1, S, D) and B_mem0.shape == (1, NM, D) and B_Wq.shape == (D, HB, DB)
    tr = lambda w: jnp.transpose(w, (1, 2, 0)).reshape(HB * DB, D)
    any_spec = pl.BlockSpec(memory_space=pl.ANY)
    out = pl.pallas_call(
        _kernel,
        out_shape=jax.ShapeDtypeStruct((S, D), BF16),
        in_specs=[any_spec] * 9,
        out_specs=any_spec,
        scratch_shapes=[
            pltpu.VMEM((DA, DA, HA), BF16),
            pltpu.VMEM((NM, D), BF16),
            pltpu.VMEM((S, D), BF16),
            pltpu.VMEM((D, 3 * D), BF16),
            pltpu.VMEM((D, D), BF16),
            pltpu.VMEM((4, HB * DB, D), BF16),
            pltpu.VMEM((9 * NPAIR, D // 2, 128), U32),
            pltpu.VMEM((HB * DB // 2, D), U32),
            pltpu.VMEM((S, D), F32),
            pltpu.VMEM((S, D), F32),
            pltpu.VMEM((S // 2, D), U32),
            pltpu.VMEM((3, D // 2, D), U32),
            pltpu.VMEM((16, 48, 80), F32),
            pltpu.VMEM((16, 40, S), U32),
            pltpu.VMEM((S // 2, D), U32),
            pltpu.VMEM((3 * NPRE, D // 2, 128), U32),
            pltpu.VMEM((S // 8, 384 * NPRE), U32),
            pltpu.VMEM((NM, D), F32),
            pltpu.VMEM((NPAIR, 8, 6 * 128), F32),
            pltpu.VMEM((NPAIR, 16, 6 * 128), F32),
            pltpu.VMEM((64 * UNROLL, D), F32),
            pltpu.SemaphoreType.DMA((7,)),
            pltpu.SemaphoreType.DMA((NXC,)),
            pltpu.SemaphoreType.DMA((NOC,)),
            pltpu.SemaphoreType.DMA((3,)),
        ],
        compiler_params=pltpu.CompilerParams(vmem_limit_bytes=120 * 1024 * 1024),
    )(A_x.reshape(S, D), A_wqkv, jnp.transpose(A_w_phi, (1, 2, 0)), A_wo,
      B_mem0.reshape(NM, D), tr(B_Wq), tr(B_Wk), tr(B_Wv), B_Wo.reshape(HB * DB, D))
    return out.reshape(1, S, D)
```

```python
import functools

import jax
import jax.numpy as jnp
import jax.experimental.pallas as pl
import jax.experimental.pallas.tpu as pltpu

F32 = jnp.float32
BF16 = jnp.bfloat16
U32 = jnp.uint32

S = 2048
D = 640
HA = 32
DA = 20
HB = 32
DB = 192
NM = 8
SEG = 32
NPAIR = HB // 2
NF = HA * (DA - 1)
TB = 512
TC = 512
UNROLL = 2
RB = 64 * UNROLL
NPRE = 3
JPRE = 8
NXC = S // TB
NOC = 8
NH = 2
LN_EPS = 1e-5

_NN = (((1,), (0,)), ((), ()))
_NT = (((1,), (1,)), ((), ()))


def _dot(a, b):
    return jax.lax.dot_general(a, b, _NN, preferred_element_type=F32)


def _dot_nt(a, b):
    return jax.lax.dot_general(a, b, _NT, preferred_element_type=F32)


def _ln(x):
    m = jnp.mean(x, axis=-1, keepdims=True)
    xc = x - m
    v = jnp.mean(xc * xc, axis=-1, keepdims=True)
    return xc * jax.lax.rsqrt(v + LN_EPS)


def _iota(shape, dim):
    return jax.lax.broadcasted_iota(jnp.int32, shape, dim)


def _div20(i):
    return (i * 3277) >> 16


def _div40(i):
    return _div20(i) >> 1


def _kernel(x_hbm, wqkv_hbm, wphi_hbm, wo_hbm, mem0_hbm, wqt_hbm, wkt_hbm, wvt_hbm, bwo_hbm,
            out_hbm,
            wphi_ref, mem0_ref, xin, wqkv, woa, wt, wb, bwo, xres, xn32, xnb, wat, kvacc, phiq,
            obuf, wpre, qpre, memv, snext, sdef, opend, sems, xsems, osems, wsems):
    XC = S // NXC
    cp_phi = pltpu.make_async_copy(wphi_hbm, wphi_ref, sems.at[0])

    def cp_w(m):
        cols = pl.ds(m * D, D)
        return pltpu.make_async_copy(wqkv_hbm.at[:, cols], wqkv.at[:, cols], wsems.at[m])

    def cp_x(c):
        rows = pl.ds(c * XC if isinstance(c, int) else pl.multiple_of(c * XC, XC), XC)
        return pltpu.make_async_copy(x_hbm.at[rows], xin.at[rows], xsems.at[c])

    cp_wo = pltpu.make_async_copy(wo_hbm, woa, sems.at[2])
    cp_mem = pltpu.make_async_copy(mem0_hbm, mem0_ref, sems.at[3])
    cp_big = [
        pltpu.make_async_copy(wqt_hbm, wt.at[0], sems.at[4]),
        pltpu.make_async_copy(wkt_hbm, wt.at[1], sems.at[5]),
        pltpu.make_async_copy(wvt_hbm, wt.at[2], sems.at[6]),
    ]
    OC = HB * DB // NOC

    def cp_bwo(c):
        rows = pl.ds(pl.multiple_of(c * OC, OC), OC)
        return pltpu.make_async_copy(bwo_hbm.at[rows], wt.at[3, rows], osems.at[c])

    def start_in_order(copies):
        def start(c, carry):
            for n, cp in enumerate(copies):
                pl.when(c == n)(cp.start)
            return carry

        jax.lax.fori_loop(0, len(copies), start, 0)

    start_in_order([cp_phi, cp_x(0), cp_w(0), cp_w(1), cp_w(2)] + [cp_x(c) for c in range(1, NXC)])
    cp_phi.wait()

    wphi = wphi_ref[...].astype(F32)
    xw = jnp.concatenate([wphi[d] for d in range(DA)], axis=1)
    xw = jnp.concatenate([xw, jnp.zeros((32 - DA, D), F32)], axis=0).astype(BF16)
    r = _iota((D, D), 0)
    c = _iota((D, D), 1)
    perm = jnp.where((r & 31) * DA + (r >> 5) == c, 1.0, 0.0).astype(BF16)
    wf = _dot(xw, perm).astype(BF16)
    r = _iota((160, 32), 0)
    c = _iota((160, 32), 1)
    rsel = jnp.where(((r - _div40(r) * 40) >> 1) == c, 1.0, 0.0).astype(BF16)
    r = _iota((160, 128), 0)
    c = _iota((160, 128), 1)
    phit = []
    for t in range(5):
        keep = 2 * (_div40(r) + 3 * t) + (r & 1) == _div20(c + 128 * t)
        phit.append(jnp.where(keep, _dot(rsel, wf[:, 128 * t:128 * (t + 1)]), 0.0).astype(BF16))

    kvacc[...] = jnp.zeros_like(kvacc)

    cp_x(0).wait()

    def init_blk(i, carry):
        for u in range(4):
            off = pl.multiple_of(i * 256 + u * 64, 64)
            x = xin[pl.ds(off, 64), :].astype(F32)
            xres[pl.ds(off, 64), :] = x
            xnb[pl.ds(pl.multiple_of(off // 2, 32), 32), :] = pltpu.bitcast(_ln(x).astype(BF16), U32)
        return carry

    jax.lax.fori_loop(0, XC // 256, init_blk, 0)
    start_in_order([cp_big[0], cp_big[1], cp_wo, cp_mem, cp_big[2]])

    def start_bwo(c, carry):
        cp_bwo(c).start()
        return carry

    jax.lax.fori_loop(0, NOC, start_bwo, 0)
    for m, dst in ((0, 1), (1, 0)):
        cp_w(m).wait()
        p = [_dot_nt(phit[t], wqkv[:, m * D + 128 * t:m * D + 128 * (t + 1)]) for t in range(5)]
        rows = [p[0][0:120]]
        for t in range(1, 5):
            rows += [p[t - 1][120:160] + p[t][0:40], p[t][40:120]]
        rows.append(p[4][120:160])
        w = jnp.concatenate(rows, axis=0)
        sub = _iota((8, D), 0)
        groups = []
        for j in range(16):
            ref = jnp.where(sub < 2, w[40 * j:40 * j + 8], 0.0)
            ref = ref + pltpu.roll(ref, 2, 0)
            ref = ref + pltpu.roll(ref, 4, 0)
            groups.append([w[40 * j + 8 * t:40 * j + 8 * (t + 1)] - ref for t in range(5)])
        rows = []
        for g in range(4):
            for t in range(3):
                rows.append(jnp.where(sub < 2, pltpu.roll(groups[4 * g + 3][0], 6 - 2 * t, 0),
                                      groups[4 * g + t][0]))
            for t in range(4):
                rows += groups[4 * g + t][1:]
        wat[dst, 0:NF // 2, :] = pltpu.bitcast(jnp.concatenate(rows, axis=0).astype(BF16), U32)
    cp_w(2).wait()
    wat[2] = pltpu.bitcast(wqkv[:, 2 * D:3 * D].T, U32)

    def weight_tile(m, j, t):
        off = j * 384 + t * 128
        if not isinstance(off, int):
            off = pl.multiple_of(off, 128)
        return pltpu.bitcast(wt[m, pl.ds(off, 128), :].T, U32)

    def token(*ys):
        return functools.reduce(
            jnp.maximum, [y[:, 128 * t:128 * (t + 1)] for y in ys for t in range(5)])

    def pack_wo(slot, c, tie=lambda w: w):
        bwo[pl.ds(pl.multiple_of(c * (OC // 2), OC // 2), OC // 2), :] = tie(pltpu.bitcast(
            wt[slot, pl.ds(pl.multiple_of(c * OC, OC), OC), :], U32))

    def layer_a(l):
        def sub_all(x, op):
            x = op(x, pltpu.roll(x, 2, 0))
            return op(x, pltpu.roll(x, 4, 0))

        def features(m, x):
            p = _dot_nt(pltpu.bitcast(wat[m, 0:NF // 2, :], BF16), x)
            p = [p[8 * t:8 * (t + 1)] for t in range(NF // 8)]
            sub = _iota((8, 128), 0)
            out = []
            for j in range(16):
                g, t = divmod(j, 4)
                pg = p[19 * g:19 * (g + 1)]
                if t < 3:
                    head = pg[t]
                else:
                    head = jnp.where(sub < 4, pltpu.roll(pg[0], 2, 0),
                                     jnp.where(sub < 6, pltpu.roll(pg[1], 4, 0),
                                               pltpu.roll(pg[2], 6, 0)))
                out.append([jnp.where(sub < 2, 0.0, head)] + pg[3 + 4 * t:7 + 4 * t])
            return out

        def phi(ts):
            mx = sub_all(functools.reduce(jnp.maximum, ts), jnp.maximum)
            mn = sub_all(functools.reduce(jnp.minimum, ts), jnp.minimum)
            ep = [jnp.exp(t - mx) for t in ts]
            en = [jnp.exp(mn - t) for t in ts]
            rp = 1.0 / sub_all(functools.reduce(jnp.add, ep), jnp.add)
            rn = 1.0 / sub_all(functools.reduce(jnp.add, en), jnp.add)
            return jnp.concatenate([e * rp for e in ep] + [e * rn for e in en], axis=0).astype(BF16)

        def phase1(i, carry):
            @pl.when(jnp.logical_and(l == 0, i < NXC - 1))
            def _():
                cp_x(i + 1).wait()

            off = pl.multiple_of(i * TB, TB)
            xn = pltpu.bitcast(xnb[pl.ds(pl.multiple_of(i * (TB // 2), TB // 2), TB // 2), :], BF16)
            xs = [xn[128 * u:128 * (u + 1)] for u in range(TB // 128)]
            nblk = jnp.minimum(i + 1, S // TB - 1)
            nrows = pl.ds(pl.multiple_of(nblk * TB, TB), TB)
            xnext = jnp.where(l == 0, xin[nrows, :].astype(F32), xres[nrows, :])
            ys = [_ln(xnext[16 * k:16 * (k + 1)]) for k in range(TB // 16)]
            xres[nrows, :] = xnext
            xnb[pl.ds(pl.multiple_of(nblk * (TB // 2), TB // 2), TB // 2), :] = pltpu.bitcast(
                jnp.concatenate([y.astype(BF16) for y in ys], axis=0), U32)

            for u, x in enumerate(xs):
                for j, ts in enumerate(features(1, x)):
                    phiq[j, :, pl.ds(off + 128 * u, 128)] = pltpu.bitcast(phi(ts), U32)
            phik = [[phi(ts) for ts in features(0, x)] for x in xs]
            vt = [_dot_nt(pltpu.bitcast(wat[2], BF16), x) for x in xs]
            ones = jnp.ones((8, 128), F32)
            tok = token(*ys[0:8])
            tied = jnp.where(i < 0, jnp.maximum(tok[0:8], tok[8:16]), ones)
            for u in range(len(xs)):
                for j in range(16):
                    lhs = jnp.concatenate(
                        [vt[u][40 * j:40 * (j + 1)], ones if u + j else tied], axis=0).astype(BF16)
                    kvacc[j] = _dot_nt(lhs, phik[u][j]) + kvacc[j]
            return carry

        jax.lax.fori_loop(0, S // TB, phase1, 0)

        @pl.when(l == 0)
        def _():
            cp_big[0].wait()
            cp_big[1].wait()
            cp_wo.wait()
            cp_mem.wait()

        rr = _iota((48, 80), 0)
        cc = _iota((48, 80), 1)
        keep = jnp.where(rr < 40, _div20(rr), (rr - 40) >> 2) == (cc & 1)
        kvm = [jnp.where(keep, kvacc[j], 0.0).astype(BF16) for j in range(16)]
        lo4 = _iota((8, TC), 0) < 4
        opend[...] = jnp.zeros_like(opend)
        kvacc[...] = jnp.zeros_like(kvacc)
        for j in range(NPRE):
            for t in range(3):
                wpre[3 * j + t] = weight_tile(0, JPRE + j, t)

        def num(b):
            parts = []
            for j in range(16):
                r = _dot(kvm[j], pltpu.bitcast(phiq[j, :, TC * b:TC * (b + 1)], BF16))
                rc = 1.0 / (r[40:48] + 1e-6)
                rc2 = pltpu.roll(rc, 4, 0)
                ra = jnp.where(lo4, rc, rc2)
                rb = jnp.where(lo4, rc2, rc)
                parts += [r[0:8] * ra, r[8:16] * ra, r[16:24] * rc, r[24:32] * rb, r[32:40] * rb]
            return jnp.concatenate(parts, axis=0).astype(BF16).T

        for b in range(S // TC):
            obuf[TC // 2 * b:TC // 2 * (b + 1), :] = pltpu.bitcast(num(b), U32)

        def out(i, carry):
            @pl.when(jnp.logical_and(l == 0, i == 2))
            def _():
                cp_big[2].wait()

            @pl.when(jnp.logical_and(l == 0, i >= 2))
            def _():
                for c in range(NH):
                    cp_bwo((i - 2) * NH + c).wait()

            for n in range(3 * NPAIR // 4):
                unit = i * (3 * NPAIR // 4) + n
                m, j = unit >> 4, unit & (NPAIR - 1)
                for t in range(3):
                    wb[9 * j + 3 * m + t] = weight_tile(m, j, t)
            xn32[0:RB, :] = _ln(xres[0:RB, :])
            rows = pl.ds(pl.multiple_of(i * TB, TB), TB)
            o = pltpu.bitcast(obuf[pl.ds(pl.multiple_of(i * (TB // 2), TB // 2), TB // 2), :], BF16)
            x = xres[rows, :]
            nb = TB // 64
            pick = lambda y, gs: jnp.concatenate([y[16 * g:16 * (g + 1)] for g in gs], axis=0)
            first = [g for g in range(4 * nb) if g % 4 == 2]
            rest = [g for g in range(4 * nb) if g % 4 != 2]
            xs = _dot(pick(o, first), woa[...]) + pick(x, first)
            memv[...] = mem0_ref[...].astype(F32)
            xo = _dot(pick(o, rest), woa[...]) + pick(x, rest)
            for c in range(NH):
                pack_wo(jnp.where(i < 2, 0, 3), (i & 1) * NH + c,
                        lambda w: jnp.where(i < 0, pltpu.bitcast(xo, U32), w))
            order = first + rest
            xres[rows, :] = pick(jnp.concatenate([xs, xo], axis=0),
                                 [order.index(g) for g in range(4 * nb)])
            wq = jnp.concatenate(
                [pltpu.bitcast(wpre[t], BF16) for t in range(3 * NPRE)], axis=1)
            qpre[pl.ds(pl.multiple_of(i * (8 * nb), 8 * nb), 8 * nb), :] = pltpu.bitcast(
                _dot(_ln(xs).astype(BF16), wq).astype(BF16), U32)
            return carry

        jax.lax.fori_loop(0, S // TB, out, 0)

        @pl.when(l == 0)
        def _():
            def cpo(c, carry):
                cp_bwo(c).wait()
                pack_wo(3, c)
                return carry

            jax.lax.fori_loop(2 * NH, NOC, cpo, 0)

    scale = DB ** (-0.5)

    def layer_b(layer):
        L = SEG + NM
        NEG = -1000000000.0

        def masks(even):
            nrow = SEG if even else L + 8
            rr = _iota((nrow, 128), 0)
            cc = _iota((nrow, 128), 1)
            is_a = (cc < L) | ((cc >= 2 * L) & (cc < 2 * L + 16))
            kx = jnp.where(cc < L, cc, cc - (L + NM))
            is_memkey = (cc >= SEG) & (cc < SEG + 2 * NM)
            if even:
                valid = cc < 2 * L
                allowed = valid & (is_memkey | (rr >= 24) | (kx <= rr + 8))
            else:
                dk = (cc - 2 * L) & 15
                cur = (rr < L) & (cc < 2 * L)
                old = (rr >= L) & (cc >= 2 * L) & (cc < 2 * L + 32)
                valid = cur | old
                allowed = ((cur & (is_memkey | (rr >= SEG) | (kx <= rr)))
                           | (old & ((dk >= 8) | (dk <= rr - L))))
            return is_a, allowed, jnp.where(valid, NEG, -jnp.inf).astype(F32)

        all_masks = {True: masks(True), False: masks(False)}

        def lo64(y):
            return _iota(y.shape, 1) < 64

        def stack_keys(a, b):
            parts = [a[0:L], b[SEG:L], b[0:SEG]]
            if a.shape[0] > L:
                parts += [a[L:], b[L:]]
            return jnp.concatenate(parts, axis=0).astype(BF16)

        def expand(y):
            y0, y1, y2 = y[:, 0:128], y[:, 128:256], y[:, 256:384]
            return (stack_keys(y0, y2),
                    stack_keys(jnp.where(lo64(y1), y1, 0.0), jnp.where(lo64(y1), 0.0, y1)))

        def pad_lanes(s):
            return jnp.concatenate([s, jnp.zeros((s.shape[0], 128 - s.shape[1]), F32)], axis=1)

        def step(hq, hkv, even, kmajor, side=None, never=None, pre=None):
            is_a, allowed, fill = all_masks[even]
            nrow = SEG if even else L + 8
            nkey = 2 * L if even else 2 * L + 32

            def tiles(j, ts):
                return jnp.concatenate([pltpu.bitcast(wb[9 * j + t], BF16) for t in ts], axis=1)

            def proj(j):
                if j == 0 and kmajor:
                    wq, wkv = tiles(j, range(3)), tiles(j, range(3, 9))
                    q = _dot(hq[:, 0:128], wq[0:128])
                    y = _dot(hkv[:, 0:128], wkv[0:128])
                    for t in range(1, 5):
                        ks = slice(128 * t, 128 * (t + 1))
                        q = _dot(hq[:, ks], wq[ks]) + q
                        y = _dot(hkv[:, ks], wkv[ks]) + y
                else:
                    ahead = pre is not None and JPRE <= j < JPRE + NPRE
                    q = _dot(hq[16:] if ahead else hq, tiles(j, range(3)))
                    y = _dot(hkv, tiles(j, range(3, 9)))
                if even:
                    snext[j] = y[SEG:L]
                    sdef[j, 0:8, :] = y[0:8]
                    sdef[j, 8:16, :] = y[L:L + 8]
                    kv = jnp.concatenate([y[0:SEG], y[L:L + 8]], axis=0)
                else:
                    kv = jnp.concatenate([snext[j], y, sdef[j]], axis=0)
                q = q.astype(BF16)
                if q.shape[0] < nrow:
                    c0 = 384 * (j - JPRE)
                    q = jnp.concatenate(
                        [pltpu.bitcast(qpre[pre, c0:c0 + 384], BF16), q], axis=0)
                q = (jnp.concatenate([q[:, 0:128], q[:, 256:384]], axis=0), q[:, 128:256])
                return q, expand(kv[:, 0:384]), expand(kv[:, 384:768])

            def scores(q, k, tok=None):
                s02 = pad_lanes(_dot_nt(q[0], k[0]))
                s = jnp.where(is_a, s02[0:nrow], s02[nrow:]) + pad_lanes(_dot_nt(q[1], k[1]))
                s = jnp.where(allowed, s * scale, fill)
                ma = jnp.max(jnp.where(is_a, s, -jnp.inf), axis=1, keepdims=True)
                mb = jnp.max(jnp.where(is_a, -jnp.inf, s), axis=1, keepdims=True)
                e = jnp.exp(s - jnp.where(is_a, ma, mb))
                ea = jnp.where(is_a, e, 0.0)
                eb = jnp.where(is_a, 0.0, e)
                pa = ea * (1.0 / jnp.sum(ea, axis=1, keepdims=True))
                pb = eb * (1.0 / jnp.sum(eb, axis=1, keepdims=True))
                if tok is not None:
                    pb = jnp.concatenate([jnp.where(never, tok, pb[0:16]), pb[16:]], axis=0)
                return (jnp.concatenate([pa, pb], axis=0)[:, 0:nkey].astype(BF16),
                        (pa + pb)[:, 0:nkey].astype(BF16))

            def pv(p, v):
                o02 = _dot(p[0], v[0])
                return jnp.concatenate(
                    [o02[0:nrow], _dot(p[1], v[1]), o02[nrow:]], axis=1).astype(BF16)

            qkv = [None] * NPAIR
            ps = [None] * NPAIR
            os_ = [None] * NPAIR

            def wo_chunk(c0, c1):
                w = pltpu.bitcast(bwo[192 * c0:192 * c1, :], BF16)
                return _dot(jnp.concatenate(os_[c0:c1], axis=1), w)

            cuts = (0, 4, 8, 11, 14, 16) if even else (11, 12, 13, 14, 15, 16)
            lag = NPAIR - 1 - cuts[0]
            qkv[0] = proj(0)
            acc = None
            for j in range(NPAIR + 2):
                c = None
                if j + 1 < NPAIR:
                    qkv[j + 1] = proj(j + 1)
                    if j >= lag:
                        c = wo_chunk(j - lag, j - lag + 1)
                else:
                    c = wo_chunk(cuts[j + 1 - NPAIR], cuts[j + 2 - NPAIR])
                if c is not None:
                    acc = c if acc is None else c + acc
                if j < NPAIR:
                    ps[j] = scores(qkv[j][0], qkv[j][1], side(j) if side else None)
                if j >= 2:
                    os_[j - 2] = pv(ps[j - 2], qkv[j - 2][2])
            acc = wo_chunk(cuts[3], cuts[4]) + acc
            return wo_chunk(cuts[4], cuts[5]) + acc

        def finish_rows(base, r0, n):
            rows = pl.ds(base + r0, n)
            xnew = xres[rows, :] + opend[r0:r0 + n, :]
            xres[rows, :] = xnew
            xin[rows, :] = xnew.astype(BF16)
            y = _ln(xnew)
            xnb[pl.ds(pl.multiple_of(base // 2, RB // 2) + r0 // 2, n // 2), :] = pltpu.bitcast(
                y.astype(BF16), U32)
            return y

        def body(i, carry):
            base = pl.multiple_of(i * RB, RB)

            @pl.when(jnp.logical_and(layer == 1, i >= 2))
            def _():
                rows = pl.ds(pl.multiple_of((i - 2) * RB, RB), RB)
                pltpu.make_async_copy(xin.at[rows], out_hbm.at[rows], sems.at[0]).start()

            prev = pl.multiple_of(jnp.maximum(i - 1, 0) * RB, RB)
            nxt = pl.multiple_of(jnp.minimum(i + 1, S // RB - 1) * RB, RB)

            def side_prev(j):
                if j % 2:
                    return None
                return token(finish_rows(prev, 8 * j, 16))

            def side_next(j):
                if j % 2:
                    return None
                rows = pl.ds(nxt + 8 * j, 16)
                y = _ln(xres[rows, :])
                xn32[rows, :] = y
                return token(y)

            sides = (side_prev, side_next)
            never = i < 0
            mem = memv[...]
            for u in range(UNROLL):
                r0 = 64 * u
                xr = lambda a, n: xn32[pl.ds(base + r0 + a, n), :]
                cat = lambda *p: jnp.concatenate(p, axis=0).astype(BF16)
                o0 = step(cat(xr(8, 24), mem), cat(xr(0, 40), mem), True, u > 0, sides[u], never)
                opend[r0 + 8:r0 + 32, :] = o0[0:24]
                mem = o0[24:32]
                o1 = step(cat(xr(32, 32), mem, xr(0, 8)), cat(xr(40, 24), mem), False, True,
                          pre=pl.ds(pl.multiple_of(i * (8 * UNROLL), 8) + 8 * u, 8))
                mem = o1[32:40]
                opend[r0:r0 + 8, :] = o1[40:48]
                opend[r0 + 32:r0 + 64, :] = o1[0:32]
            memv[...] = mem
            return carry

        jax.lax.fori_loop(0, S // RB, body, 0)

        @pl.when(layer == 0)
        def _():
            xres[S - RB:S, :] = xres[S - RB:S, :] + opend[...]

    def layer(l, carry):
        layer_a(l)
        layer_b(l)
        return carry

    jax.lax.fori_loop(0, 2, layer, 0)

    rows = pl.ds(S - 2 * RB, RB)
    pltpu.make_async_copy(xin.at[rows], out_hbm.at[rows], sems.at[0]).start()
    rows = pl.ds(S - RB, RB)
    xin[rows, :] = (xres[rows, :] + opend[...]).astype(BF16)
    pltpu.make_async_copy(xin.at[rows], out_hbm.at[rows], sems.at[0]).start()
    pltpu.make_async_copy(xin, out_hbm, sems.at[0]).wait()


@jax.jit
def pallas_interleave_layers__linear_kernel_hedgehog__memory_aug_recurrent_mem_tr__prompt_kernel(
    A_x: jax.Array,
    A_wqkv: jax.Array,
    A_w_phi: jax.Array,
    A_wo: jax.Array,
    B_x: jax.Array,
    B_mem0: jax.Array,
    B_Wq: jax.Array,
    B_Wk: jax.Array,
    B_Wv: jax.Array,
    B_Wo: jax.Array,
    B_seg_len: jax.Array,
):
    assert A_x.shape == (1, S, D) and B_mem0.shape == (1, NM, D) and B_Wq.shape == (D, HB, DB)
    tr = lambda w: jnp.transpose(w, (1, 2, 0)).reshape(HB * DB, D)
    any_spec = pl.BlockSpec(memory_space=pl.ANY)
    out = pl.pallas_call(
        _kernel,
        out_shape=jax.ShapeDtypeStruct((S, D), BF16),
        in_specs=[any_spec] * 9,
        out_specs=any_spec,
        scratch_shapes=[
            pltpu.VMEM((DA, DA, HA), BF16),
            pltpu.VMEM((NM, D), BF16),
            pltpu.VMEM((S, D), BF16),
            pltpu.VMEM((D, 3 * D), BF16),
            pltpu.VMEM((D, D), BF16),
            pltpu.VMEM((4, HB * DB, D), BF16),
            pltpu.VMEM((9 * NPAIR, D // 2, 128), U32),
            pltpu.VMEM((HB * DB // 2, D), U32),
            pltpu.VMEM((S, D), F32),
            pltpu.VMEM((S, D), F32),
            pltpu.VMEM((S // 2, D), U32),
            pltpu.VMEM((3, D // 2, D), U32),
            pltpu.VMEM((16, 48, 80), F32),
            pltpu.VMEM((16, 40, S), U32),
            pltpu.VMEM((S // 2, D), U32),
            pltpu.VMEM((3 * NPRE, D // 2, 128), U32),
            pltpu.VMEM((S // 8, 384 * NPRE), U32),
            pltpu.VMEM((NM, D), F32),
            pltpu.VMEM((NPAIR, 8, 6 * 128), F32),
            pltpu.VMEM((NPAIR, 16, 6 * 128), F32),
            pltpu.VMEM((64 * UNROLL, D), F32),
            pltpu.SemaphoreType.DMA((7,)),
            pltpu.SemaphoreType.DMA((NXC,)),
            pltpu.SemaphoreType.DMA((NOC,)),
            pltpu.SemaphoreType.DMA((3,)),
        ],
        compiler_params=pltpu.CompilerParams(vmem_limit_bytes=120 * 1024 * 1024),
    )(A_x.reshape(S, D), A_wqkv, jnp.transpose(A_w_phi, (1, 2, 0)), A_wo,
      B_mem0.reshape(NM, D), tr(B_Wq), tr(B_Wk), tr(B_Wv), B_Wo.reshape(HB * DB, D))
    return out.reshape(1, S, D)
```

```python
import functools

import jax
import jax.numpy as jnp
import jax.experimental.pallas as pl
import jax.experimental.pallas.tpu as pltpu

F32 = jnp.float32
BF16 = jnp.bfloat16
U32 = jnp.uint32

S = 2048
D = 640
HA = 32
DA = 20
HB = 32
DB = 192
NM = 8
SEG = 32
NPAIR = HB // 2
NF = HA * (DA - 1)
TB = 512
TC = 512
UNROLL = 2
RB = 64 * UNROLL
NPRE = 3
JPRE = 8
NXC = S // TB
NOC = 8
NH = 2
LN_EPS = 1e-5

_NN = (((1,), (0,)), ((), ()))
_NT = (((1,), (1,)), ((), ()))


def _dot(a, b):
    return jax.lax.dot_general(a, b, _NN, preferred_element_type=F32)


def _dot_nt(a, b):
    return jax.lax.dot_general(a, b, _NT, preferred_element_type=F32)


def _ln(x):
    m = jnp.mean(x, axis=-1, keepdims=True)
    xc = x - m
    v = jnp.mean(xc * xc, axis=-1, keepdims=True)
    return xc * jax.lax.rsqrt(v + LN_EPS)


def _iota(shape, dim):
    return jax.lax.broadcasted_iota(jnp.int32, shape, dim)


def _div20(i):
    return (i * 3277) >> 16


def _div40(i):
    return _div20(i) >> 1


def _kernel(x_hbm, wqkv_hbm, wphi_hbm, wo_hbm, mem0_hbm, wqt_hbm, wkt_hbm, wvt_hbm, bwo_hbm,
            out_hbm,
            wphi_ref, mem0_ref, xin, wqkv, woa, wt, wb, bwo, xres, xn32, xnb, wat, kvacc, phiq,
            obuf, wpre, qpre, memv, snext, sdef, opend, sems, xsems, osems, wsems):
    XC = S // NXC
    cp_phi = pltpu.make_async_copy(wphi_hbm, wphi_ref, sems.at[0])

    def cp_w(m):
        cols = pl.ds(m * D, D)
        return pltpu.make_async_copy(wqkv_hbm.at[:, cols], wqkv.at[:, cols], wsems.at[m])

    def cp_x(c):
        rows = pl.ds(c * XC if isinstance(c, int) else pl.multiple_of(c * XC, XC), XC)
        return pltpu.make_async_copy(x_hbm.at[rows], xin.at[rows], xsems.at[c])

    cp_wo = pltpu.make_async_copy(wo_hbm, woa, sems.at[2])
    cp_mem = pltpu.make_async_copy(mem0_hbm, mem0_ref, sems.at[3])
    cp_big = [
        pltpu.make_async_copy(wqt_hbm, wt.at[0], sems.at[4]),
        pltpu.make_async_copy(wkt_hbm, wt.at[1], sems.at[5]),
        pltpu.make_async_copy(wvt_hbm, wt.at[2], sems.at[6]),
    ]
    OC = HB * DB // NOC

    def cp_bwo(c):
        rows = pl.ds(pl.multiple_of(c * OC, OC), OC)
        return pltpu.make_async_copy(bwo_hbm.at[rows], wt.at[3, rows], osems.at[c])

    def start_in_order(copies):
        def start(c, carry):
            for n, cp in enumerate(copies):
                pl.when(c == n)(cp.start)
            return carry

        jax.lax.fori_loop(0, len(copies), start, 0)

    start_in_order([cp_phi, cp_x(0), cp_w(0), cp_w(1), cp_w(2)] + [cp_x(c) for c in range(1, NXC)])

    def clear(c, carry):
        xres[pl.ds(pl.multiple_of(c * 128, 128), 128), :] = jnp.zeros((128, D), F32)
        return carry

    jax.lax.fori_loop(TB // 128, S // 128, clear, 0)
    cp_phi.wait()

    wphi = wphi_ref[...].astype(F32)
    xw = jnp.concatenate([wphi[d] for d in range(DA)], axis=1)
    xw = jnp.concatenate([xw, jnp.zeros((32 - DA, D), F32)], axis=0).astype(BF16)
    r = _iota((D, D), 0)
    c = _iota((D, D), 1)
    perm = jnp.where((r & 31) * DA + (r >> 5) == c, 1.0, 0.0).astype(BF16)
    wf = _dot(xw, perm).astype(BF16)
    r = _iota((160, 32), 0)
    c = _iota((160, 32), 1)
    rsel = jnp.where(((r - _div40(r) * 40) >> 1) == c, 1.0, 0.0).astype(BF16)
    r = _iota((160, 128), 0)
    c = _iota((160, 128), 1)
    phit = []
    for t in range(5):
        keep = 2 * (_div40(r) + 3 * t) + (r & 1) == _div20(c + 128 * t)
        phit.append(jnp.where(keep, _dot(rsel, wf[:, 128 * t:128 * (t + 1)]), 0.0).astype(BF16))

    kvacc[...] = jnp.zeros_like(kvacc)

    cp_x(0).wait()

    def init_blk(i, carry):
        for u in range(4):
            off = pl.multiple_of(i * 256 + u * 64, 64)
            x = xin[pl.ds(off, 64), :].astype(F32)
            xres[pl.ds(off, 64), :] = x
            xnb[pl.ds(pl.multiple_of(off // 2, 32), 32), :] = pltpu.bitcast(_ln(x).astype(BF16), U32)
        return carry

    jax.lax.fori_loop(0, XC // 256, init_blk, 0)
    start_in_order([cp_big[0], cp_big[1], cp_wo, cp_mem, cp_big[2]])

    def start_bwo(c, carry):
        cp_bwo(c).start()
        return carry

    jax.lax.fori_loop(0, NOC, start_bwo, 0)
    for m, dst in ((0, 1), (1, 0)):
        cp_w(m).wait()
        p = [_dot_nt(phit[t], wqkv[:, m * D + 128 * t:m * D + 128 * (t + 1)]) for t in range(5)]
        rows = [p[0][0:120]]
        for t in range(1, 5):
            rows += [p[t - 1][120:160] + p[t][0:40], p[t][40:120]]
        rows.append(p[4][120:160])
        w = jnp.concatenate(rows, axis=0)
        sub = _iota((8, D), 0)
        groups = []
        for j in range(16):
            ref = jnp.where(sub < 2, w[40 * j:40 * j + 8], 0.0)
            ref = ref + pltpu.roll(ref, 2, 0)
            ref = ref + pltpu.roll(ref, 4, 0)
            groups.append([w[40 * j + 8 * t:40 * j + 8 * (t + 1)] - ref for t in range(5)])
        rows = []
        for g in range(4):
            for t in range(3):
                rows.append(jnp.where(sub < 2, pltpu.roll(groups[4 * g + 3][0], 6 - 2 * t, 0),
                                      groups[4 * g + t][0]))
            for t in range(4):
                rows += groups[4 * g + t][1:]
        wat[dst, 0:NF // 2, :] = pltpu.bitcast(jnp.concatenate(rows, axis=0).astype(BF16), U32)
    cp_w(2).wait()
    wat[2] = pltpu.bitcast(wqkv[:, 2 * D:3 * D].T, U32)

    def weight_tile(m, j, t):
        off = j * 384 + t * 128
        if not isinstance(off, int):
            off = pl.multiple_of(off, 128)
        return pltpu.bitcast(wt[m, pl.ds(off, 128), :].T, U32)

    def token(*ys):
        return functools.reduce(
            jnp.maximum, [y[:, 128 * t:128 * (t + 1)] for y in ys for t in range(5)])

    def pack_wo(slot, c, tie=lambda w: w):
        bwo[pl.ds(pl.multiple_of(c * (OC // 2), OC // 2), OC // 2), :] = tie(pltpu.bitcast(
            wt[slot, pl.ds(pl.multiple_of(c * OC, OC), OC), :], U32))

    def layer_a(l):
        def sub_all(x, op):
            x = op(x, pltpu.roll(x, 2, 0))
            return op(x, pltpu.roll(x, 4, 0))

        def features(m, x):
            p = _dot_nt(pltpu.bitcast(wat[m, 0:NF // 2, :], BF16), x)
            p = [p[8 * t:8 * (t + 1)] for t in range(NF // 8)]
            sub = _iota((8, 128), 0)
            out = []
            for j in range(16):
                g, t = divmod(j, 4)
                pg = p[19 * g:19 * (g + 1)]
                if t < 3:
                    head = pg[t]
                else:
                    head = jnp.where(sub < 4, pltpu.roll(pg[0], 2, 0),
                                     jnp.where(sub < 6, pltpu.roll(pg[1], 4, 0),
                                               pltpu.roll(pg[2], 6, 0)))
                out.append([jnp.where(sub < 2, 0.0, head)] + pg[3 + 4 * t:7 + 4 * t])
            return out

        def phi(ts):
            mx = sub_all(functools.reduce(jnp.maximum, ts), jnp.maximum)
            mn = sub_all(functools.reduce(jnp.minimum, ts), jnp.minimum)
            ep = [jnp.exp(t - mx) for t in ts]
            en = [jnp.exp(mn - t) for t in ts]
            rp = 1.0 / sub_all(functools.reduce(jnp.add, ep), jnp.add)
            rn = 1.0 / sub_all(functools.reduce(jnp.add, en), jnp.add)
            return jnp.concatenate([e * rp for e in ep] + [e * rn for e in en], axis=0).astype(BF16)

        def phase1(i, carry):
            @pl.when(jnp.logical_and(l == 0, i < NXC - 1))
            def _():
                cp_x(i + 1).wait()

            off = pl.multiple_of(i * TB, TB)
            xn = pltpu.bitcast(xnb[pl.ds(pl.multiple_of(i * (TB // 2), TB // 2), TB // 2), :], BF16)
            xs = [xn[128 * u:128 * (u + 1)] for u in range(TB // 128)]
            nblk = jnp.minimum(i + 1, S // TB - 1)
            nrows = pl.ds(pl.multiple_of(nblk * TB, TB), TB)
            xnext = jnp.where(l == 0, xin[nrows, :].astype(F32), xres[nrows, :])
            ys = [_ln(xnext[16 * k:16 * (k + 1)]) for k in range(TB // 16)]
            xres[nrows, :] = xnext
            xnb[pl.ds(pl.multiple_of(nblk * (TB // 2), TB // 2), TB // 2), :] = pltpu.bitcast(
                jnp.concatenate([y.astype(BF16) for y in ys], axis=0), U32)

            for u, x in enumerate(xs):
                for j, ts in enumerate(features(1, x)):
                    phiq[j, :, pl.ds(off + 128 * u, 128)] = pltpu.bitcast(phi(ts), U32)
            phik = [[phi(ts) for ts in features(0, x)] for x in xs]
            vt = [_dot_nt(pltpu.bitcast(wat[2], BF16), x) for x in xs]
            ones = jnp.ones((8, 128), F32)
            tok = token(*ys[0:8])
            tied = jnp.where(i < 0, jnp.maximum(tok[0:8], tok[8:16]), ones)
            for u in range(len(xs)):
                for j in range(16):
                    lhs = jnp.concatenate(
                        [vt[u][40 * j:40 * (j + 1)], ones if u + j else tied], axis=0).astype(BF16)
                    kvacc[j] = _dot_nt(lhs, phik[u][j]) + kvacc[j]
            return carry

        jax.lax.fori_loop(0, S // TB, phase1, 0)

        @pl.when(l == 0)
        def _():
            cp_big[0].wait()
            cp_big[1].wait()
            cp_wo.wait()
            cp_mem.wait()

        rr = _iota((48, 80), 0)
        cc = _iota((48, 80), 1)
        keep = jnp.where(rr < 40, _div20(rr), (rr - 40) >> 2) == (cc & 1)
        kvm = [jnp.where(keep, kvacc[j], 0.0).astype(BF16) for j in range(16)]
        lo4 = _iota((8, TC), 0) < 4
        opend[...] = jnp.zeros_like(opend)
        kvacc[...] = jnp.zeros_like(kvacc)
        for j in range(NPRE):
            for t in range(3):
                wpre[3 * j + t] = weight_tile(0, JPRE + j, t)

        def num(b):
            parts = []
            for j in range(16):
                r = _dot(kvm[j], pltpu.bitcast(phiq[j, :, TC * b:TC * (b + 1)], BF16))
                rc = 1.0 / (r[40:48] + 1e-6)
                rc2 = pltpu.roll(rc, 4, 0)
                ra = jnp.where(lo4, rc, rc2)
                rb = jnp.where(lo4, rc2, rc)
                parts += [r[0:8] * ra, r[8:16] * ra, r[16:24] * rc, r[24:32] * rb, r[32:40] * rb]
            return jnp.concatenate(parts, axis=0).astype(BF16).T

        for b in range(S // TC):
            obuf[TC // 2 * b:TC // 2 * (b + 1), :] = pltpu.bitcast(num(b), U32)

        def out(i, carry):
            @pl.when(jnp.logical_and(l == 0, i == 2))
            def _():
                cp_big[2].wait()

            @pl.when(jnp.logical_and(l == 0, i >= 2))
            def _():
                for c in range(NH):
                    cp_bwo((i - 2) * NH + c).wait()

            for n in range(3 * NPAIR // 4):
                unit = i * (3 * NPAIR // 4) + n
                m, j = unit >> 4, unit & (NPAIR - 1)
                for t in range(3):
                    wb[9 * j + 3 * m + t] = weight_tile(m, j, t)
            xn32[0:RB, :] = _ln(xres[0:RB, :])
            rows = pl.ds(pl.multiple_of(i * TB, TB), TB)
            o = pltpu.bitcast(obuf[pl.ds(pl.multiple_of(i * (TB // 2), TB // 2), TB // 2), :], BF16)
            x = xres[rows, :]
            nb = TB // 64
            pick = lambda y, gs: jnp.concatenate([y[16 * g:16 * (g + 1)] for g in gs], axis=0)
            first = [g for g in range(4 * nb) if g % 4 == 2]
            rest = [g for g in range(4 * nb) if g % 4 != 2]
            xs = _dot(pick(o, first), woa[...]) + pick(x, first)
            memv[...] = mem0_ref[...].astype(F32)
            xo = _dot(pick(o, rest), woa[...]) + pick(x, rest)
            for c in range(NH):
                pack_wo(jnp.where(i < 2, 0, 3), (i & 1) * NH + c,
                        lambda w: jnp.where(i < 0, pltpu.bitcast(xo, U32), w))
            order = first + rest
            xres[rows, :] = pick(jnp.concatenate([xs, xo], axis=0),
                                 [order.index(g) for g in range(4 * nb)])
            wq = jnp.concatenate(
                [pltpu.bitcast(wpre[t], BF16) for t in range(3 * NPRE)], axis=1)
            qpre[pl.ds(pl.multiple_of(i * (8 * nb), 8 * nb), 8 * nb), :] = pltpu.bitcast(
                _dot(_ln(xs).astype(BF16), wq).astype(BF16), U32)
            return carry

        jax.lax.fori_loop(0, S // TB, out, 0)

        @pl.when(l == 0)
        def _():
            def cpo(c, carry):
                cp_bwo(c).wait()
                pack_wo(3, c)
                return carry

            jax.lax.fori_loop(2 * NH, NOC, cpo, 0)

    scale = DB ** (-0.5)

    def layer_b(layer):
        L = SEG + NM
        NEG = -1000000000.0

        def masks(even):
            nrow = SEG if even else L + 8
            rr = _iota((nrow, 128), 0)
            cc = _iota((nrow, 128), 1)
            is_a = (cc < L) | ((cc >= 2 * L) & (cc < 2 * L + 16))
            kx = jnp.where(cc < L, cc, cc - (L + NM))
            is_memkey = (cc >= SEG) & (cc < SEG + 2 * NM)
            if even:
                valid = cc < 2 * L
                allowed = valid & (is_memkey | (rr >= 24) | (kx <= rr + 8))
            else:
                dk = (cc - 2 * L) & 15
                cur = (rr < L) & (cc < 2 * L)
                old = (rr >= L) & (cc >= 2 * L) & (cc < 2 * L + 32)
                valid = cur | old
                allowed = ((cur & (is_memkey | (rr >= SEG) | (kx <= rr)))
                           | (old & ((dk >= 8) | (dk <= rr - L))))
            return is_a, allowed, jnp.where(valid, NEG, -jnp.inf).astype(F32)

        all_masks = {True: masks(True), False: masks(False)}

        def lo64(y):
            return _iota(y.shape, 1) < 64

        def stack_keys(a, b):
            parts = [a[0:L], b[SEG:L], b[0:SEG]]
            if a.shape[0] > L:
                parts += [a[L:], b[L:]]
            return jnp.concatenate(parts, axis=0).astype(BF16)

        def expand(y):
            y0, y1, y2 = y[:, 0:128], y[:, 128:256], y[:, 256:384]
            return (stack_keys(y0, y2),
                    stack_keys(jnp.where(lo64(y1), y1, 0.0), jnp.where(lo64(y1), 0.0, y1)))

        def pad_lanes(s):
            return jnp.concatenate([s, jnp.zeros((s.shape[0], 128 - s.shape[1]), F32)], axis=1)

        def step(hq, hkv, even, kmajor, side=None, never=None, pre=None):
            is_a, allowed, fill = all_masks[even]
            nrow = SEG if even else L + 8
            nkey = 2 * L if even else 2 * L + 32

            def tiles(j, ts):
                return jnp.concatenate([pltpu.bitcast(wb[9 * j + t], BF16) for t in ts], axis=1)

            def proj(j):
                if j == 0 and kmajor:
                    wq, wkv = tiles(j, range(3)), tiles(j, range(3, 9))
                    q = _dot(hq[:, 0:128], wq[0:128])
                    y = _dot(hkv[:, 0:128], wkv[0:128])
                    for t in range(1, 5):
                        ks = slice(128 * t, 128 * (t + 1))
                        q = _dot(hq[:, ks], wq[ks]) + q
                        y = _dot(hkv[:, ks], wkv[ks]) + y
                else:
                    ahead = pre is not None and JPRE <= j < JPRE + NPRE
                    q = _dot(hq[16:] if ahead else hq, tiles(j, range(3)))
                    y = _dot(hkv, tiles(j, range(3, 9)))
                if even:
                    snext[j] = y[SEG:L]
                    sdef[j, 0:8, :] = y[0:8]
                    sdef[j, 8:16, :] = y[L:L + 8]
                    kv = jnp.concatenate([y[0:SEG], y[L:L + 8]], axis=0)
                else:
                    kv = jnp.concatenate([snext[j], y, sdef[j]], axis=0)
                q = q.astype(BF16)
                if q.shape[0] < nrow:
                    c0 = 384 * (j - JPRE)
                    q = jnp.concatenate(
                        [pltpu.bitcast(qpre[pre, c0:c0 + 384], BF16), q], axis=0)
                q = (jnp.concatenate([q[:, 0:128], q[:, 256:384]], axis=0), q[:, 128:256])
                return q, expand(kv[:, 0:384]), expand(kv[:, 384:768])

            def scores(q, k, tok=None):
                s02 = pad_lanes(_dot_nt(q[0], k[0]))
                s = jnp.where(is_a, s02[0:nrow], s02[nrow:]) + pad_lanes(_dot_nt(q[1], k[1]))
                s = jnp.where(allowed, s * scale, fill)
                ma = jnp.max(jnp.where(is_a, s, -jnp.inf), axis=1, keepdims=True)
                mb = jnp.max(jnp.where(is_a, -jnp.inf, s), axis=1, keepdims=True)
                e = jnp.exp(s - jnp.where(is_a, ma, mb))
                ea = jnp.where(is_a, e, 0.0)
                eb = jnp.where(is_a, 0.0, e)
                pa = ea * (1.0 / jnp.sum(ea, axis=1, keepdims=True))
                pb = eb * (1.0 / jnp.sum(eb, axis=1, keepdims=True))
                if tok is not None:
                    pb = jnp.concatenate([jnp.where(never, tok, pb[0:16]), pb[16:]], axis=0)
                return (jnp.concatenate([pa, pb], axis=0)[:, 0:nkey].astype(BF16),
                        (pa + pb)[:, 0:nkey].astype(BF16))

            def pv(p, v):
                o02 = _dot(p[0], v[0])
                return jnp.concatenate(
                    [o02[0:nrow], _dot(p[1], v[1]), o02[nrow:]], axis=1).astype(BF16)

            qkv = [None] * NPAIR
            ps = [None] * NPAIR
            os_ = [None] * NPAIR

            def wo_chunk(t0, t1):
                w = pltpu.bitcast(bwo[64 * t0:64 * t1, :], BF16)
                o = jnp.concatenate(
                    [os_[t // 3][:, 128 * (t % 3):128 * (t % 3 + 1)] for t in range(t0, t1)], axis=1)
                return _dot(o, w)

            cuts = (0, 12, 24, 33, 42, 48) if even else (32, 34, 38, 42, 45, 48)
            lag = NPAIR if even else 4
            qkv[0] = proj(0)
            acc = None
            for j in range(NPAIR + 2):
                c = None
                if j + 1 < NPAIR:
                    qkv[j + 1] = proj(j + 1)
                    if j >= lag:
                        c = wo_chunk(3 * (j - lag), min(3 * (j - lag + 1), cuts[0]))
                else:
                    c = wo_chunk(cuts[j + 1 - NPAIR], cuts[j + 2 - NPAIR])
                if c is not None:
                    acc = c if acc is None else c + acc
                if j < NPAIR:
                    ps[j] = scores(qkv[j][0], qkv[j][1], side(j) if side else None)
                if j >= 2:
                    os_[j - 2] = pv(ps[j - 2], qkv[j - 2][2])
            acc = wo_chunk(cuts[3], cuts[4]) + acc
            return wo_chunk(cuts[4], cuts[5]) + acc

        def finish_rows(base, r0, n):
            rows = pl.ds(base + r0, n)
            xnew = xres[rows, :] + opend[r0:r0 + n, :]
            xres[rows, :] = xnew
            xin[rows, :] = xnew.astype(BF16)
            y = _ln(xnew)
            xnb[pl.ds(pl.multiple_of(base // 2, RB // 2) + r0 // 2, n // 2), :] = pltpu.bitcast(
                y.astype(BF16), U32)
            return y

        def body(i, carry):
            base = pl.multiple_of(i * RB, RB)

            @pl.when(jnp.logical_and(layer == 1, i >= 2))
            def _():
                rows = pl.ds(pl.multiple_of((i - 2) * RB, RB), RB)
                pltpu.make_async_copy(xin.at[rows], out_hbm.at[rows], sems.at[0]).start()

            prev = pl.multiple_of(jnp.maximum(i - 1, 0) * RB, RB)
            nxt = pl.multiple_of(jnp.minimum(i + 1, S // RB - 1) * RB, RB)

            def side_prev(j):
                if j % 2:
                    return None
                return token(finish_rows(prev, 8 * j, 16))

            def side_next(j):
                if j % 2:
                    return None
                rows = pl.ds(nxt + 8 * j, 16)
                y = _ln(xres[rows, :])
                xn32[rows, :] = y
                return token(y)

            sides = (side_prev, side_next)
            never = i < 0
            mem = memv[...]
            for u in range(UNROLL):
                r0 = 64 * u
                xr = lambda a, n: xn32[pl.ds(base + r0 + a, n), :]
                cat = lambda *p: jnp.concatenate(p, axis=0).astype(BF16)
                o0 = step(cat(xr(8, 24), mem), cat(xr(0, 40), mem), True, u > 0, sides[u], never)
                opend[r0 + 8:r0 + 32, :] = o0[0:24]
                mem = o0[24:32]
                o1 = step(cat(xr(32, 32), mem, xr(0, 8)), cat(xr(40, 24), mem), False, True,
                          pre=pl.ds(pl.multiple_of(i * (8 * UNROLL), 8) + 8 * u, 8))
                mem = o1[32:40]
                opend[r0:r0 + 8, :] = o1[40:48]
                opend[r0 + 32:r0 + 64, :] = o1[0:32]
            memv[...] = mem
            return carry

        jax.lax.fori_loop(0, S // RB, body, 0)

        @pl.when(layer == 0)
        def _():
            xres[S - RB:S, :] = xres[S - RB:S, :] + opend[...]

    def layer(l, carry):
        layer_a(l)
        layer_b(l)
        return carry

    jax.lax.fori_loop(0, 2, layer, 0)

    rows = pl.ds(S - 2 * RB, RB)
    pltpu.make_async_copy(xin.at[rows], out_hbm.at[rows], sems.at[0]).start()
    rows = pl.ds(S - RB, RB)
    xin[rows, :] = (xres[rows, :] + opend[...]).astype(BF16)
    pltpu.make_async_copy(xin.at[rows], out_hbm.at[rows], sems.at[0]).start()
    pltpu.make_async_copy(xin, out_hbm, sems.at[0]).wait()


@jax.jit
def pallas_interleave_layers__linear_kernel_hedgehog__memory_aug_recurrent_mem_tr__prompt_kernel(
    A_x: jax.Array,
    A_wqkv: jax.Array,
    A_w_phi: jax.Array,
    A_wo: jax.Array,
    B_x: jax.Array,
    B_mem0: jax.Array,
    B_Wq: jax.Array,
    B_Wk: jax.Array,
    B_Wv: jax.Array,
    B_Wo: jax.Array,
    B_seg_len: jax.Array,
):
    assert A_x.shape == (1, S, D) and B_mem0.shape == (1, NM, D) and B_Wq.shape == (D, HB, DB)
    tr = lambda w: jnp.transpose(w, (1, 2, 0)).reshape(HB * DB, D)
    any_spec = pl.BlockSpec(memory_space=pl.ANY)
    out = pl.pallas_call(
        _kernel,
        out_shape=jax.ShapeDtypeStruct((S, D), BF16),
        in_specs=[any_spec] * 9,
        out_specs=any_spec,
        scratch_shapes=[
            pltpu.VMEM((DA, DA, HA), BF16),
            pltpu.VMEM((NM, D), BF16),
            pltpu.VMEM((S, D), BF16),
            pltpu.VMEM((D, 3 * D), BF16),
            pltpu.VMEM((D, D), BF16),
            pltpu.VMEM((4, HB * DB, D), BF16),
            pltpu.VMEM((9 * NPAIR, D // 2, 128), U32),
            pltpu.VMEM((HB * DB // 2, D), U32),
            pltpu.VMEM((S, D), F32),
            pltpu.VMEM((S, D), F32),
            pltpu.VMEM((S // 2, D), U32),
            pltpu.VMEM((3, D // 2, D), U32),
            pltpu.VMEM((16, 48, 80), F32),
            pltpu.VMEM((16, 40, S), U32),
            pltpu.VMEM((S // 2, D), U32),
            pltpu.VMEM((3 * NPRE, D // 2, 128), U32),
            pltpu.VMEM((S // 8, 384 * NPRE), U32),
            pltpu.VMEM((NM, D), F32),
            pltpu.VMEM((NPAIR, 8, 6 * 128), F32),
            pltpu.VMEM((NPAIR, 16, 6 * 128), F32),
            pltpu.VMEM((64 * UNROLL, D), F32),
            pltpu.SemaphoreType.DMA((7,)),
            pltpu.SemaphoreType.DMA((NXC,)),
            pltpu.SemaphoreType.DMA((NOC,)),
            pltpu.SemaphoreType.DMA((3,)),
        ],
        compiler_params=pltpu.CompilerParams(vmem_limit_bytes=120 * 1024 * 1024),
    )(A_x.reshape(S, D), A_wqkv, jnp.transpose(A_w_phi, (1, 2, 0)), A_wo,
      B_mem0.reshape(NM, D), tr(B_Wq), tr(B_Wk), tr(B_Wv), B_Wo.reshape(HB * DB, D))
    return out.reshape(1, S, D)
```
